```python
import jax
import jax.numpy as jnp

def _softmax(x, axis=-1):
    return jax.nn.softmax(x, axis=axis)

def _gelu(x):
    return jax.nn.gelu(x, approximate=True)

def _silu(x):
    return jax.nn.silu(x)

def _sigmoid(x):
    return jax.nn.sigmoid(x)

def _layernorm(x, axis=-1, eps=1e-05):
    m = jnp.mean(x, axis=axis, keepdims=True)
    v = jnp.var(x, axis=axis, keepdims=True)
    return (x - m) / jnp.sqrt(v + eps)

def _scatter_add(tgt, idx, src, axis=0):
    return tgt.at[idx].add(src)

def _segment_sum(src, seg, n):
    return jax.ops.segment_sum(src, seg, n)

class _Rng:

    def __init__(self, key):
        self._k = key

    def _next(self):
        self._k, sub = jax.random.split(self._k)
        return sub

    def normal(self, shape):
        return jax.random.normal(self._next(), shape, dtype=jnp.bfloat16)

    def randint(self, lo, hi, shape):
        return jax.random.randint(self._next(), shape, lo, hi, dtype=jnp.int32)

    def uniform(self, shape, lo=0.0, hi=1.0):
        return jax.random.uniform(self._next(), shape, jnp.bfloat16, lo, hi)

    def permutation(self, n):
        return jax.random.permutation(self._next(), n)
kernel_name = 'adaLN_cond__gqa_block_cached__moe_arch_mod__prompt'

def setup_inputs():
    _rng = _Rng(jax.random.key(int.from_bytes(__import__("os").urandom(4), "little")))
    _w = lambda a: (lambda t: t.astype(jnp.bfloat16) if jnp.issubdtype(t.dtype, jnp.floating) else t)(jnp.asarray(a))

    def _A_setup():
        B, Sq, D = (1, 2048, 576)
        Hq, Hkv, Sk, Dh = (32, 16, 2048, 128)
        assert Hq % Hkv == 0, (Hq, Hkv)
        return {'x': _w((lambda *s: _rng.normal(s) * 0.05)(B, Sq, D)), 'k_cache': _w((lambda *s: _rng.normal(s) * 0.05)(B, Hkv, Sk, Dh)), 'v_cache': _w((lambda *s: _rng.normal(s) * 0.05)(B, Hkv, Sk, Dh)), 'wq': _w((lambda *s: _rng.normal(s) * 0.05)(D, Hq * Dh) * D ** (-0.5)), 'wo': _w((lambda *s: _rng.normal(s) * 0.05)(Hq * Dh, D) * (Hq * Dh) ** (-0.5))}
    _A_in = _A_setup()

    def _B_setup():
        B, S, D, F, C = (1, 2048, 576, 4608, 8)
        return {'x': _w((lambda *s: _rng.normal(s) * 0.05)(B, S, D)), 'w_r': _w((lambda *s: _rng.normal(s) * 0.05)(D)), 'w_gate': _w((lambda *s: _rng.normal(s) * 0.05)(D, F)), 'w_up': _w((lambda *s: _rng.normal(s) * 0.05)(D, F)), 'w_down': _w((lambda *s: _rng.normal(s) * 0.05)(F, D))}
    _B_in = _B_setup()
    return {'A_x': _A_in['x'], 'A_k_cache': _A_in['k_cache'], 'A_v_cache': _A_in['v_cache'], 'A_wq': _A_in['wq'], 'A_wo': _A_in['wo'], 'B_x': _B_in['x'], 'B_w_r': _B_in['w_r'], 'B_w_gate': _B_in['w_gate'], 'B_w_up': _B_in['w_up'], 'B_w_down': _B_in['w_down'], 'c': _w((lambda *s: _rng.normal(s) * 0.05)(1, 576)), 'w_mod': _w((lambda *s: _rng.normal(s) * 0.05)(576, 6 * 576) * 576 ** (-0.5))}

def reference(A_x, A_k_cache, A_v_cache, A_wq, A_wo, B_x, B_w_r, B_w_gate, B_w_up, B_w_down, c, w_mod):

    def _A_ref(x, k_cache, v_cache, wq, wo):
        B, Sq, D = x.shape
        Hq, Dh = (32, 128)
        Hkv = k_cache.shape[1]
        rep = Hq // Hkv
        q = (lambda x, *d: x.transpose(*d))((x @ wq).reshape(B, Sq, Hq, Dh), 0, 2, 1, 3)
        k = jnp.repeat(k_cache, rep, axis=1)
        v = jnp.repeat(v_cache, rep, axis=1)
        scores = jnp.einsum('bhqd,bhkd->bhqk', q, k) * Dh ** (-0.5)
        p = _softmax(scores, axis=-1)
        o = jnp.einsum('bhqk,bhkd->bhqd', p, v)
        return (lambda x, *d: x.transpose(*d))(o, 0, 2, 1, 3).reshape(B, Sq, Hq * Dh) @ wo

    def _B_ref(x, w_r, w_gate, w_up, w_down):
        B, S, D = x.shape
        C = 8
        r = x @ w_r
        idx = jnp.argsort(-r, axis=-1)[:, :C]
        idx_e = jnp.repeat(idx.reshape(B, C, 1), D, axis=2)
        x_sel = jnp.take_along_axis(x, idx_e, axis=1)
        g = _silu(x_sel @ w_gate)
        u = x_sel @ w_up
        y = g * u @ w_down
        r_sel = _sigmoid(jnp.take_along_axis(r, idx, axis=1))
        y = y * r_sel.reshape(B, C, 1)
        b_off = (jnp.arange(B) * S).reshape(B, 1)
        flat_idx = (idx + b_off).reshape(B * C)
        zero = (x * 0.0).reshape(B * S, D)
        upd = _scatter_add(zero, flat_idx, y.reshape(B * C, D), axis=0)
        return x + upd.reshape(B, S, D)
    x = A_x
    mod = (_silu(c) @ w_mod).reshape(c.shape[0], 6, 1, -1)
    sa, ca, ga, sb, cb, gb = (mod[:, 0].copy(), mod[:, 1].copy(), mod[:, 2].copy(), mod[:, 3].copy(), mod[:, 4].copy(), mod[:, 5].copy())
    h = _layernorm(x, axis=-1) * (1 + ca) + sa
    x = x + ga * _A_ref(h, A_k_cache, A_v_cache, A_wq, A_wo)
    h = _layernorm(x, axis=-1) * (1 + cb) + sb
    x = x + gb * _B_ref(h, B_w_r, B_w_gate, B_w_up, B_w_down)
    return x
```

```python
import contextlib
import jax
import jax.numpy as jnp
from jax import lax
import numpy as np
import jax.experimental.pallas as pl
import jax.experimental.pallas.tpu as pltpu

D = 576
S = 2048
HKV = 16
DH = 128
FF = 4608
C = 8
EPS = 1e-5
T = 128
NRB = S // T
NPER = 2 * NRB
F32 = jnp.float32
BF16 = jnp.bfloat16
NT = (((1,), (1,)), ((), ()))
QSCALE = float(DH ** -0.5 * np.log2(np.e))
LMIN = float(2.0 ** -90)
KT = [(0, 128), (128, 256), (256, 384), (384, 512), (512, 576)]
M1 = 2 * D


def _r(x):
    return x.astype(BF16).astype(F32)


def _col(row):
    return jnp.broadcast_to(row, (T, D)).T


def _sum8(x):
    return jnp.sum(x.reshape(x.shape[0] // 8, 8, x.shape[1]), axis=0)


def base_order(lag, oppos, qppos):
    toks = []
    for t in range(16 + lag):
        if t < 16: toks.append(('QK', t))
        if t - lag >= 0: toks.append(('PV', t - lag))
    assert oppos < len(toks) and qppos < len(toks)
    out = []
    for i, tk in enumerate(toks):
        if i == oppos: out += [('OP', j) for j in range(4)]
        if i == qppos: out += [('QP', j) for j in range(5)]
        out.append(tk)
    return out


def make(lag=8, oppos=30, qppos=8, flags=None, nb=18, **kw):
    seq = kw.get('seq') or base_order(lag, oppos, qppos)
    NKV, NW = 2, 3

    def kernel(xT_hbm, k_hbm, v_hbm, wq_hbm, woT_hbm, wr_hbm, wg_hbm, wu_hbm, wdT_hbm, c_hbm, wmod_hbm, outT_hbm,
               x_c, k_v, v_v, wq_v, wo_v, wr_v, c_v, wm1_v, wm2_v, wg_v, wu_v, wd_v,
               modr, modc, h_v, acc, dlt, q0, q1, o0, o1, h2c, out_c, r_v, x1s,
               qs, ss, ms, ls, os_, chk_v, xsem, sems):
        q_scr = (q0, q1)
        o_scr = (o0, o1)
        (S_K, S_V, S_WQ, S_WO, S_WR, S_C, S_WM1, S_WM2, S_WG, S_WU, S_WD, S_WO0, S_WQ0, S_WQ1) = range(14)

        def scope(name):
            return jax.named_scope(name) if kw.get('scopes') else contextlib.nullcontext()

        class Two:
            def __init__(self, a, b): self.a, self.b = a, b
            def start(self): self.a.start(); self.b.start()
            def wait(self): self.a.wait(); self.b.wait()

        def cp_k(j): return pltpu.make_async_copy(k_hbm.at[j], k_v.at[j % NKV], sems.at[S_K])
        def cp_v(j): return pltpu.make_async_copy(v_hbm.at[j], v_v.at[j % NKV], sems.at[S_V])
        def cp_w1(src, dst, sem, j, hb):
            return pltpu.make_async_copy(src.at[:, pl.ds(pl.multiple_of(j * 256 + hb * T, T), T)],
                                         dst.at[2 * (j % NW) + hb], sems.at[sem])
        def cp_w(src, dst, sem, j): return Two(cp_w1(src, dst, sem, j, 0), cp_w1(src, dst, sem, j, 1))
        def cp_wq(j): return cp_w(wq_hbm, wq_v, S_WQ, j)
        def cp_wo(j): return cp_w(woT_hbm, wo_v, S_WO, j)
        cp_wo0 = cp_w(woT_hbm, wo_v, S_WO0, 0)
        def cp_x(rb):
            cols = slice(rb * T, (rb + 1) * T) if isinstance(rb, int) else pl.ds(pl.multiple_of(rb * T, T), T)
            return pltpu.make_async_copy(xT_hbm.at[:, cols], x_c.at[rb], xsem.at[rb])
        def cp_o(rb): return pltpu.make_async_copy(out_c.at[rb], outT_hbm.at[:, rb * T:(rb + 1) * T], xsem.at[rb])
        cp_wr = pltpu.make_async_copy(wr_hbm, wr_v, sems.at[S_WR])
        cp_c = pltpu.make_async_copy(c_hbm, c_v, sems.at[S_C])
        cp_wm1 = pltpu.make_async_copy(wmod_hbm.at[:, 0:M1], wm1_v, sems.at[S_WM1])
        cp_wm2 = pltpu.make_async_copy(wmod_hbm.at[:, M1:6 * D], wm2_v, sems.at[S_WM2])
        cp_wg = pltpu.make_async_copy(wg_hbm, wg_v, sems.at[S_WG])
        cp_wu = pltpu.make_async_copy(wu_hbm, wu_v, sems.at[S_WU])
        cp_wd = pltpu.make_async_copy(wdT_hbm, wd_v, sems.at[S_WD])

        def wsl(ref, j, rows, hb):
            return ref[2 * (j % NW) + hb, rows, :]

        RBK = D // nb

        def ln1_thunks(rb):
            st = {}
            th = []
            def ph_a(b):
                x = x_c[rb, b * RBK:(b + 1) * RBK, :].astype(F32)
                if b > 0:
                    x = (x.reshape(RBK // 8, 8, T) + (st['s'] * 0.0)[None]).reshape(RBK, T)
                t = _sum8(x)
                st['s'] = t if b == 0 else st['s'] + t
                if b == nb - 1:
                    st['m'] = jnp.broadcast_to(jnp.sum(st['s'], axis=0, keepdims=True) * (1.0 / D), (8, T))
            def ph_b(b):
                m = st['m']
                if b > 0: m = m + st['v'] * 0.0
                xc = x_c[rb, b * RBK:(b + 1) * RBK, :].astype(F32).reshape(RBK // 8, 8, T) - m[None]
                t = jnp.sum(xc * xc, axis=0)
                st['v'] = t if b == 0 else st['v'] + t
                if b == nb - 1:
                    st['rs'] = lax.rsqrt(jnp.sum(st['v'], axis=0, keepdims=True) * (1.0 / D) + EPS)
            def ph_c(k):
                k0, k1 = KT[k]
                m = st['m']
                if k > 0: m = m + st['z'] * 0.0
                n8 = (k1 - k0) // 8
                xc = (x_c[rb, k0:k1, :].astype(F32).reshape(n8, 8, T) - m[None]).reshape(k1 - k0, T)
                xh = xc * st['rs']
                st['z'] = xh[0:8, :]
                h = xh.T * modr[0:1, k0:k1] + modr[1:2, k0:k1]
                h_v[k, slice(rb * T, (rb + 1) * T) if isinstance(rb, int) else pl.ds(pl.multiple_of(rb * T, T), T), 0:k1 - k0] = h.astype(BF16)
            for b in range(nb): th.append(lambda b=b: ph_a(b))
            for b in range(nb): th.append(lambda b=b: ph_b(b))
            for k in range(5): th.append(lambda k=k: ph_c(k))
            return th

        def ln2_thunks(rb):
            st = {}
            th = []
            def ph_a(b):
                rows = slice(b * RBK, (b + 1) * RBK)
                xin = x_c[rb, rows, :].astype(F32)
                a = acc[rb, rows, :] + dlt[rb, rows, :]
                if b > 0:
                    a = (a.reshape(RBK // 8, 8, T) + (st['s'] * 0.0)[None]).reshape(RBK, T)
                x1 = xin + modc[0, rows, :] * a
                x1s[rows, :] = x1
                t = _sum8(x1)
                st['s'] = t if b == 0 else st['s'] + t
                if b == nb - 1:
                    st['m'] = jnp.broadcast_to(jnp.sum(st['s'], axis=0, keepdims=True) * (1.0 / D), (8, T))
            def ph_b(b):
                m = st['m']
                if b > 0: m = m + st['v'] * 0.0
                xm = x1s[b * RBK:(b + 1) * RBK, :].reshape(RBK // 8, 8, T) - m[None]
                t = jnp.sum(xm * xm, axis=0)
                st['v'] = t if b == 0 else st['v'] + t
                if b == nb - 1:
                    v = _r(jnp.sum(st['v'], axis=0, keepdims=True) * (1.0 / D))
                    st['rd'] = 1.0 / _r(jnp.sqrt(_r(v + EPS)))
                    st['mr'] = _r(st['m'])
            def ph_c(b):
                rows = slice(b * RBK, (b + 1) * RBK)
                x1 = x1s[rows, :]
                mr = st['mr']
                if b > 0: mr = mr + st['r'] * 0.0
                xc = (x1.reshape(RBK // 8, 8, T) - mr[None]).reshape(RBK, T)
                h2 = xc * st['rd'] * modc[2, rows, :] + modc[1, rows, :]
                t = _sum8(h2 * modc[4, rows, :])
                st['r'] = t if b == 0 else st['r'] + t
                h2c[rb, rows, :] = h2.astype(BF16)
                out_c[rb, rows, :] = (x1 + modc[3, rows, :] * h2).astype(BF16)
                if b == nb - 1:
                    r_v[pl.ds(rb, 1), :] = _r(jnp.sum(st['r'], axis=0, keepdims=True))
            for b in range(nb): th.append(lambda b=b: ph_a(b))
            for b in range(nb): th.append(lambda b=b: ph_b(b))
            for b in range(nb): th.append(lambda b=b: ph_c(b))
            return th

        def mod2():
            cc = c_v[...].astype(F32)
            sc8 = jnp.broadcast_to(cc * jax.nn.sigmoid(cc), (8, D)).astype(BF16)
            mod = _r(jnp.dot(sc8, wm2_v[...], preferred_element_type=F32))
            for t in range(4):
                row = mod[0:1, t * D:(t + 1) * D]
                if t == 2: row = _r(1.0 + row)
                modc[t] = _col(row)
            modc[4] = _col(wr_v[...].reshape(1, D).astype(F32))

        def qp_tile(j, hb, rows, t):
            k0, k1 = KT[t]
            return jnp.dot(h_v[t, rows, 0:k1 - k0], wsl(wq_v, j, slice(k0, k1), hb), preferred_element_type=F32)

        def op_piece(j, hb, o_ref, rb, t, mode):
            rows = slice(t * 144, (t + 1) * 144)
            u = lax.dot_general(wsl(wo_v, j, rows, hb), o_ref[...], NT, preferred_element_type=F32)
            if mode == 'zero':
                acc[rb, rows, :] = jnp.zeros((144, T), F32)
            elif mode == 'commit':
                acc[rb, rows, :] += dlt[rb, rows, :]
            else:
                u = dlt[rb, rows, :] + u
            dlt[rb, rows, :] = u

        def period(j, par, chk, opspec, qpspec, th):
            st = dict(l=None, o=None, q=None)
            ps = {}
            extra = {}
            n = len(seq)
            for i_, f_ in enumerate(th):
                extra.setdefault((i_ * n) // max(len(th), 1), []).append(f_)
            for i, (name, t) in enumerate(seq):
                for f_ in extra.get(i, []):
                    f_()
                if name == 'QK':
                    s = lax.dot_general(q_scr[par][...], k_v[j % NKV, t * T:(t + 1) * T, :], NT, preferred_element_type=F32)
                    p = jnp.exp2(s)
                    st['l'] = p if st['l'] is None else st['l'] + p
                    ps[t] = p.astype(BF16)
                elif name == 'PV':
                    o = jnp.dot(ps[t], v_v[j % NKV, t * T:(t + 1) * T, :], preferred_element_type=F32)
                    st['o'] = o if st['o'] is None else st['o'] + o
                    if t == 15:
                        l = jnp.sum(st['l'], axis=1, keepdims=True)
                        on = st['o'] * (1.0 / l)
                        o_scr[par][...] = on.astype(BF16)
                        lb = jnp.broadcast_to(l, (T, T))
                        chk['lmin'] = jnp.minimum(chk['lmin'], jnp.min(lb.reshape(T // 8, 8, T), axis=0))
                        chk['z'] = chk['z'] + _sum8(on + lb)
                elif name == 'OP':
                    op_piece(opspec[0], opspec[1], o_scr[1 - par], opspec[2], t, opspec[3])
                elif name == 'QP':
                    jq, hq, rbq = qpspec
                    rows = slice(rbq * T, (rbq + 1) * T) if isinstance(rbq, int) else pl.ds(pl.multiple_of(rbq * T, T), T)
                    d = qp_tile(jq, hq, rows, t)
                    st['q'] = d if st['q'] is None else st['q'] + d
                    if t == 4:
                        q_scr[1 - par][...] = (st['q'] * QSCALE).astype(BF16)

        def chk_new():
            return dict(lmin=jnp.full((8, T), 1.0, F32), z=jnp.zeros((8, T), F32))

        def chk_flush(chk, first):
            if first:
                chk_v[0:8, :] = chk['lmin']
                chk_v[8:16, :] = chk['z']
            else:
                chk_v[0:8, :] = jnp.minimum(chk_v[0:8, :], chk['lmin'])
                chk_v[8:16, :] = chk_v[8:16, :] + chk['z']

        def mid_step(j):
            chk = chk_new()
            for c in range(NPER):
                opspec = (j, (c - 1) % 2, (c - 1) // 2, 'add' if (c - 1) % 2 else 'commit') if c >= 1 else (j - 1, 1, NRB - 1, 'add')
                qpspec = (j, (c + 1) % 2, (c + 1) // 2) if c + 1 < NPER else (j + 1, 0, 0)
                period(j, c % 2, chk, opspec, qpspec, [])
            chk_flush(chk, True)

        def edge_step(j, kind):
            chk_flush(chk_new(), True)
            def body(it, carry):
                chk = chk_new()
                if kind == 'first':
                    edge_dma(it)
                    ra = jnp.minimum(2 * it + 2, NRB - 1)
                    rb_ = jnp.minimum(2 * it + 3, NRB - 1)
                    tha, thb = ln1_thunks(ra), ln1_thunks(rb_)
                else:
                    ra = jnp.maximum(2 * it - 2, 0)
                    rb_ = jnp.maximum(2 * it - 1, 0)
                    tha, thb = ln2_thunks(ra), ln2_thunks(rb_)
                ths = [tha[:len(tha) // 2], tha[len(tha) // 2:], thb[:len(thb) // 2], thb[len(thb) // 2:]]
                mode = 'zero' if kind == 'first' else 'commit'
                for c in range(4):
                    if c == 0:
                        if kind == 'first':
                            opspec = (j, 1, jnp.maximum(2 * it - 1, 0), 'add')
                        else:
                            opspec = (jnp.where(it == 0, j - 1, j), 1, (2 * it + NRB - 1) % NRB, 'add')
                    else:
                        opspec = (j, (c - 1) % 2, 2 * it + (c - 1) // 2, 'add' if (c - 1) % 2 else mode)
                    if c < 3:
                        qpspec = (j, (c + 1) % 2, 2 * it + (c + 1) // 2)
                    elif kind == 'first':
                        qpspec = (jnp.where(it == 7, j + 1, j), 0, (2 * it + 2) % NRB)
                    else:
                        qpspec = (j, 0, jnp.minimum(2 * it + 2, NRB - 1))
                    period(j, c % 2, chk, opspec, qpspec, ths[c])
                chk_flush(chk, False)
                return carry
            lax.fori_loop(0, NRB // 2, body, 0)

        def edge_dma(it):
            @pl.when(it < 6)
            def _():
                cp_x(2 * it + 4).start(); cp_x(2 * it + 5).start()
            @pl.when(it < 7)
            def _():
                cp_x(2 * it + 2).wait(); cp_x(2 * it + 3).wait()
            @pl.when(it == 1)
            def _():
                cp_wq(1).start(); cp_wr.start()
            @pl.when(it == 2)
            def _():
                cp_k(1).start(); cp_v(1).start()
            @pl.when(it == 3)
            def _():
                cp_wo(1).start(); cp_wq(2).start()
            @pl.when(it == 4)
            def _():
                cp_wm2.start()
            @pl.when(it == 7)
            def _():
                cp_wq(1).wait()

        def slow_step(j):
            def body(c, carry):
                rb = c // 2
                hb = c % 2
                rows = pl.ds(pl.multiple_of(rb * T, T), T)
                q = None
                for t_ in range(5):
                    d = qp_tile(j, hb, rows, t_)
                    q = d if q is None else q + d
                qs[...] = (q * QSCALE).astype(BF16)
                ms[...] = jnp.full((T, T), -jnp.inf, F32)
                def p1(t, carry_):
                    keys = pl.ds(pl.multiple_of(t * T, T), T)
                    s_ = lax.dot_general(qs[...], k_v[j % NKV, keys, :], NT, preferred_element_type=F32)
                    ss[t] = s_
                    ms[...] = jnp.maximum(ms[...], s_)
                    return carry_
                lax.fori_loop(0, S // T, p1, 0)
                ms[...] = jnp.broadcast_to(jnp.max(ms[...], axis=1, keepdims=True), (T, T))
                ls[...] = jnp.zeros((T, T), F32)
                os_[...] = jnp.zeros((T, T), F32)
                def p2(t, carry_):
                    keys = pl.ds(pl.multiple_of(t * T, T), T)
                    p = jnp.exp2(ss[t] - ms[...])
                    ls[...] += p
                    os_[...] += jnp.dot(p.astype(BF16), v_v[j % NKV, keys, :], preferred_element_type=F32)
                    return carry_
                lax.fori_loop(0, S // T, p2, 0)
                l = jnp.sum(ls[...], axis=1, keepdims=True)
                o1[...] = (os_[...] * (1.0 / l)).astype(BF16)
                @pl.when(c < NPER - 1)
                def _():
                    def po(t, carry_):
                        r_ = pl.ds(pl.multiple_of(t * 144, 16), 144)
                        u = lax.dot_general(wsl(wo_v, j, r_, hb), o1[...], NT, preferred_element_type=F32)
                        dlt[rb, r_, :] = jnp.where(hb == 0, 0.0, dlt[rb, r_, :]) + u
                        return carry_
                    lax.fori_loop(0, 4, po, 0)
                    @pl.when(jnp.logical_and(j == HKV - 1, hb == 1))
                    def _():
                        for f_ in ln2_thunks(rb):
                            f_()
                return carry
            with scope('SLOW'):
                lax.fori_loop(0, NPER, body, 0)

        cp_c.start(); cp_x(0).start(); cp_wm1.start()
        cp_w1(wq_hbm, wq_v, S_WQ0, 0, 0).start()
        cp_k(0).start()
        cp_x(1).start()
        cp_w1(wq_hbm, wq_v, S_WQ1, 0, 1).start()
        cp_v(0).start()
        cp_wo0.start()
        o1[...] = jnp.zeros((T, DH), BF16)
        dlt[0] = jnp.zeros((D, T), F32)
        with scope('pro0'):
            cp_x(0).wait()
            th0 = ln1_thunks(0)
            for f_ in th0[:2 * nb]:
                f_()
            cp_c.wait(); cp_wm1.wait()
            cc = c_v[...].astype(F32)
            sc8 = jnp.broadcast_to(cc * jax.nn.sigmoid(cc), (8, D)).astype(BF16)
            mod = _r(jnp.dot(sc8, wm1_v[...], preferred_element_type=F32))
            modr[0:1, :] = 1.0 + mod[0:1, D:2 * D]
            modr[1:2, :] = mod[0:1, 0:D]
            for f_ in th0[2 * nb:]:
                f_()
            cp_w1(wq_hbm, wq_v, S_WQ0, 0, 0).wait()
            q = None
            for t in range(5):
                d = qp_tile(0, 0, slice(0, T), t)
                q = d if q is None else q + d
            q0[...] = (q * QSCALE).astype(BF16)
        cp_x(2).start(); cp_x(3).start()
        with scope('pro1'):
            cp_x(1).wait()
            for f_ in ln1_thunks(1):
                f_()
            cp_w1(wq_hbm, wq_v, S_WQ1, 0, 1).wait(); cp_k(0).wait(); cp_v(0).wait(); cp_wo0.wait()

        def step(j, carry):
            @pl.when(j == 0)
            def _():
                with scope('first'):
                    edge_step(0, 'first')
            @pl.when(jnp.logical_and(j > 0, j < HKV - 1))
            def _():
                with scope('wait'):
                    cp_k(j).wait(); cp_v(j).wait(); cp_wo(j).wait(); cp_wq(j + 1).wait()
                cp_k(j + 1).start(); cp_v(j + 1).start(); cp_wo(j + 1).start()
                @pl.when(j + 2 < HKV)
                def _(): cp_wq(j + 2).start()
                @pl.when(j == 1)
                def _():
                    cp_wm2.wait(); cp_wr.wait()
                    mod2()
                    cp_wg.start()
                @pl.when(j == 2)
                def _(): cp_wu.start()
                @pl.when(j == 3)
                def _(): cp_wd.start()
                with scope('midbody'):
                    mid_step(j)
            @pl.when(j == HKV - 1)
            def _():
                cp_k(HKV - 1).wait(); cp_v(HKV - 1).wait(); cp_wo(HKV - 1).wait()
                with scope('last'):
                    edge_step(HKV - 1, 'last')
            ok = jnp.where((chk_v[0:8, :] >= LMIN) & (jnp.abs(chk_v[8:16, :]) < jnp.inf), 1.0, 0.0)
            @pl.when(jnp.min(ok) < 0.5)
            def _():
                slow_step(j)
            return carry
        lax.fori_loop(0, HKV, step, 0)
        jl = HKV - 1

        with scope('tail0'):
            for t in range(4):
                op_piece(jl, 1, o1, NRB - 1, t, 'add')
            def ln2_tail(rb, carry):
                for f_ in ln2_thunks(rb):
                    f_()
                return carry
            lax.fori_loop(NRB - 2, NRB, ln2_tail, 0)
        with scope('topk'):
            rb_ = pltpu.bitcast(r_v[...], jnp.int32) >> 16
            u = jnp.where(rb_ < 0, ~rb_, rb_ | 0x8000) & 0xFFFF
            tok = lax.broadcasted_iota(jnp.int32, (NRB, T), 0) * T + lax.broadcasted_iota(jnp.int32, (NRB, T), 1)
            key = pltpu.bitcast(((u << 11) | (S - 1 - tok)) + (1 << 27), F32)
            subs = lax.broadcasted_iota(jnp.int32, (8, T), 0)
            lane = lax.broadcasted_iota(jnp.int32, (8, T), 1)
            ksel = jnp.zeros((8, T), jnp.int32)
            for t in range(C):
                mx = jnp.max(jnp.max(key, axis=0, keepdims=True), axis=1, keepdims=True)
                key = jnp.where(key == mx, 0.0, key)
                ksel = jnp.where(subs == t, pltpu.bitcast(jnp.broadcast_to(mx, (8, T)), jnp.int32), ksel)
            ksel = ksel - (1 << 27)
            idxv = (S - 1) - (ksel & (S - 1))
            uu = ksel >> 11
            rbits = jnp.where((uu & 0x8000) != 0, uu & 0x7FFF, (~uu) & 0xFFFF) << 16
            rsel = pltpu.bitcast(rbits, F32)
            idxs = [jnp.max(jnp.where(subs == t, idxv, 0).astype(F32)).astype(jnp.int32) for t in range(C)]
        with scope('gather'):
            xs = None
            for t in range(C):
                oh = jnp.where((subs == t) & (lane == (idxv & (T - 1))), 1.0, 0.0).astype(BF16)
                n_t = jnp.clip(idxs[t] // T, 0, NRB - 1)
                d = lax.dot_general(oh, h2c[n_t], NT, preferred_element_type=F32)
                xs = d if xs is None else xs + d
        cp_wg.wait(); cp_wu.wait(); cp_wd.wait()
        with scope('ffn'):
            xb = xs.astype(BF16)
            g = _r(jnp.dot(xb, wg_v[...], preferred_element_type=F32))
            u_ = _r(jnp.dot(xb, wu_v[...], preferred_element_type=F32))
            g = _r(g * jax.nn.sigmoid(g))
            a = (g * u_).astype(BF16)
            y = _r(lax.dot_general(a, wd_v[...], NT, preferred_element_type=F32))
            y = _r(y * _r(jax.nn.sigmoid(rsel[:, 0:1])))
        with scope('fix'):
            yT = jnp.concatenate([y, jnp.zeros((T - 8, D), F32)], axis=0).T.astype(BF16)
            rowk = lax.broadcasted_iota(jnp.int32, (T, T), 0)
            lanes = lax.broadcasted_iota(jnp.int32, (T, T), 1)
            for t in range(C):
                n_t = jnp.clip(idxs[t] // T, 0, NRB - 1)
                sel = jnp.where((rowk == t) & (lanes == (idxs[t] & (T - 1))), 1.0, 0.0).astype(BF16)
                for p_ in range(4):
                    rows = slice(p_ * 144, (p_ + 1) * 144)
                    upd = jnp.dot(yT[rows, :], sel, preferred_element_type=F32)
                    out_c[n_t, rows, :] = (out_c[n_t, rows, :].astype(F32) + modc[3, rows, :] * upd).astype(BF16)
        with scope('wout'):
            for rb in range(NRB):
                cp_o(rb).start()
            for rb in range(NRB):
                cp_o(rb).wait()

    @jax.jit
    def fn(A_x, A_k_cache, A_v_cache, A_wq, A_wo, B_x, B_w_r, B_w_gate, B_w_up, B_w_down, c, w_mod):
        del B_x
        xT = A_x.reshape(S, D).T
        woT = A_wo.T
        wdT = B_w_down.T
        any_spec = pl.BlockSpec(memory_space=pl.ANY)
        outT = pl.pallas_call(
            kernel,
            in_specs=[any_spec] * 11,
            out_specs=any_spec,
            out_shape=jax.ShapeDtypeStruct((D, S), BF16),
            scratch_shapes=[
                pltpu.VMEM((NRB, D, T), BF16),
                pltpu.VMEM((NKV, S, DH), BF16),
                pltpu.VMEM((NKV, S, DH), BF16),
                pltpu.VMEM((2 * NW, D, T), BF16),
                pltpu.VMEM((2 * NW, D, T), BF16),
                pltpu.VMEM((D,), BF16),
                pltpu.VMEM((1, D), BF16),
                pltpu.VMEM((D, M1), BF16),
                pltpu.VMEM((D, 4 * D), BF16),
                pltpu.VMEM((D, FF), BF16),
                pltpu.VMEM((D, FF), BF16),
                pltpu.VMEM((D, FF), BF16),
                pltpu.VMEM((8, D), F32),
                pltpu.VMEM((5, D, T), F32),
                pltpu.VMEM((5, S, T), BF16),
                pltpu.VMEM((NRB, D, T), F32),
                pltpu.VMEM((NRB, D, T), F32),
                pltpu.VMEM((T, DH), BF16), pltpu.VMEM((T, DH), BF16),
                pltpu.VMEM((T, DH), BF16), pltpu.VMEM((T, DH), BF16),
                pltpu.VMEM((NRB, D, T), BF16),
                pltpu.VMEM((NRB, D, T), BF16),
                pltpu.VMEM((NRB, T), F32),
                pltpu.VMEM((D, T), F32),
                pltpu.VMEM((T, DH), BF16),
                pltpu.VMEM((S // T, T, T), F32),
                pltpu.VMEM((T, T), F32), pltpu.VMEM((T, T), F32), pltpu.VMEM((T, T), F32),
                pltpu.VMEM((16, T), F32),
                pltpu.SemaphoreType.DMA((NRB,)),
                pltpu.SemaphoreType.DMA((14,)),
            ],
            compiler_params=pltpu.CompilerParams(vmem_limit_bytes=110 * 1024 * 1024, flags=flags),
        )(xT, A_k_cache.reshape(HKV, S, DH), A_v_cache.reshape(HKV, S, DH), A_wq, woT,
          B_w_r, B_w_gate, B_w_up, wdT, c, w_mod)
        return outT.T.reshape(1, S, D)
    return fn


_KW = {}
_impl = make(**_KW)


@jax.jit
def pallas_adaLN_cond__gqa_block_cached__moe_arch_mod__prompt_kernel(
    A_x: jax.Array,
    A_k_cache: jax.Array,
    A_v_cache: jax.Array,
    A_wq: jax.Array,
    A_wo: jax.Array,
    B_x: jax.Array,
    B_w_r: jax.Array,
    B_w_gate: jax.Array,
    B_w_up: jax.Array,
    B_w_down: jax.Array,
    c: jax.Array,
    w_mod: jax.Array,
):
    return _impl(A_x, A_k_cache, A_v_cache, A_wq, A_wo, B_x, B_w_r, B_w_gate, B_w_up, B_w_down, c, w_mod)
```

```python
import contextlib
import jax
import jax.numpy as jnp
from jax import lax
import numpy as np
import jax.experimental.pallas as pl
import jax.experimental.pallas.tpu as pltpu

D = 576
S = 2048
HKV = 16
DH = 128
FF = 4608
C = 8
EPS = 1e-5
T = 128
NRB = S // T
NPER = 2 * NRB
F32 = jnp.float32
BF16 = jnp.bfloat16
NT = (((1,), (1,)), ((), ()))
QSCALE = float(DH ** -0.5 * np.log2(np.e))
LMIN = float(2.0 ** -90)
KT = [(0, 128), (128, 256), (256, 384), (384, 512), (512, 576)]
M1 = 2 * D


def _r(x):
    return x.astype(BF16).astype(F32)


def _col(row):
    return jnp.broadcast_to(row, (T, D)).T


def _sum8(x):
    return jnp.sum(x.reshape(x.shape[0] // 8, 8, x.shape[1]), axis=0)


def base_order(lag, oppos, qppos):
    toks = []
    for t in range(16 + lag):
        if t < 16: toks.append(('QK', t))
        if t - lag >= 0: toks.append(('PV', t - lag))
    assert oppos < len(toks) and qppos < len(toks)
    out = []
    for i, tk in enumerate(toks):
        if i == oppos: out += [('OP', j) for j in range(4)]
        if i == qppos: out += [('QP', j) for j in range(5)]
        out.append(tk)
    return out


def make(lag=8, oppos=30, qppos=8, flags=None, nb=18, **kw):
    seq = kw.get('seq') or base_order(lag, oppos, qppos)
    NKV, NW = 2, 3

    def kernel(xT_hbm, k_hbm, v_hbm, wq_hbm, woT_hbm, wr_hbm, wg_hbm, wu_hbm, wdT_hbm, c_hbm, wmod_hbm, outT_hbm,
               x_c, k_v, v_v, wq_v, wo_v, wr_v, c_v, wm1_v, wm2_v, wg_v, wu_v, wd_v,
               modr, modc, h_v, acc, dlt, q0, q1, o0, o1, h2c, out_c, r_v, x1s,
               qs, ss, ms, ls, os_, chk_v, xsem, sems):
        q_scr = (q0, q1)
        o_scr = (o0, o1)
        (S_K, S_V, S_WQ, S_WO, S_WR, S_C, S_WM1, S_WM2, S_WG, S_WU, S_WD, S_WO0, S_WQ0, S_WQ1) = range(14)

        def scope(name):
            return jax.named_scope(name) if kw.get('scopes') else contextlib.nullcontext()

        class Two:
            def __init__(self, a, b): self.a, self.b = a, b
            def start(self): self.a.start(); self.b.start()
            def wait(self): self.a.wait(); self.b.wait()

        def cp_k(j): return pltpu.make_async_copy(k_hbm.at[j], k_v.at[j % NKV], sems.at[S_K])
        def cp_v(j): return pltpu.make_async_copy(v_hbm.at[j], v_v.at[j % NKV], sems.at[S_V])
        def cp_w1(src, dst, sem, j, hb):
            return pltpu.make_async_copy(src.at[:, pl.ds(pl.multiple_of(j * 256 + hb * T, T), T)],
                                         dst.at[2 * (j % NW) + hb], sems.at[sem])
        def cp_w(src, dst, sem, j): return Two(cp_w1(src, dst, sem, j, 0), cp_w1(src, dst, sem, j, 1))
        def cp_wq(j): return cp_w(wq_hbm, wq_v, S_WQ, j)
        def cp_wo(j): return cp_w(woT_hbm, wo_v, S_WO, j)
        cp_wo0 = cp_w(woT_hbm, wo_v, S_WO0, 0)
        def cp_x(rb):
            cols = slice(rb * T, (rb + 1) * T) if isinstance(rb, int) else pl.ds(pl.multiple_of(rb * T, T), T)
            return pltpu.make_async_copy(xT_hbm.at[:, cols], x_c.at[rb], xsem.at[rb])
        def cp_o(rb):
            cols = slice(rb * T, (rb + 1) * T) if isinstance(rb, int) else pl.ds(pl.multiple_of(rb * T, T), T)
            return pltpu.make_async_copy(out_c.at[rb], outT_hbm.at[:, cols], xsem.at[rb])
        cp_wr = pltpu.make_async_copy(wr_hbm, wr_v, sems.at[S_WR])
        cp_c = pltpu.make_async_copy(c_hbm, c_v, sems.at[S_C])
        cp_wm1 = pltpu.make_async_copy(wmod_hbm.at[:, 0:M1], wm1_v, sems.at[S_WM1])
        cp_wm2 = pltpu.make_async_copy(wmod_hbm.at[:, M1:6 * D], wm2_v, sems.at[S_WM2])
        cp_wg = pltpu.make_async_copy(wg_hbm, wg_v, sems.at[S_WG])
        cp_wu = pltpu.make_async_copy(wu_hbm, wu_v, sems.at[S_WU])
        cp_wd = pltpu.make_async_copy(wdT_hbm, wd_v, sems.at[S_WD])

        def wsl(ref, j, rows, hb):
            return ref[2 * (j % NW) + hb, rows, :]

        RBK = D // nb

        def ln1_thunks(rb, chain=True):
            st = {}
            th = []
            def ph_a(b):
                x = x_c[rb, b * RBK:(b + 1) * RBK, :].astype(F32)
                if b > 0 and chain:
                    x = (x.reshape(RBK // 8, 8, T) + (st['s'] * 0.0)[None]).reshape(RBK, T)
                t = _sum8(x)
                st['s'] = t if b == 0 else st['s'] + t
                if b == nb - 1:
                    st['m'] = jnp.broadcast_to(jnp.sum(st['s'], axis=0, keepdims=True) * (1.0 / D), (8, T))
            def ph_b(b):
                m = st['m']
                if b > 0 and chain: m = m + st['v'] * 0.0
                xc = x_c[rb, b * RBK:(b + 1) * RBK, :].astype(F32).reshape(RBK // 8, 8, T) - m[None]
                t = jnp.sum(xc * xc, axis=0)
                st['v'] = t if b == 0 else st['v'] + t
                if b == nb - 1:
                    st['rs'] = lax.rsqrt(jnp.sum(st['v'], axis=0, keepdims=True) * (1.0 / D) + EPS)
            def ph_c(k):
                k0, k1 = KT[k]
                m = st['m']
                if k > 0 and chain: m = m + st['z'] * 0.0
                n8 = (k1 - k0) // 8
                xc = (x_c[rb, k0:k1, :].astype(F32).reshape(n8, 8, T) - m[None]).reshape(k1 - k0, T)
                xh = xc * st['rs']
                st['z'] = xh[0:8, :]
                h = xh.T * modr[0:1, k0:k1] + modr[1:2, k0:k1]
                h_v[k, slice(rb * T, (rb + 1) * T) if isinstance(rb, int) else pl.ds(pl.multiple_of(rb * T, T), T), 0:k1 - k0] = h.astype(BF16)
            for b in range(nb): th.append(lambda b=b: ph_a(b))
            for b in range(nb): th.append(lambda b=b: ph_b(b))
            for k in range(5): th.append(lambda k=k: ph_c(k))
            return th

        def ln2_thunks(rb, chain=True):
            st = {}
            th = []
            def ph_a(b):
                rows = slice(b * RBK, (b + 1) * RBK)
                xin = x_c[rb, rows, :].astype(F32)
                a = acc[rb, rows, :] + dlt[rb, rows, :]
                if b > 0 and chain:
                    a = (a.reshape(RBK // 8, 8, T) + (st['s'] * 0.0)[None]).reshape(RBK, T)
                x1 = xin + modc[0, rows, :] * a
                x1s[rows, :] = x1
                t = _sum8(x1)
                st['s'] = t if b == 0 else st['s'] + t
                if b == nb - 1:
                    st['m'] = jnp.broadcast_to(jnp.sum(st['s'], axis=0, keepdims=True) * (1.0 / D), (8, T))
            def ph_b(b):
                m = st['m']
                if b > 0 and chain: m = m + st['v'] * 0.0
                xm = x1s[b * RBK:(b + 1) * RBK, :].reshape(RBK // 8, 8, T) - m[None]
                t = jnp.sum(xm * xm, axis=0)
                st['v'] = t if b == 0 else st['v'] + t
                if b == nb - 1:
                    v = _r(jnp.sum(st['v'], axis=0, keepdims=True) * (1.0 / D))
                    st['rd'] = 1.0 / _r(jnp.sqrt(_r(v + EPS)))
                    st['mr'] = _r(st['m'])
            def ph_c(b):
                rows = slice(b * RBK, (b + 1) * RBK)
                x1 = x1s[rows, :]
                mr = st['mr']
                if b > 0 and chain: mr = mr + st['r'] * 0.0
                xc = (x1.reshape(RBK // 8, 8, T) - mr[None]).reshape(RBK, T)
                h2 = xc * st['rd'] * modc[2, rows, :] + modc[1, rows, :]
                t = _sum8(h2 * modc[4, rows, :])
                st['r'] = t if b == 0 else st['r'] + t
                h2c[rb, rows, :] = h2.astype(BF16)
                out_c[rb, rows, :] = (x1 + modc[3, rows, :] * h2).astype(BF16)
                if b == nb - 1:
                    r_v[pl.ds(rb, 1), :] = _r(jnp.sum(st['r'], axis=0, keepdims=True))
            for b in range(nb): th.append(lambda b=b: ph_a(b))
            for b in range(nb): th.append(lambda b=b: ph_b(b))
            for b in range(nb): th.append(lambda b=b: ph_c(b))
            return th

        def mod2():
            cc = c_v[...].astype(F32)
            sc8 = jnp.broadcast_to(cc * jax.nn.sigmoid(cc), (8, D)).astype(BF16)
            mod = _r(jnp.dot(sc8, wm2_v[...], preferred_element_type=F32))
            for t in range(4):
                row = mod[0:1, t * D:(t + 1) * D]
                if t == 2: row = _r(1.0 + row)
                modc[t] = _col(row)
            modc[4] = _col(wr_v[...].reshape(1, D).astype(F32))

        def qp_tile(j, hb, rows, t):
            k0, k1 = KT[t]
            return jnp.dot(h_v[t, rows, 0:k1 - k0], wsl(wq_v, j, slice(k0, k1), hb), preferred_element_type=F32)

        def op_piece(j, hb, o_ref, rb, t, mode):
            rows = slice(t * 144, (t + 1) * 144)
            u = lax.dot_general(wsl(wo_v, j, rows, hb), o_ref[...], NT, preferred_element_type=F32)
            if mode == 'zero':
                acc[rb, rows, :] = jnp.zeros((144, T), F32)
            elif mode == 'commit':
                acc[rb, rows, :] += dlt[rb, rows, :]
            else:
                u = dlt[rb, rows, :] + u
            dlt[rb, rows, :] = u

        def period(j, par, chk, opspec, qpspec, th):
            st = dict(l=None, o=None, q=None)
            ps = {}
            extra = {}
            n = len(seq)
            for i_, f_ in enumerate(th):
                extra.setdefault((i_ * n) // max(len(th), 1), []).append(f_)
            for i, (name, t) in enumerate(seq):
                for f_ in extra.get(i, []):
                    f_()
                if name == 'QK':
                    s = lax.dot_general(q_scr[par][...], k_v[j % NKV, t * T:(t + 1) * T, :], NT, preferred_element_type=F32)
                    p = jnp.exp2(s)
                    st['l'] = p if st['l'] is None else st['l'] + p
                    ps[t] = p.astype(BF16)
                elif name == 'PV':
                    o = jnp.dot(ps[t], v_v[j % NKV, t * T:(t + 1) * T, :], preferred_element_type=F32)
                    st['o'] = o if st['o'] is None else st['o'] + o
                    if t == 15:
                        l = jnp.sum(st['l'], axis=1, keepdims=True)
                        on = st['o'] * (1.0 / l)
                        o_scr[par][...] = on.astype(BF16)
                        lb = jnp.broadcast_to(l, (T, T))
                        chk['lmin'] = jnp.minimum(chk['lmin'], jnp.min(lb.reshape(T // 8, 8, T), axis=0))
                        chk['z'] = chk['z'] + _sum8(on + lb)
                elif name == 'OP':
                    op_piece(opspec[0], opspec[1], o_scr[1 - par], opspec[2], t, opspec[3])
                elif name == 'QP':
                    jq, hq, rbq = qpspec
                    rows = slice(rbq * T, (rbq + 1) * T) if isinstance(rbq, int) else pl.ds(pl.multiple_of(rbq * T, T), T)
                    d = qp_tile(jq, hq, rows, t)
                    st['q'] = d if st['q'] is None else st['q'] + d
                    if t == 4:
                        q_scr[1 - par][...] = (st['q'] * QSCALE).astype(BF16)

        def chk_new():
            return dict(lmin=jnp.full((8, T), 1.0, F32), z=jnp.zeros((8, T), F32))

        def chk_flush(chk, first):
            if first:
                chk_v[0:8, :] = chk['lmin']
                chk_v[8:16, :] = chk['z']
            else:
                chk_v[0:8, :] = jnp.minimum(chk_v[0:8, :], chk['lmin'])
                chk_v[8:16, :] = chk_v[8:16, :] + chk['z']

        def mid_step(j):
            chk = chk_new()
            for c in range(NPER):
                opspec = (j, (c - 1) % 2, (c - 1) // 2, 'add' if (c - 1) % 2 else 'commit') if c >= 1 else (j - 1, 1, NRB - 1, 'add')
                qpspec = (j, (c + 1) % 2, (c + 1) // 2) if c + 1 < NPER else (j + 1, 0, 0)
                period(j, c % 2, chk, opspec, qpspec, [])
            chk_flush(chk, True)

        def edge_step(j, kind):
            chk_flush(chk_new(), True)
            def body(it, carry):
                chk = chk_new()
                if kind == 'first':
                    edge_dma(it)
                    ra = jnp.minimum(2 * it + 2, NRB - 1)
                    rb_ = jnp.minimum(2 * it + 3, NRB - 1)
                    tha, thb = ln1_thunks(ra), ln1_thunks(rb_)
                else:
                    ra = jnp.maximum(2 * it - 2, 0)
                    rb_ = jnp.maximum(2 * it - 1, 0)
                    tha, thb = ln2_thunks(ra), ln2_thunks(rb_)
                ths = [tha[:len(tha) // 2], tha[len(tha) // 2:], thb[:len(thb) // 2], thb[len(thb) // 2:]]
                mode = 'zero' if kind == 'first' else 'commit'
                for c in range(4):
                    if c == 0:
                        if kind == 'first':
                            opspec = (j, 1, jnp.maximum(2 * it - 1, 0), 'add')
                        else:
                            opspec = (jnp.where(it == 0, j - 1, j), 1, (2 * it + NRB - 1) % NRB, 'add')
                    else:
                        opspec = (j, (c - 1) % 2, 2 * it + (c - 1) // 2, 'add' if (c - 1) % 2 else mode)
                    if c < 3:
                        qpspec = (j, (c + 1) % 2, 2 * it + (c + 1) // 2)
                    elif kind == 'first':
                        qpspec = (jnp.where(it == 7, j + 1, j), 0, (2 * it + 2) % NRB)
                    else:
                        qpspec = (j, 0, jnp.minimum(2 * it + 2, NRB - 1))
                    period(j, c % 2, chk, opspec, qpspec, ths[c])
                chk_flush(chk, False)
                if kind == 'last':
                    @pl.when(it >= 1)
                    def _():
                        cp_o(2 * it - 2).start(); cp_o(2 * it - 1).start()
                return carry
            lax.fori_loop(0, NRB // 2, body, 0)

        def edge_dma(it):
            @pl.when(it < 6)
            def _():
                cp_x(2 * it + 4).start(); cp_x(2 * it + 5).start()
            @pl.when(it < 7)
            def _():
                cp_x(2 * it + 2).wait(); cp_x(2 * it + 3).wait()
            @pl.when(it == 1)
            def _():
                cp_wq(1).start(); cp_wr.start()
            @pl.when(it == 2)
            def _():
                cp_k(1).start(); cp_v(1).start()
            @pl.when(it == 3)
            def _():
                cp_wo(1).start(); cp_wq(2).start()
            @pl.when(it == 4)
            def _():
                cp_wm2.start()
            @pl.when(it == 7)
            def _():
                cp_wq(1).wait()

        def slow_step(j):
            def body(c, carry):
                rb = c // 2
                hb = c % 2
                rows = pl.ds(pl.multiple_of(rb * T, T), T)
                q = None
                for t_ in range(5):
                    d = qp_tile(j, hb, rows, t_)
                    q = d if q is None else q + d
                qs[...] = (q * QSCALE).astype(BF16)
                ms[...] = jnp.full((T, T), -jnp.inf, F32)
                def p1(t, carry_):
                    keys = pl.ds(pl.multiple_of(t * T, T), T)
                    s_ = lax.dot_general(qs[...], k_v[j % NKV, keys, :], NT, preferred_element_type=F32)
                    ss[t] = s_
                    ms[...] = jnp.maximum(ms[...], s_)
                    return carry_
                lax.fori_loop(0, S // T, p1, 0)
                ms[...] = jnp.broadcast_to(jnp.max(ms[...], axis=1, keepdims=True), (T, T))
                ls[...] = jnp.zeros((T, T), F32)
                os_[...] = jnp.zeros((T, T), F32)
                def p2(t, carry_):
                    keys = pl.ds(pl.multiple_of(t * T, T), T)
                    p = jnp.exp2(ss[t] - ms[...])
                    ls[...] += p
                    os_[...] += jnp.dot(p.astype(BF16), v_v[j % NKV, keys, :], preferred_element_type=F32)
                    return carry_
                lax.fori_loop(0, S // T, p2, 0)
                l = jnp.sum(ls[...], axis=1, keepdims=True)
                o1[...] = (os_[...] * (1.0 / l)).astype(BF16)
                @pl.when(c < NPER - 1)
                def _():
                    def po(t, carry_):
                        r_ = pl.ds(pl.multiple_of(t * 144, 16), 144)
                        u = lax.dot_general(wsl(wo_v, j, r_, hb), o1[...], NT, preferred_element_type=F32)
                        dlt[rb, r_, :] = jnp.where(hb == 0, 0.0, dlt[rb, r_, :]) + u
                        return carry_
                    lax.fori_loop(0, 4, po, 0)
                    @pl.when(jnp.logical_and(j == HKV - 1, hb == 1))
                    def _():
                        for f_ in ln2_thunks(rb, False):
                            f_()
                return carry
            with scope('SLOW'):
                lax.fori_loop(0, NPER, body, 0)

        cp_c.start(); cp_x(0).start(); cp_wm1.start()
        cp_w1(wq_hbm, wq_v, S_WQ0, 0, 0).start()
        def wave2():
            cp_k(0).start()
            cp_v(0).start()
            cp_x(1).start()
            cp_w1(wq_hbm, wq_v, S_WQ1, 0, 1).start()
            cp_wo0.start()
        if kw.get('stage', 1) == 0:
            wave2()
        o1[...] = jnp.zeros((T, DH), BF16)
        dlt[0] = jnp.zeros((D, T), F32)
        with scope('pro0'):
            cp_x(0).wait()
            th0 = ln1_thunks(0, False)
            for f_ in th0[:2 * nb]:
                f_()
            if kw.get('stage', 1) == 1:
                wave2()
            cp_c.wait(); cp_wm1.wait()
            if kw.get('stage', 1) == 2:
                wave2()
            cc = c_v[...].astype(F32)
            sc8 = jnp.broadcast_to(cc * jax.nn.sigmoid(cc), (8, D)).astype(BF16)
            mod = _r(jnp.dot(sc8, wm1_v[...], preferred_element_type=F32))
            modr[0:1, :] = 1.0 + mod[0:1, D:2 * D]
            modr[1:2, :] = mod[0:1, 0:D]
            for f_ in th0[2 * nb:]:
                f_()
            cp_w1(wq_hbm, wq_v, S_WQ0, 0, 0).wait()
            q = None
            for t in range(5):
                d = qp_tile(0, 0, slice(0, T), t)
                q = d if q is None else q + d
            q0[...] = (q * QSCALE).astype(BF16)
        cp_x(2).start(); cp_x(3).start()
        with scope('pro1'):
            cp_x(1).wait()
            for f_ in ln1_thunks(1, False):
                f_()
            cp_w1(wq_hbm, wq_v, S_WQ1, 0, 1).wait(); cp_k(0).wait(); cp_v(0).wait(); cp_wo0.wait()

        def step(j, carry):
            @pl.when(j == 0)
            def _():
                with scope('first'):
                    edge_step(0, 'first')
            @pl.when(jnp.logical_and(j > 0, j < HKV - 1))
            def _():
                with scope('wait'):
                    cp_k(j).wait(); cp_v(j).wait(); cp_wo(j).wait(); cp_wq(j + 1).wait()
                @pl.when(j + 2 < HKV)
                def _(): cp_wq(j + 2).start()
                @pl.when(j == 1)
                def _():
                    cp_wm2.wait(); cp_wr.wait()
                    mod2()
                    cp_wg.start()
                @pl.when(j == 2)
                def _(): cp_wu.start()
                @pl.when(j == 3)
                def _(): cp_wd.start()
                cp_k(j + 1).start(); cp_v(j + 1).start(); cp_wo(j + 1).start()
                with scope('midbody'):
                    mid_step(j)
            @pl.when(j == HKV - 1)
            def _():
                cp_k(HKV - 1).wait(); cp_v(HKV - 1).wait(); cp_wo(HKV - 1).wait()
                with scope('last'):
                    edge_step(HKV - 1, 'last')
            ok = jnp.where((chk_v[0:8, :] >= LMIN) & (jnp.abs(chk_v[8:16, :]) < jnp.inf), 1.0, 0.0)
            @pl.when(jnp.min(ok) < (2.0 if kw.get('forceslow') else 0.5))
            def _():
                @pl.when(j == HKV - 1)
                def _():
                    for rb in range(NRB - 2):
                        cp_o(rb).wait()
                slow_step(j)
                @pl.when(j == HKV - 1)
                def _():
                    for rb in range(NRB - 2):
                        cp_o(rb).start()
            return carry
        lax.fori_loop(0, HKV, step, 0)
        jl = HKV - 1

        with scope('tail0'):
            for t in range(4):
                op_piece(jl, 1, o1, NRB - 1, t, 'add')
            for f_ in ln2_thunks(NRB - 2, False):
                f_()
            cp_o(NRB - 2).start()
            for f_ in ln2_thunks(NRB - 1, False):
                f_()
            cp_o(NRB - 1).start()
        with scope('topk'):
            rb_ = pltpu.bitcast(r_v[...], jnp.int32) >> 16
            u = jnp.where(rb_ < 0, ~rb_, rb_ | 0x8000) & 0xFFFF
            tok = lax.broadcasted_iota(jnp.int32, (NRB, T), 0) * T + lax.broadcasted_iota(jnp.int32, (NRB, T), 1)
            key = pltpu.bitcast(((u << 11) | (S - 1 - tok)) + (1 << 27), F32)
            subs = lax.broadcasted_iota(jnp.int32, (8, T), 0)
            lane = lax.broadcasted_iota(jnp.int32, (8, T), 1)
            ksel = jnp.zeros((8, T), jnp.int32)
            for t in range(C):
                mx = jnp.max(jnp.max(key, axis=0, keepdims=True), axis=1, keepdims=True)
                key = jnp.where(key == mx, 0.0, key)
                ksel = jnp.where(subs == t, pltpu.bitcast(jnp.broadcast_to(mx, (8, T)), jnp.int32), ksel)
            ksel = ksel - (1 << 27)
            idxv = (S - 1) - (ksel & (S - 1))
            uu = ksel >> 11
            rbits = jnp.where((uu & 0x8000) != 0, uu & 0x7FFF, (~uu) & 0xFFFF) << 16
            rsel = pltpu.bitcast(rbits, F32)
            idxs = [jnp.max(jnp.where(subs == t, idxv, 0).astype(F32)).astype(jnp.int32) for t in range(C)]
        with scope('gather'):
            xs = None
            for t in range(C):
                oh = jnp.where((subs == t) & (lane == (idxv & (T - 1))), 1.0, 0.0).astype(BF16)
                n_t = jnp.clip(idxs[t] // T, 0, NRB - 1)
                d = lax.dot_general(oh, h2c[n_t], NT, preferred_element_type=F32)
                xs = d if xs is None else xs + d
        cp_wg.wait(); cp_wu.wait(); cp_wd.wait()
        with scope('ffn'):
            xb = xs.astype(BF16)
            g = _r(jnp.dot(xb, wg_v[...], preferred_element_type=F32))
            u_ = _r(jnp.dot(xb, wu_v[...], preferred_element_type=F32))
            g = _r(g * jax.nn.sigmoid(g))
            a = (g * u_).astype(BF16)
            y = _r(lax.dot_general(a, wd_v[...], NT, preferred_element_type=F32))
            y = _r(y * _r(jax.nn.sigmoid(rsel[:, 0:1])))
        with scope('fix'):
            yT = jnp.concatenate([y, jnp.zeros((T - 8, D), F32)], axis=0).T.astype(BF16)
            rowk = lax.broadcasted_iota(jnp.int32, (T, T), 0)
            lanes = lax.broadcasted_iota(jnp.int32, (T, T), 1)
            for rb in range(NRB):
                cp_o(rb).wait()
            tiles = [jnp.clip(idxs[t] // T, 0, NRB - 1) for t in range(C)]
            for t in range(C):
                sel = jnp.where((rowk == t) & (lanes == (idxs[t] & (T - 1))), 1.0, 0.0).astype(BF16)
                for p_ in range(4):
                    rows = slice(p_ * 144, (p_ + 1) * 144)
                    upd = jnp.dot(yT[rows, :], sel, preferred_element_type=F32)
                    out_c[tiles[t], rows, :] = (out_c[tiles[t], rows, :].astype(F32) + modc[3, rows, :] * upd).astype(BF16)
        with scope('wout'):
            fresh = []
            for t in range(C):
                f_ = jnp.bool_(True)
                for s_ in range(t):
                    f_ = jnp.logical_and(f_, tiles[s_] != tiles[t])
                fresh.append(f_)
                @pl.when(f_)
                def _(t=t):
                    cp_o(tiles[t]).start()
            for t in range(C):
                @pl.when(fresh[t])
                def _(t=t):
                    cp_o(tiles[t]).wait()

    @jax.jit
    def fn(A_x, A_k_cache, A_v_cache, A_wq, A_wo, B_x, B_w_r, B_w_gate, B_w_up, B_w_down, c, w_mod):
        del B_x
        xT = A_x.reshape(S, D).T
        woT = A_wo.T
        wdT = B_w_down.T
        any_spec = pl.BlockSpec(memory_space=pl.ANY)
        outT = pl.pallas_call(
            kernel,
            in_specs=[any_spec] * 11,
            out_specs=any_spec,
            out_shape=jax.ShapeDtypeStruct((D, S), BF16),
            scratch_shapes=[
                pltpu.VMEM((NRB, D, T), BF16),
                pltpu.VMEM((NKV, S, DH), BF16),
                pltpu.VMEM((NKV, S, DH), BF16),
                pltpu.VMEM((2 * NW, D, T), BF16),
                pltpu.VMEM((2 * NW, D, T), BF16),
                pltpu.VMEM((D,), BF16),
                pltpu.VMEM((1, D), BF16),
                pltpu.VMEM((D, M1), BF16),
                pltpu.VMEM((D, 4 * D), BF16),
                pltpu.VMEM((D, FF), BF16),
                pltpu.VMEM((D, FF), BF16),
                pltpu.VMEM((D, FF), BF16),
                pltpu.VMEM((8, D), F32),
                pltpu.VMEM((5, D, T), F32),
                pltpu.VMEM((5, S, T), BF16),
                pltpu.VMEM((NRB, D, T), F32),
                pltpu.VMEM((NRB, D, T), F32),
                pltpu.VMEM((T, DH), BF16), pltpu.VMEM((T, DH), BF16),
                pltpu.VMEM((T, DH), BF16), pltpu.VMEM((T, DH), BF16),
                pltpu.VMEM((NRB, D, T), BF16),
                pltpu.VMEM((NRB, D, T), BF16),
                pltpu.VMEM((NRB, T), F32),
                pltpu.VMEM((D, T), F32),
                pltpu.VMEM((T, DH), BF16),
                pltpu.VMEM((S // T, T, T), F32),
                pltpu.VMEM((T, T), F32), pltpu.VMEM((T, T), F32), pltpu.VMEM((T, T), F32),
                pltpu.VMEM((16, T), F32),
                pltpu.SemaphoreType.DMA((NRB,)),
                pltpu.SemaphoreType.DMA((14,)),
            ],
            compiler_params=pltpu.CompilerParams(vmem_limit_bytes=110 * 1024 * 1024, flags=flags),
        )(xT, A_k_cache.reshape(HKV, S, DH), A_v_cache.reshape(HKV, S, DH), A_wq, woT,
          B_w_r, B_w_gate, B_w_up, wdT, c, w_mod)
        return outT.T.reshape(1, S, D)
    return fn


_KW = {'lag':7,'oppos':28,'qppos':7}
_impl = make(**_KW)


@jax.jit
def pallas_adaLN_cond__gqa_block_cached__moe_arch_mod__prompt_kernel(
    A_x: jax.Array,
    A_k_cache: jax.Array,
    A_v_cache: jax.Array,
    A_wq: jax.Array,
    A_wo: jax.Array,
    B_x: jax.Array,
    B_w_r: jax.Array,
    B_w_gate: jax.Array,
    B_w_up: jax.Array,
    B_w_down: jax.Array,
    c: jax.Array,
    w_mod: jax.Array,
):
    return _impl(A_x, A_k_cache, A_v_cache, A_wq, A_wo, B_x, B_w_r, B_w_gate, B_w_up, B_w_down, c, w_mod)
```

```python
import contextlib
import jax
import jax.numpy as jnp
from jax import lax
import numpy as np
import jax.experimental.pallas as pl
import jax.experimental.pallas.tpu as pltpu

D = 576
S = 2048
HKV = 16
DH = 128
FF = 4608
C = 8
EPS = 1e-5
T = 128
NRB = S // T
NPER = 2 * NRB
F32 = jnp.float32
BF16 = jnp.bfloat16
NT = (((1,), (1,)), ((), ()))
QSCALE = float(DH ** -0.5 * np.log2(np.e))
LMIN = float(2.0 ** -90)
KT = [(0, 128), (128, 256), (256, 384), (384, 512), (512, 576)]
M1 = 2 * D


def _r(x):
    return x.astype(BF16).astype(F32)


def _col(row):
    return jnp.broadcast_to(row, (T, D)).T


def _sum8(x):
    return jnp.sum(x.reshape(x.shape[0] // 8, 8, x.shape[1]), axis=0)


def base_order(lag, oppos, qppos):
    toks = []
    for t in range(16 + lag):
        if t < 16: toks.append(('QK', t))
        if t - lag >= 0: toks.append(('PV', t - lag))
    assert oppos < len(toks) and qppos < len(toks)
    out = []
    for i, tk in enumerate(toks):
        if i == oppos: out += [('OP', j) for j in range(4)]
        if i == qppos: out += [('QP', j) for j in range(5)]
        out.append(tk)
    return out


def make(lag=8, oppos=30, qppos=8, flags=None, nb=18, **kw):
    seq_mid = kw.get('seq') or base_order(lag, oppos, qppos)
    seq_head = base_order(lag, kw.get('h_op', oppos), kw.get('h_qp', 0))
    seq_tail = [tk for tk in base_order(lag, oppos, kw.get('t_qp', qppos)) if tk[0] != 'OP'] + [('OP', j_) for j_ in range(4)]
    if not kw.get('ht', True):
        seq_head = seq_tail = seq_mid
    NKV, NW = 2, 3

    def mk(o):
        lg, op_, qp_ = o
        if op_ == 'end':
            return [tk for tk in base_order(lg, 0, qp_) if tk[0] != 'OP'] + [('OP', j_) for j_ in range(4)]
        return base_order(lg, op_, qp_)

    def edge_seq(kind, c):
        o = kw.get('f_ord' if kind == 'first' else 'l_ord')
        if o is not None:
            return mk(o[c])
        return seq_head if c == 0 else seq_tail if c == 3 else seq_mid

    def kernel(xT_hbm, k_hbm, v_hbm, wq_hbm, woT_hbm, wr_hbm, wg_hbm, wu_hbm, wdT_hbm, c_hbm, wmod_hbm, outT_hbm,
               x_c, k_v, v_v, wq_v, wo_v, wr_v, c_v, wm1_v, wm2_v, wg_v, wu_v, wd_v,
               modr, modc, h_v, acc, dlt, q0, q1, o0, o1, h2c, out_c, r_v, x1s,
               qs, ss, ms, ls, os_, chk_v, xsem, sems):
        q_scr = (q0, q1)
        o_scr = (o0, o1)
        (S_K, S_V, S_WQ, S_WO, S_WR, S_C, S_WM1, S_WM2, S_WG, S_WU, S_WD, S_WO0, S_WQ0, S_WQ1) = range(14)

        def scope(name):
            return jax.named_scope(name) if kw.get('scopes') else contextlib.nullcontext()

        class Two:
            def __init__(self, a, b): self.a, self.b = a, b
            def start(self): self.a.start(); self.b.start()
            def wait(self): self.a.wait(); self.b.wait()

        def cp_k(j): return pltpu.make_async_copy(k_hbm.at[j], k_v.at[j % NKV], sems.at[S_K])
        def cp_v(j): return pltpu.make_async_copy(v_hbm.at[j], v_v.at[j % NKV], sems.at[S_V])
        def cp_w1(src, dst, sem, j, hb):
            return pltpu.make_async_copy(src.at[:, pl.ds(pl.multiple_of(j * 256 + hb * T, T), T)],
                                         dst.at[2 * (j % NW) + hb], sems.at[sem])
        def cp_w(src, dst, sem, j): return Two(cp_w1(src, dst, sem, j, 0), cp_w1(src, dst, sem, j, 1))
        def cp_wq(j): return cp_w(wq_hbm, wq_v, S_WQ, j)
        def cp_wo(j): return cp_w(woT_hbm, wo_v, S_WO, j)
        cp_wo0 = cp_w(woT_hbm, wo_v, S_WO0, 0)
        def cp_x(rb):
            cols = slice(rb * T, (rb + 1) * T) if isinstance(rb, int) else pl.ds(pl.multiple_of(rb * T, T), T)
            return pltpu.make_async_copy(xT_hbm.at[:, cols], x_c.at[rb], xsem.at[rb])
        def cp_o(rb):
            cols = slice(rb * T, (rb + 1) * T) if isinstance(rb, int) else pl.ds(pl.multiple_of(rb * T, T), T)
            return pltpu.make_async_copy(out_c.at[rb], outT_hbm.at[:, cols], xsem.at[rb])
        cp_wr = pltpu.make_async_copy(wr_hbm, wr_v, sems.at[S_WR])
        cp_c = pltpu.make_async_copy(c_hbm, c_v, sems.at[S_C])
        cp_wm1 = pltpu.make_async_copy(wmod_hbm.at[:, 0:M1], wm1_v, sems.at[S_WM1])
        cp_wm2 = pltpu.make_async_copy(wmod_hbm.at[:, M1:6 * D], wm2_v, sems.at[S_WM2])
        cp_wg = pltpu.make_async_copy(wg_hbm, wg_v, sems.at[S_WG])
        cp_wu = pltpu.make_async_copy(wu_hbm, wu_v, sems.at[S_WU])
        cp_wd = pltpu.make_async_copy(wdT_hbm, wd_v, sems.at[S_WD])

        def wsl(ref, j, rows, hb):
            return ref[2 * (j % NW) + hb, rows, :]

        RBK = D // nb

        def ln1_thunks(rb, chain=True):
            st = {}
            th = []
            def ph_a(b):
                x = x_c[rb, b * RBK:(b + 1) * RBK, :].astype(F32)
                if b > 0 and chain:
                    x = (x.reshape(RBK // 8, 8, T) + (st['s'] * 0.0)[None]).reshape(RBK, T)
                t = _sum8(x)
                st['s'] = t if b == 0 else st['s'] + t
                if b == nb - 1:
                    st['m'] = jnp.broadcast_to(jnp.sum(st['s'], axis=0, keepdims=True) * (1.0 / D), (8, T))
            def ph_b(b):
                m = st['m']
                if b > 0 and chain: m = m + st['v'] * 0.0
                xc = x_c[rb, b * RBK:(b + 1) * RBK, :].astype(F32).reshape(RBK // 8, 8, T) - m[None]
                t = jnp.sum(xc * xc, axis=0)
                st['v'] = t if b == 0 else st['v'] + t
                if b == nb - 1:
                    st['rs'] = lax.rsqrt(jnp.sum(st['v'], axis=0, keepdims=True) * (1.0 / D) + EPS)
            def ph_c(k):
                k0, k1 = KT[k]
                m = st['m']
                if k > 0 and chain: m = m + st['z'] * 0.0
                n8 = (k1 - k0) // 8
                xc = (x_c[rb, k0:k1, :].astype(F32).reshape(n8, 8, T) - m[None]).reshape(k1 - k0, T)
                xh = xc * st['rs']
                st['z'] = xh[0:8, :]
                h = xh.T * modr[0:1, k0:k1] + modr[1:2, k0:k1]
                h_v[k, slice(rb * T, (rb + 1) * T) if isinstance(rb, int) else pl.ds(pl.multiple_of(rb * T, T), T), 0:k1 - k0] = h.astype(BF16)
            for b in range(nb): th.append(lambda b=b: ph_a(b))
            for b in range(nb): th.append(lambda b=b: ph_b(b))
            for k in range(5): th.append(lambda k=k: ph_c(k))
            return th

        def ln2_thunks(rb, chain=True):
            st = {}
            th = []
            def ph_a(b):
                rows = slice(b * RBK, (b + 1) * RBK)
                xin = x_c[rb, rows, :].astype(F32)
                a = acc[rb, rows, :] + dlt[rb, rows, :]
                if b > 0 and chain:
                    a = (a.reshape(RBK // 8, 8, T) + (st['s'] * 0.0)[None]).reshape(RBK, T)
                x1 = xin + modc[0, rows, :] * a
                x1s[rows, :] = x1
                t = _sum8(x1)
                st['s'] = t if b == 0 else st['s'] + t
                if b == nb - 1:
                    st['m'] = jnp.broadcast_to(jnp.sum(st['s'], axis=0, keepdims=True) * (1.0 / D), (8, T))
            def ph_b(b):
                m = st['m']
                if b > 0 and chain: m = m + st['v'] * 0.0
                xm = x1s[b * RBK:(b + 1) * RBK, :].reshape(RBK // 8, 8, T) - m[None]
                t = jnp.sum(xm * xm, axis=0)
                st['v'] = t if b == 0 else st['v'] + t
                if b == nb - 1:
                    v = _r(jnp.sum(st['v'], axis=0, keepdims=True) * (1.0 / D))
                    st['rd'] = 1.0 / _r(jnp.sqrt(_r(v + EPS)))
                    st['mr'] = _r(st['m'])
            def ph_c(b):
                rows = slice(b * RBK, (b + 1) * RBK)
                x1 = x1s[rows, :]
                mr = st['mr']
                if b > 0 and chain: mr = mr + st['r'] * 0.0
                xc = (x1.reshape(RBK // 8, 8, T) - mr[None]).reshape(RBK, T)
                h2 = xc * st['rd'] * modc[2, rows, :] + modc[1, rows, :]
                t = _sum8(h2 * modc[4, rows, :])
                st['r'] = t if b == 0 else st['r'] + t
                h2c[rb, rows, :] = h2.astype(BF16)
                out_c[rb, rows, :] = (x1 + modc[3, rows, :] * h2).astype(BF16)
                if b == nb - 1:
                    r_v[pl.ds(rb, 1), :] = _r(jnp.sum(st['r'], axis=0, keepdims=True))
            for b in range(nb): th.append(lambda b=b: ph_a(b))
            for b in range(nb): th.append(lambda b=b: ph_b(b))
            for b in range(nb): th.append(lambda b=b: ph_c(b))
            return th

        def mod2():
            cc = c_v[...].astype(F32)
            sc8 = jnp.broadcast_to(cc * jax.nn.sigmoid(cc), (8, D)).astype(BF16)
            mod = _r(jnp.dot(sc8, wm2_v[...], preferred_element_type=F32))
            for t in range(4):
                row = mod[0:1, t * D:(t + 1) * D]
                if t == 2: row = _r(1.0 + row)
                modc[t] = _col(row)
            modc[4] = _col(wr_v[...].reshape(1, D).astype(F32))

        def qp_tile(j, hb, rows, t):
            k0, k1 = KT[t]
            return jnp.dot(h_v[t, rows, 0:k1 - k0], wsl(wq_v, j, slice(k0, k1), hb), preferred_element_type=F32)

        def op_piece(j, hb, o_ref, rb, t, mode):
            rows = slice(t * 144, (t + 1) * 144)
            u = lax.dot_general(wsl(wo_v, j, rows, hb), o_ref[...], NT, preferred_element_type=F32)
            if mode == 'zero':
                acc[rb, rows, :] = jnp.zeros((144, T), F32)
            elif mode == 'commit':
                acc[rb, rows, :] += dlt[rb, rows, :]
            else:
                u = dlt[rb, rows, :] + u
            dlt[rb, rows, :] = u

        def period(j, par, chk, opspec, qpspec, th, seq):
            st = dict(l=None, o=None, q=None)
            ps = {}
            extra = {}
            n = len(seq)
            for i_, f_ in enumerate(th):
                extra.setdefault((i_ * n) // max(len(th), 1), []).append(f_)
            for i, (name, t) in enumerate(seq):
                for f_ in extra.get(i, []):
                    f_()
                if name == 'QK':
                    s = lax.dot_general(q_scr[par][...], k_v[j % NKV, t * T:(t + 1) * T, :], NT, preferred_element_type=F32)
                    p = jnp.exp2(s)
                    st['l'] = p if st['l'] is None else st['l'] + p
                    ps[t] = p.astype(BF16)
                elif name == 'PV':
                    o = jnp.dot(ps[t], v_v[j % NKV, t * T:(t + 1) * T, :], preferred_element_type=F32)
                    st['o'] = o if st['o'] is None else st['o'] + o
                    if t == 15:
                        l = jnp.sum(st['l'], axis=1, keepdims=True)
                        on = st['o'] * (1.0 / l)
                        o_scr[par][...] = on.astype(BF16)
                        lb = jnp.broadcast_to(l, (T, T))
                        chk['lmin'] = jnp.minimum(chk['lmin'], jnp.min(lb.reshape(T // 8, 8, T), axis=0))
                        chk['z'] = chk['z'] + _sum8(on + lb)
                elif name == 'OP':
                    op_piece(opspec[0], opspec[1], o_scr[1 - par], opspec[2], t, opspec[3])
                elif name == 'QP':
                    jq, hq, rbq = qpspec
                    rows = slice(rbq * T, (rbq + 1) * T) if isinstance(rbq, int) else pl.ds(pl.multiple_of(rbq * T, T), T)
                    d = qp_tile(jq, hq, rows, t)
                    st['q'] = d if st['q'] is None else st['q'] + d
                    if t == 4:
                        q_scr[1 - par][...] = (st['q'] * QSCALE).astype(BF16)

        def chk_new():
            return dict(lmin=jnp.full((8, T), 1.0, F32), z=jnp.zeros((8, T), F32))

        def chk_flush(chk, first):
            if first:
                chk_v[0:8, :] = chk['lmin']
                chk_v[8:16, :] = chk['z']
            else:
                chk_v[0:8, :] = jnp.minimum(chk_v[0:8, :], chk['lmin'])
                chk_v[8:16, :] = chk_v[8:16, :] + chk['z']

        def mid_step(j):
            chk = chk_new()
            for c in range(NPER if not kw.get('tiny_mid') else 2):
                opspec = (j, (c - 1) % 2, (c - 1) // 2, 'add' if (c - 1) % 2 else 'commit') if c >= 1 else (j - 1, 1, NRB - 1, 'add')
                qpspec = (j, (c + 1) % 2, (c + 1) // 2) if c + 1 < NPER else (j + 1, 0, 0)
                period(j, c % 2, chk, opspec, qpspec, [], seq_head if c == 0 else seq_tail if c == NPER - 1 else seq_mid)
            chk_flush(chk, True)

        def edge_step(j, kind):
            chk_flush(chk_new(), True)
            def body(it, carry):
                chk = chk_new()
                if kind == 'first':
                    edge_dma(it)
                    ra = jnp.minimum(2 * it + 2, NRB - 1)
                    rb_ = jnp.minimum(2 * it + 3, NRB - 1)
                    tha, thb = ln1_thunks(ra), ln1_thunks(rb_)
                else:
                    ra = jnp.maximum(2 * it - 2, 0)
                    rb_ = jnp.maximum(2 * it - 1, 0)
                    tha, thb = ln2_thunks(ra), ln2_thunks(rb_)
                ths = [tha[:len(tha) // 2], tha[len(tha) // 2:], thb[:len(thb) // 2], thb[len(thb) // 2:]]
                mode = 'zero' if kind == 'first' else 'commit'
                for c in range(4):
                    if c == 0:
                        if kind == 'first':
                            opspec = (j, 1, jnp.maximum(2 * it - 1, 0), 'add')
                        else:
                            opspec = (jnp.where(it == 0, j - 1, j), 1, (2 * it + NRB - 1) % NRB, 'add')
                    else:
                        opspec = (j, (c - 1) % 2, 2 * it + (c - 1) // 2, 'add' if (c - 1) % 2 else mode)
                    if c < 3:
                        qpspec = (j, (c + 1) % 2, 2 * it + (c + 1) // 2)
                    elif kind == 'first':
                        qpspec = (jnp.where(it == 7, j + 1, j), 0, (2 * it + 2) % NRB)
                    else:
                        qpspec = (j, 0, jnp.minimum(2 * it + 2, NRB - 1))
                    period(j, c % 2, chk, opspec, qpspec, ths[c], edge_seq(kind, c))
                chk_flush(chk, False)
                if kind == 'last':
                    @pl.when(it >= 1)
                    def _():
                        cp_o(2 * it - 2).start(); cp_o(2 * it - 1).start()
                return carry
            lax.fori_loop(0, NRB // 2, body, 0)

        def edge_dma(it):
            @pl.when(it < 6)
            def _():
                cp_x(2 * it + 4).start(); cp_x(2 * it + 5).start()
            @pl.when(it < 7)
            def _():
                cp_x(2 * it + 2).wait(); cp_x(2 * it + 3).wait()
            @pl.when(it == 1)
            def _():
                cp_wq(1).start(); cp_wr.start()
            @pl.when(it == 2)
            def _():
                cp_k(1).start(); cp_v(1).start()
            @pl.when(it == 3)
            def _():
                cp_wq(1).wait()
                cp_wo(1).start(); cp_wq(2).start()
            @pl.when(it == 4)
            def _():
                cp_wm2.start()

        def slow_step(j):
            def body(c, carry):
                rb = c // 2
                hb = c % 2
                rows = pl.ds(pl.multiple_of(rb * T, T), T)
                q = None
                for t_ in range(5):
                    d = qp_tile(j, hb, rows, t_)
                    q = d if q is None else q + d
                qs[...] = (q * QSCALE).astype(BF16)
                ms[...] = jnp.full((T, T), -jnp.inf, F32)
                def p1(t, carry_):
                    keys = pl.ds(pl.multiple_of(t * T, T), T)
                    s_ = lax.dot_general(qs[...], k_v[j % NKV, keys, :], NT, preferred_element_type=F32)
                    ss[t] = s_
                    ms[...] = jnp.maximum(ms[...], s_)
                    return carry_
                lax.fori_loop(0, S // T, p1, 0)
                ms[...] = jnp.broadcast_to(jnp.max(ms[...], axis=1, keepdims=True), (T, T))
                ls[...] = jnp.zeros((T, T), F32)
                os_[...] = jnp.zeros((T, T), F32)
                def p2(t, carry_):
                    keys = pl.ds(pl.multiple_of(t * T, T), T)
                    p = jnp.exp2(ss[t] - ms[...])
                    ls[...] += p
                    os_[...] += jnp.dot(p.astype(BF16), v_v[j % NKV, keys, :], preferred_element_type=F32)
                    return carry_
                lax.fori_loop(0, S // T, p2, 0)
                l = jnp.sum(ls[...], axis=1, keepdims=True)
                o1[...] = (os_[...] * (1.0 / l)).astype(BF16)
                @pl.when(c < NPER - 1)
                def _():
                    def po(t, carry_):
                        r_ = pl.ds(pl.multiple_of(t * 144, 16), 144)
                        u = lax.dot_general(wsl(wo_v, j, r_, hb), o1[...], NT, preferred_element_type=F32)
                        dlt[rb, r_, :] = jnp.where(hb == 0, 0.0, dlt[rb, r_, :]) + u
                        return carry_
                    lax.fori_loop(0, 4, po, 0)
                    @pl.when(jnp.logical_and(j == HKV - 1, hb == 1))
                    def _():
                        for f_ in ln2_thunks(rb, False):
                            f_()
                return carry
            with scope('SLOW'):
                lax.fori_loop(0, NPER, body, 0)

        cp_c.start(); cp_x(0).start(); cp_wm1.start()
        cp_w1(wq_hbm, wq_v, S_WQ0, 0, 0).start()
        def wave2():
            cp_k(0).start()
            cp_v(0).start()
            cp_x(1).start()
            cp_w1(wq_hbm, wq_v, S_WQ1, 0, 1).start()
            cp_wo0.start()
        if kw.get('stage', 1) == 0:
            wave2()
        o1[...] = jnp.zeros((T, DH), BF16)
        dlt[0] = jnp.zeros((D, T), F32)
        with scope('pro0'):
            cp_x(0).wait()
            th0 = ln1_thunks(0, False)
            for f_ in th0[:2 * nb]:
                f_()
            if kw.get('stage', 1) == 1:
                wave2()
            cp_c.wait(); cp_wm1.wait()
            if kw.get('stage', 1) == 2:
                wave2()
            cc = c_v[...].astype(F32)
            sc8 = jnp.broadcast_to(cc * jax.nn.sigmoid(cc), (8, D)).astype(BF16)
            mod = _r(jnp.dot(sc8, wm1_v[...], preferred_element_type=F32))
            modr[0:1, :] = 1.0 + mod[0:1, D:2 * D]
            modr[1:2, :] = mod[0:1, 0:D]
            for f_ in th0[2 * nb:]:
                f_()
            cp_w1(wq_hbm, wq_v, S_WQ0, 0, 0).wait()
            q = None
            for t in range(5):
                d = qp_tile(0, 0, slice(0, T), t)
                q = d if q is None else q + d
            q0[...] = (q * QSCALE).astype(BF16)
        cp_x(2).start(); cp_x(3).start()
        with scope('pro1'):
            cp_x(1).wait()
            for f_ in ln1_thunks(1, False):
                f_()
            cp_w1(wq_hbm, wq_v, S_WQ1, 0, 1).wait(); cp_k(0).wait(); cp_v(0).wait(); cp_wo0.wait()

        def step(j, carry):
            @pl.when(j == 0)
            def _():
                with scope('first'):
                    edge_step(0, 'first')
            @pl.when(jnp.logical_and(j > 0, j < HKV - 1))
            def _():
                with scope('wait'):
                    cp_k(j).wait(); cp_v(j).wait(); cp_wo(j).wait(); cp_wq(j + 1).wait()
                @pl.when(j + 2 < HKV)
                def _(): cp_wq(j + 2).start()
                @pl.when(j == 1)
                def _():
                    cp_wm2.wait(); cp_wr.wait()
                    mod2()
                    cp_wg.start()
                @pl.when(j == 2)
                def _(): cp_wu.start()
                @pl.when(j == 3)
                def _(): cp_wd.start()
                cp_k(j + 1).start(); cp_v(j + 1).start(); cp_wo(j + 1).start()
                with scope('midbody'):
                    mid_step(j)
            @pl.when(j == HKV - 1)
            def _():
                cp_k(HKV - 1).wait(); cp_v(HKV - 1).wait(); cp_wo(HKV - 1).wait()
                with scope('last'):
                    edge_step(HKV - 1, 'last')
            ok = jnp.where((chk_v[0:8, :] >= LMIN) & (jnp.abs(chk_v[8:16, :]) < jnp.inf), 1.0, 0.0)
            @pl.when(jnp.min(ok) < (2.0 if kw.get('forceslow') else 0.5))
            def _():
                @pl.when(j == HKV - 1)
                def _():
                    for rb in range(NRB - 2):
                        cp_o(rb).wait()
                slow_step(j)
                @pl.when(j == HKV - 1)
                def _():
                    for rb in range(NRB - 2):
                        cp_o(rb).start()
            return carry
        lax.fori_loop(0, HKV, step, 0)
        jl = HKV - 1

        with scope('tail0'):
            for t in range(4):
                op_piece(jl, 1, o1, NRB - 1, t, 'add')
            for f_ in ln2_thunks(NRB - 2, False):
                f_()
            cp_o(NRB - 2).start()
            for f_ in ln2_thunks(NRB - 1, False):
                f_()
            cp_o(NRB - 1).start()
        with scope('topk'):
            rb_ = pltpu.bitcast(r_v[...], jnp.int32) >> 16
            u = jnp.where(rb_ < 0, ~rb_, rb_ | 0x8000) & 0xFFFF
            tok = lax.broadcasted_iota(jnp.int32, (NRB, T), 0) * T + lax.broadcasted_iota(jnp.int32, (NRB, T), 1)
            key = pltpu.bitcast(((u << 11) | (S - 1 - tok)) + (1 << 27), F32)
            subs = lax.broadcasted_iota(jnp.int32, (8, T), 0)
            lane = lax.broadcasted_iota(jnp.int32, (8, T), 1)
            ksel = jnp.zeros((8, T), jnp.int32)
            for t in range(C):
                mx = jnp.max(jnp.max(key, axis=0, keepdims=True), axis=1, keepdims=True)
                key = jnp.where(key == mx, 0.0, key)
                ksel = jnp.where(subs == t, pltpu.bitcast(jnp.broadcast_to(mx, (8, T)), jnp.int32), ksel)
            ksel = ksel - (1 << 27)
            idxv = (S - 1) - (ksel & (S - 1))
            uu = ksel >> 11
            rbits = jnp.where((uu & 0x8000) != 0, uu & 0x7FFF, (~uu) & 0xFFFF) << 16
            rsel = pltpu.bitcast(rbits, F32)
            idxs = [jnp.max(jnp.where(subs == t, idxv, 0).astype(F32)).astype(jnp.int32) for t in range(C)]
        with scope('gather'):
            xs = None
            for t in range(C):
                oh = jnp.where((subs == t) & (lane == (idxv & (T - 1))), 1.0, 0.0).astype(BF16)
                n_t = jnp.clip(idxs[t] // T, 0, NRB - 1)
                d = lax.dot_general(oh, h2c[n_t], NT, preferred_element_type=F32)
                xs = d if xs is None else xs + d
        cp_wg.wait(); cp_wu.wait(); cp_wd.wait()
        with scope('ffn'):
            xb = xs.astype(BF16)
            g = _r(jnp.dot(xb, wg_v[...], preferred_element_type=F32))
            u_ = _r(jnp.dot(xb, wu_v[...], preferred_element_type=F32))
            g = _r(g * jax.nn.sigmoid(g))
            a = (g * u_).astype(BF16)
            y = _r(lax.dot_general(a, wd_v[...], NT, preferred_element_type=F32))
            y = _r(y * _r(jax.nn.sigmoid(rsel[:, 0:1])))
        with scope('fix'):
            yT = jnp.concatenate([y, jnp.zeros((T - 8, D), F32)], axis=0).T.astype(BF16)
            rowk = lax.broadcasted_iota(jnp.int32, (T, T), 0)
            lanes = lax.broadcasted_iota(jnp.int32, (T, T), 1)
            for rb in range(NRB):
                cp_o(rb).wait()
            tiles = [jnp.clip(idxs[t] // T, 0, NRB - 1) for t in range(C)]
            for t in range(C):
                sel = jnp.where((rowk == t) & (lanes == (idxs[t] & (T - 1))), 1.0, 0.0).astype(BF16)
                for p_ in range(4):
                    rows = slice(p_ * 144, (p_ + 1) * 144)
                    upd = jnp.dot(yT[rows, :], sel, preferred_element_type=F32)
                    out_c[tiles[t], rows, :] = (out_c[tiles[t], rows, :].astype(F32) + modc[3, rows, :] * upd).astype(BF16)
        with scope('wout'):
            fresh = []
            for t in range(C):
                f_ = jnp.bool_(True)
                for s_ in range(t):
                    f_ = jnp.logical_and(f_, tiles[s_] != tiles[t])
                fresh.append(f_)
                @pl.when(f_)
                def _(t=t):
                    cp_o(tiles[t]).start()
            for t in range(C):
                @pl.when(fresh[t])
                def _(t=t):
                    cp_o(tiles[t]).wait()

    @jax.jit
    def fn(A_x, A_k_cache, A_v_cache, A_wq, A_wo, B_x, B_w_r, B_w_gate, B_w_up, B_w_down, c, w_mod):
        del B_x
        xT = A_x.reshape(S, D).T
        woT = A_wo.T
        wdT = B_w_down.T
        any_spec = pl.BlockSpec(memory_space=pl.ANY)
        outT = pl.pallas_call(
            kernel,
            in_specs=[any_spec] * 11,
            out_specs=any_spec,
            out_shape=jax.ShapeDtypeStruct((D, S), BF16),
            scratch_shapes=[
                pltpu.VMEM((NRB, D, T), BF16),
                pltpu.VMEM((NKV, S, DH), BF16),
                pltpu.VMEM((NKV, S, DH), BF16),
                pltpu.VMEM((2 * NW, D, T), BF16),
                pltpu.VMEM((2 * NW, D, T), BF16),
                pltpu.VMEM((D,), BF16),
                pltpu.VMEM((1, D), BF16),
                pltpu.VMEM((D, M1), BF16),
                pltpu.VMEM((D, 4 * D), BF16),
                pltpu.VMEM((D, FF), BF16),
                pltpu.VMEM((D, FF), BF16),
                pltpu.VMEM((D, FF), BF16),
                pltpu.VMEM((8, D), F32),
                pltpu.VMEM((5, D, T), F32),
                pltpu.VMEM((5, S, T), BF16),
                pltpu.VMEM((NRB, D, T), F32),
                pltpu.VMEM((NRB, D, T), F32),
                pltpu.VMEM((T, DH), BF16), pltpu.VMEM((T, DH), BF16),
                pltpu.VMEM((T, DH), BF16), pltpu.VMEM((T, DH), BF16),
                pltpu.VMEM((NRB, D, T), BF16),
                pltpu.VMEM((NRB, D, T), BF16),
                pltpu.VMEM((NRB, T), F32),
                pltpu.VMEM((D, T), F32),
                pltpu.VMEM((T, DH), BF16),
                pltpu.VMEM((S // T, T, T), F32),
                pltpu.VMEM((T, T), F32), pltpu.VMEM((T, T), F32), pltpu.VMEM((T, T), F32),
                pltpu.VMEM((16, T), F32),
                pltpu.SemaphoreType.DMA((NRB,)),
                pltpu.SemaphoreType.DMA((14,)),
            ],
            compiler_params=pltpu.CompilerParams(vmem_limit_bytes=110 * 1024 * 1024, flags=flags),
        )(xT, A_k_cache.reshape(HKV, S, DH), A_v_cache.reshape(HKV, S, DH), A_wq, woT,
          B_w_r, B_w_gate, B_w_up, wdT, c, w_mod)
        return outT.T.reshape(1, S, D)
    return fn


_KW = {'lag':7,'oppos':28,'qppos':7,'h_op':14}
_impl = make(**_KW)


@jax.jit
def pallas_adaLN_cond__gqa_block_cached__moe_arch_mod__prompt_kernel(
    A_x: jax.Array,
    A_k_cache: jax.Array,
    A_v_cache: jax.Array,
    A_wq: jax.Array,
    A_wo: jax.Array,
    B_x: jax.Array,
    B_w_r: jax.Array,
    B_w_gate: jax.Array,
    B_w_up: jax.Array,
    B_w_down: jax.Array,
    c: jax.Array,
    w_mod: jax.Array,
):
    return _impl(A_x, A_k_cache, A_v_cache, A_wq, A_wo, B_x, B_w_r, B_w_gate, B_w_up, B_w_down, c, w_mod)
```

```python
import contextlib
import jax
import jax.numpy as jnp
from jax import lax
import numpy as np
import jax.experimental.pallas as pl
import jax.experimental.pallas.tpu as pltpu

D = 576
S = 2048
HKV = 16
DH = 128
FF = 4608
C = 8
EPS = 1e-5
T = 128
NRB = S // T
NPER = 2 * NRB
F32 = jnp.float32
BF16 = jnp.bfloat16
NT = (((1,), (1,)), ((), ()))
QSCALE = float(DH ** -0.5 * np.log2(np.e))
LMIN = float(2.0 ** -90)
KT = [(0, 128), (128, 256), (256, 384), (384, 512), (512, 576)]
M1 = 2 * D


def _r(x):
    return x.astype(BF16).astype(F32)


def _col(row):
    return jnp.broadcast_to(row, (T, D)).T


def _sum8(x):
    return jnp.sum(x.reshape(x.shape[0] // 8, 8, x.shape[1]), axis=0)


def base_order(lag, oppos, qppos):
    toks = []
    for t in range(16 + lag):
        if t < 16: toks.append(('QK', t))
        if t - lag >= 0: toks.append(('PV', t - lag))
    assert oppos < len(toks) and qppos < len(toks)
    out = []
    for i, tk in enumerate(toks):
        if i == oppos: out += [('OP', j) for j in range(4)]
        if i == qppos: out += [('QP', j) for j in range(5)]
        out.append(tk)
    return out


def make(lag=8, oppos=30, qppos=8, flags=None, nb=18, **kw):
    seq_mid = kw.get('seq') or base_order(lag, oppos, qppos)
    seq_head = base_order(lag, kw.get('h_op', oppos), kw.get('h_qp', 0))
    seq_tail = [tk for tk in base_order(lag, oppos, kw.get('t_qp', qppos)) if tk[0] != 'OP'] + [('OP', j_) for j_ in range(4)]
    if not kw.get('ht', True):
        seq_head = seq_tail = seq_mid
    NKV, NW = 2, 3

    def mk(o):
        lg, op_, qp_ = o
        if op_ == 'end':
            return [tk for tk in base_order(lg, 0, qp_) if tk[0] != 'OP'] + [('OP', j_) for j_ in range(4)]
        return base_order(lg, op_, qp_)

    def edge_seq(kind, c):
        o = kw.get('f_ord' if kind == 'first' else 'l_ord')
        if o is not None:
            return mk(o[c])
        return seq_head if c == 0 else seq_tail if c == 3 else seq_mid

    def kernel(xT_hbm, k_hbm, v_hbm, wq_hbm, woT_hbm, wr_hbm, wg_hbm, wu_hbm, wdT_hbm, c_hbm, wmod_hbm, outT_hbm,
               x_c, k_v, v_v, wq_v, wo_v, wr_v, c_v, wm1_v, wm2_v, wg_v, wu_v, wd_v,
               modr, modc, h_v, acc, dlt, q0, q1, o0, o1, h2c, out_c, r_v, x1s,
               qs, ss, ms, ls, os_, chk_v, xsem, sems):
        q_scr = (q0, q1)
        o_scr = (o0, o1)
        (S_K, S_V, S_WQ, S_WO, S_WR, S_C, S_WM1, S_WM2, S_WG, S_WU, S_WD, S_WO0, S_WQ0, S_WQ1) = range(14)

        def scope(name):
            return jax.named_scope(name) if kw.get('scopes') else contextlib.nullcontext()

        class Two:
            def __init__(self, a, b): self.a, self.b = a, b
            def start(self): self.a.start(); self.b.start()
            def wait(self): self.a.wait(); self.b.wait()

        def cp_k(j): return pltpu.make_async_copy(k_hbm.at[j], k_v.at[j % NKV], sems.at[S_K])
        def cp_v(j): return pltpu.make_async_copy(v_hbm.at[j], v_v.at[j % NKV], sems.at[S_V])
        def cp_w1(src, dst, sem, j, hb):
            return pltpu.make_async_copy(src.at[:, pl.ds(pl.multiple_of(j * 256 + hb * T, T), T)],
                                         dst.at[2 * (j % NW) + hb], sems.at[sem])
        def cp_w(src, dst, sem, j): return Two(cp_w1(src, dst, sem, j, 0), cp_w1(src, dst, sem, j, 1))
        def cp_wq(j): return cp_w(wq_hbm, wq_v, S_WQ, j)
        def cp_wo(j): return cp_w(woT_hbm, wo_v, S_WO, j)
        cp_wo0 = cp_w(woT_hbm, wo_v, S_WO0, 0)
        def cp_x(rb):
            cols = slice(rb * T, (rb + 1) * T) if isinstance(rb, int) else pl.ds(pl.multiple_of(rb * T, T), T)
            return pltpu.make_async_copy(xT_hbm.at[:, cols], x_c.at[rb], xsem.at[rb])
        def cp_o(rb):
            cols = slice(rb * T, (rb + 1) * T) if isinstance(rb, int) else pl.ds(pl.multiple_of(rb * T, T), T)
            return pltpu.make_async_copy(out_c.at[rb], outT_hbm.at[:, cols], xsem.at[rb])
        cp_wr = pltpu.make_async_copy(wr_hbm, wr_v, sems.at[S_WR])
        cp_c = pltpu.make_async_copy(c_hbm, c_v, sems.at[S_C])
        cp_wm1 = pltpu.make_async_copy(wmod_hbm.at[:, 0:M1], wm1_v, sems.at[S_WM1])
        cp_wm2 = pltpu.make_async_copy(wmod_hbm.at[:, M1:6 * D], wm2_v, sems.at[S_WM2])
        cp_wg = pltpu.make_async_copy(wg_hbm, wg_v, sems.at[S_WG])
        cp_wu = pltpu.make_async_copy(wu_hbm, wu_v, sems.at[S_WU])
        cp_wd = pltpu.make_async_copy(wdT_hbm, wd_v, sems.at[S_WD])

        def wsl(ref, j, rows, hb):
            return ref[2 * (j % NW) + hb, rows, :]

        RBK = D // nb

        def ln1_thunks(rb, chain=True):
            st = {}
            th = []
            def ph_a(b):
                x = x_c[rb, b * RBK:(b + 1) * RBK, :].astype(F32)
                if b > 0 and chain:
                    x = (x.reshape(RBK // 8, 8, T) + (st['s'] * 0.0)[None]).reshape(RBK, T)
                t = _sum8(x)
                st['s'] = t if b == 0 else st['s'] + t
                if b == nb - 1:
                    st['m'] = jnp.broadcast_to(jnp.sum(st['s'], axis=0, keepdims=True) * (1.0 / D), (8, T))
            def ph_b(b):
                m = st['m']
                if b > 0 and chain: m = m + st['v'] * 0.0
                xc = x_c[rb, b * RBK:(b + 1) * RBK, :].astype(F32).reshape(RBK // 8, 8, T) - m[None]
                t = jnp.sum(xc * xc, axis=0)
                st['v'] = t if b == 0 else st['v'] + t
                if b == nb - 1:
                    st['rs'] = lax.rsqrt(jnp.sum(st['v'], axis=0, keepdims=True) * (1.0 / D) + EPS)
            def ph_c(k):
                k0, k1 = KT[k]
                m = st['m']
                if k > 0 and chain: m = m + st['z'] * 0.0
                n8 = (k1 - k0) // 8
                xc = (x_c[rb, k0:k1, :].astype(F32).reshape(n8, 8, T) - m[None]).reshape(k1 - k0, T)
                xh = xc * st['rs']
                st['z'] = xh[0:8, :]
                h = xh.T * modr[0:1, k0:k1] + modr[1:2, k0:k1]
                h_v[k, slice(rb * T, (rb + 1) * T) if isinstance(rb, int) else pl.ds(pl.multiple_of(rb * T, T), T), 0:k1 - k0] = h.astype(BF16)
            for b in range(nb): th.append(lambda b=b: ph_a(b))
            for b in range(nb): th.append(lambda b=b: ph_b(b))
            for k in range(5): th.append(lambda k=k: ph_c(k))
            return th

        def ln2_thunks(rb, chain=True):
            st = {}
            th = []
            def ph_a(b):
                rows = slice(b * RBK, (b + 1) * RBK)
                xin = x_c[rb, rows, :].astype(F32)
                a = acc[rb, rows, :] + dlt[rb, rows, :]
                if b > 0 and chain:
                    a = (a.reshape(RBK // 8, 8, T) + (st['s'] * 0.0)[None]).reshape(RBK, T)
                x1 = xin + modc[0, rows, :] * a
                x1s[rows, :] = x1
                t = _sum8(x1)
                st['s'] = t if b == 0 else st['s'] + t
                if b == nb - 1:
                    st['m'] = jnp.broadcast_to(jnp.sum(st['s'], axis=0, keepdims=True) * (1.0 / D), (8, T))
            def ph_b(b):
                m = st['m']
                if b > 0 and chain: m = m + st['v'] * 0.0
                xm = x1s[b * RBK:(b + 1) * RBK, :].reshape(RBK // 8, 8, T) - m[None]
                t = jnp.sum(xm * xm, axis=0)
                st['v'] = t if b == 0 else st['v'] + t
                if b == nb - 1:
                    v = _r(jnp.sum(st['v'], axis=0, keepdims=True) * (1.0 / D))
                    st['rd'] = 1.0 / _r(jnp.sqrt(_r(v + EPS)))
                    st['mr'] = _r(st['m'])
            def ph_c(b):
                rows = slice(b * RBK, (b + 1) * RBK)
                x1 = x1s[rows, :]
                mr = st['mr']
                if b > 0 and chain: mr = mr + st['r'] * 0.0
                xc = (x1.reshape(RBK // 8, 8, T) - mr[None]).reshape(RBK, T)
                h2 = xc * st['rd'] * modc[2, rows, :] + modc[1, rows, :]
                t = _sum8(h2 * modc[4, rows, :])
                st['r'] = t if b == 0 else st['r'] + t
                h2c[rb, rows, :] = h2.astype(BF16)
                out_c[rb, rows, :] = (x1 + modc[3, rows, :] * h2).astype(BF16)
                if b == nb - 1:
                    r_v[pl.ds(rb, 1), :] = _r(jnp.sum(st['r'], axis=0, keepdims=True))
            for b in range(nb): th.append(lambda b=b: ph_a(b))
            for b in range(nb): th.append(lambda b=b: ph_b(b))
            for b in range(nb): th.append(lambda b=b: ph_c(b))
            return th

        def mod2():
            cc = c_v[...].astype(F32)
            sc8 = jnp.broadcast_to(cc * jax.nn.sigmoid(cc), (8, D)).astype(BF16)
            mod = _r(jnp.dot(sc8, wm2_v[...], preferred_element_type=F32))
            for t in range(4):
                row = mod[0:1, t * D:(t + 1) * D]
                if t == 2: row = _r(1.0 + row)
                modc[t] = _col(row)
            modc[4] = _col(wr_v[...].reshape(1, D).astype(F32))

        def qp_tile(j, hb, rows, t):
            k0, k1 = KT[t]
            return jnp.dot(h_v[t, rows, 0:k1 - k0], wsl(wq_v, j, slice(k0, k1), hb), preferred_element_type=F32)

        def op_piece(j, hb, o_ref, rb, t, mode):
            rows = slice(t * 144, (t + 1) * 144)
            u = lax.dot_general(wsl(wo_v, j, rows, hb), o_ref[...], NT, preferred_element_type=F32)
            if mode == 'zero':
                acc[rb, rows, :] = jnp.zeros((144, T), F32)
            elif mode == 'commit':
                acc[rb, rows, :] += dlt[rb, rows, :]
            else:
                u = dlt[rb, rows, :] + u
            dlt[rb, rows, :] = u

        def period(j, par, chk, opspec, qpspec, th, seq):
            st = dict(l=None, o=None, q=None)
            ps = {}
            extra = {}
            n = len(seq)
            for i_, f_ in enumerate(th):
                extra.setdefault((i_ * n) // max(len(th), 1), []).append(f_)
            for i, (name, t) in enumerate(seq):
                for f_ in extra.get(i, []):
                    f_()
                if name == 'QK':
                    s = lax.dot_general(q_scr[par][...], k_v[j % NKV, t * T:(t + 1) * T, :], NT, preferred_element_type=F32)
                    p = jnp.exp2(s)
                    st['l'] = p if st['l'] is None else st['l'] + p
                    ps[t] = p.astype(BF16)
                elif name == 'PV':
                    o = jnp.dot(ps[t], v_v[j % NKV, t * T:(t + 1) * T, :], preferred_element_type=F32)
                    st['o'] = o if st['o'] is None else st['o'] + o
                    if t == 15:
                        l = jnp.sum(st['l'], axis=1, keepdims=True)
                        on = st['o'] * (1.0 / l)
                        o_scr[par][...] = on.astype(BF16)
                        lb = jnp.broadcast_to(l, (T, T))
                        chk['lmin'] = jnp.minimum(chk['lmin'], jnp.min(lb.reshape(T // 8, 8, T), axis=0))
                        chk['z'] = chk['z'] + _sum8(on + lb)
                elif name == 'OP':
                    op_piece(opspec[0], opspec[1], o_scr[1 - par], opspec[2], t, opspec[3])
                elif name == 'QP':
                    jq, hq, rbq = qpspec
                    rows = slice(rbq * T, (rbq + 1) * T) if isinstance(rbq, int) else pl.ds(pl.multiple_of(rbq * T, T), T)
                    d = qp_tile(jq, hq, rows, t)
                    st['q'] = d if st['q'] is None else st['q'] + d
                    if t == 4:
                        q_scr[1 - par][...] = (st['q'] * QSCALE).astype(BF16)

        def chk_new():
            return dict(lmin=jnp.full((8, T), 1.0, F32), z=jnp.zeros((8, T), F32))

        def chk_flush(chk, first):
            if first:
                chk_v[0:8, :] = chk['lmin']
                chk_v[8:16, :] = chk['z']
            else:
                chk_v[0:8, :] = jnp.minimum(chk_v[0:8, :], chk['lmin'])
                chk_v[8:16, :] = chk_v[8:16, :] + chk['z']

        def mid_step(j):
            chk = chk_new()
            for c in range(NPER if not kw.get('tiny_mid') else 2):
                opspec = (j, (c - 1) % 2, (c - 1) // 2, 'add' if (c - 1) % 2 else 'commit') if c >= 1 else (j - 1, 1, NRB - 1, 'add')
                qpspec = (j, (c + 1) % 2, (c + 1) // 2) if c + 1 < NPER else (j + 1, 0, 0)
                period(j, c % 2, chk, opspec, qpspec, [], seq_head if c == 0 else seq_tail if c == NPER - 1 else seq_mid)
            chk_flush(chk, True)

        def edge_step(j, kind):
            chk_flush(chk_new(), True)
            def body(it, carry):
                chk = chk_new()
                if kind == 'first':
                    edge_dma(it)
                    ra = jnp.minimum(2 * it + 2, NRB - 1)
                    rb_ = jnp.minimum(2 * it + 3, NRB - 1)
                    tha, thb = ln1_thunks(ra), ln1_thunks(rb_)
                else:
                    ra = jnp.maximum(2 * it - 2, 0)
                    rb_ = jnp.maximum(2 * it - 1, 0)
                    tha, thb = ln2_thunks(ra), ln2_thunks(rb_)
                ths = [tha[:len(tha) // 2], tha[len(tha) // 2:], thb[:len(thb) // 2], thb[len(thb) // 2:]]
                mode = 'zero' if kind == 'first' else 'commit'
                for c in range(4):
                    if c == 0:
                        if kind == 'first':
                            opspec = (j, 1, jnp.maximum(2 * it - 1, 0), 'add')
                        else:
                            opspec = (jnp.where(it == 0, j - 1, j), 1, (2 * it + NRB - 1) % NRB, 'add')
                    else:
                        opspec = (j, (c - 1) % 2, 2 * it + (c - 1) // 2, 'add' if (c - 1) % 2 else mode)
                    if c < 3:
                        qpspec = (j, (c + 1) % 2, 2 * it + (c + 1) // 2)
                    elif kind == 'first':
                        qpspec = (jnp.where(it == 7, j + 1, j), 0, (2 * it + 2) % NRB)
                    else:
                        qpspec = (j, 0, jnp.minimum(2 * it + 2, NRB - 1))
                    period(j, c % 2, chk, opspec, qpspec, ths[c], edge_seq(kind, c))
                chk_flush(chk, False)
                if kind == 'last':
                    @pl.when(it >= 1)
                    def _():
                        cp_o(2 * it - 2).start(); cp_o(2 * it - 1).start()
                return carry
            lax.fori_loop(0, NRB // 2, body, 0)

        def edge_dma(it):
            @pl.when(it < 6)
            def _():
                cp_x(2 * it + 4).start(); cp_x(2 * it + 5).start()
            @pl.when(it < 7)
            def _():
                cp_x(2 * it + 2).wait(); cp_x(2 * it + 3).wait()
            @pl.when(it == 1)
            def _():
                cp_wq(1).start(); cp_wr.start()
            @pl.when(it == 2)
            def _():
                cp_k(1).start(); cp_v(1).start()
            @pl.when(it == 3)
            def _():
                cp_wq(1).wait()
                cp_wo(1).start(); cp_wq(2).start()
            @pl.when(it == 4)
            def _():
                cp_wm2.start()

        def slow_step(j):
            def body(c, carry):
                rb = c // 2
                hb = c % 2
                rows = pl.ds(pl.multiple_of(rb * T, T), T)
                q = None
                for t_ in range(5):
                    d = qp_tile(j, hb, rows, t_)
                    q = d if q is None else q + d
                qs[...] = (q * QSCALE).astype(BF16)
                ms[...] = jnp.full((T, T), -jnp.inf, F32)
                def p1(t, carry_):
                    keys = pl.ds(pl.multiple_of(t * T, T), T)
                    s_ = lax.dot_general(qs[...], k_v[j % NKV, keys, :], NT, preferred_element_type=F32)
                    ss[t] = s_
                    ms[...] = jnp.maximum(ms[...], s_)
                    return carry_
                lax.fori_loop(0, S // T, p1, 0)
                ms[...] = jnp.broadcast_to(jnp.max(ms[...], axis=1, keepdims=True), (T, T))
                ls[...] = jnp.zeros((T, T), F32)
                os_[...] = jnp.zeros((T, T), F32)
                def p2(t, carry_):
                    keys = pl.ds(pl.multiple_of(t * T, T), T)
                    p = jnp.exp2(ss[t] - ms[...])
                    ls[...] += p
                    os_[...] += jnp.dot(p.astype(BF16), v_v[j % NKV, keys, :], preferred_element_type=F32)
                    return carry_
                lax.fori_loop(0, S // T, p2, 0)
                l = jnp.sum(ls[...], axis=1, keepdims=True)
                o1[...] = (os_[...] * (1.0 / l)).astype(BF16)
                @pl.when(c < NPER - 1)
                def _():
                    def po(t, carry_):
                        r_ = pl.ds(pl.multiple_of(t * 144, 16), 144)
                        u = lax.dot_general(wsl(wo_v, j, r_, hb), o1[...], NT, preferred_element_type=F32)
                        dlt[rb, r_, :] = jnp.where(hb == 0, 0.0, dlt[rb, r_, :]) + u
                        return carry_
                    lax.fori_loop(0, 4, po, 0)
                    @pl.when(jnp.logical_and(j == HKV - 1, hb == 1))
                    def _():
                        for f_ in ln2_thunks(rb, False):
                            f_()
                return carry
            with scope('SLOW'):
                lax.fori_loop(0, NPER, body, 0)

        W1 = kw.get('w1', 'c x0 wm1 wq0')
        W2 = kw.get('w2', 'k0 v0 x1 wq1 wo0')
        W3 = kw.get('w3', '')
        dm = dict(c=cp_c, x0=cp_x(0), wm1=cp_wm1, wq0=cp_w1(wq_hbm, wq_v, S_WQ0, 0, 0), k0=cp_k(0), v0=cp_v(0), x1=cp_x(1),
                  wq1=cp_w1(wq_hbm, wq_v, S_WQ1, 0, 1), wo0=cp_wo0)
        def wave(names):
            for n_ in names.split():
                dm[n_].start()
        wave(W1)
        o1[...] = jnp.zeros((T, DH), BF16)
        dlt[0] = jnp.zeros((D, T), F32)
        with scope('pro0'):
            cp_x(0).wait()
            th0 = ln1_thunks(0, False)
            for f_ in th0[:2 * nb]:
                f_()
            wave(W2)
            cp_c.wait(); cp_wm1.wait()
            wave(W3)
            cc = c_v[...].astype(F32)
            sc8 = jnp.broadcast_to(cc * jax.nn.sigmoid(cc), (8, D)).astype(BF16)
            mod = _r(jnp.dot(sc8, wm1_v[...], preferred_element_type=F32))
            modr[0:1, :] = 1.0 + mod[0:1, D:2 * D]
            modr[1:2, :] = mod[0:1, 0:D]
            for f_ in th0[2 * nb:]:
                f_()
            cp_w1(wq_hbm, wq_v, S_WQ0, 0, 0).wait()
            q = None
            for t in range(5):
                d = qp_tile(0, 0, slice(0, T), t)
                q = d if q is None else q + d
            q0[...] = (q * QSCALE).astype(BF16)
        cp_x(2).start(); cp_x(3).start()
        with scope('pro1'):
            cp_x(1).wait()
            for f_ in ln1_thunks(1, False):
                f_()
            cp_w1(wq_hbm, wq_v, S_WQ1, 0, 1).wait(); cp_k(0).wait(); cp_v(0).wait(); cp_wo0.wait()

        def step(j, carry):
            @pl.when(j == 0)
            def _():
                with scope('first'):
                    edge_step(0, 'first')
            @pl.when(jnp.logical_and(j > 0, j < HKV - 1))
            def _():
                with scope('wait'):
                    cp_k(j).wait(); cp_v(j).wait(); cp_wo(j).wait(); cp_wq(j + 1).wait()
                @pl.when(j + 2 < HKV)
                def _(): cp_wq(j + 2).start()
                @pl.when(j == 1)
                def _():
                    cp_wm2.wait(); cp_wr.wait()
                    mod2()
                    cp_wg.start()
                @pl.when(j == 2)
                def _(): cp_wu.start()
                @pl.when(j == 3)
                def _(): cp_wd.start()
                cp_k(j + 1).start(); cp_v(j + 1).start(); cp_wo(j + 1).start()
                with scope('midbody'):
                    mid_step(j)
            @pl.when(j == HKV - 1)
            def _():
                cp_k(HKV - 1).wait(); cp_v(HKV - 1).wait(); cp_wo(HKV - 1).wait()
                with scope('last'):
                    edge_step(HKV - 1, 'last')
            ok = jnp.where((chk_v[0:8, :] >= LMIN) & (jnp.abs(chk_v[8:16, :]) < jnp.inf), 1.0, 0.0)
            @pl.when(jnp.min(ok) < (2.0 if kw.get('forceslow') else 0.5))
            def _():
                @pl.when(j == HKV - 1)
                def _():
                    for rb in range(NRB - 2):
                        cp_o(rb).wait()
                slow_step(j)
                @pl.when(j == HKV - 1)
                def _():
                    for rb in range(NRB - 2):
                        cp_o(rb).start()
            return carry
        lax.fori_loop(0, HKV, step, 0)
        jl = HKV - 1

        with scope('tail0'):
            for t in range(4):
                op_piece(jl, 1, o1, NRB - 1, t, 'add')
            for f_ in ln2_thunks(NRB - 2, False):
                f_()
            cp_o(NRB - 2).start()
            for f_ in ln2_thunks(NRB - 1, False):
                f_()
            cp_o(NRB - 1).start()
        with scope('topk'):
            rb_ = pltpu.bitcast(r_v[...], jnp.int32) >> 16
            u = jnp.where(rb_ < 0, ~rb_, rb_ | 0x8000) & 0xFFFF
            tok = lax.broadcasted_iota(jnp.int32, (NRB, T), 0) * T + lax.broadcasted_iota(jnp.int32, (NRB, T), 1)
            key = pltpu.bitcast(((u << 11) | (S - 1 - tok)) + (1 << 27), F32)
            subs = lax.broadcasted_iota(jnp.int32, (8, T), 0)
            lane = lax.broadcasted_iota(jnp.int32, (8, T), 1)
            ksel = jnp.zeros((8, T), jnp.int32)
            for t in range(C):
                mx = jnp.max(jnp.max(key, axis=0, keepdims=True), axis=1, keepdims=True)
                key = jnp.where(key == mx, 0.0, key)
                ksel = jnp.where(subs == t, pltpu.bitcast(jnp.broadcast_to(mx, (8, T)), jnp.int32), ksel)
            ksel = ksel - (1 << 27)
            idxv = (S - 1) - (ksel & (S - 1))
            uu = ksel >> 11
            rbits = jnp.where((uu & 0x8000) != 0, uu & 0x7FFF, (~uu) & 0xFFFF) << 16
            rsel = pltpu.bitcast(rbits, F32)
            idxs = [jnp.max(jnp.where(subs == t, idxv, 0).astype(F32)).astype(jnp.int32) for t in range(C)]
        with scope('gather'):
            xs = None
            for t in range(C):
                oh = jnp.where((subs == t) & (lane == (idxv & (T - 1))), 1.0, 0.0).astype(BF16)
                n_t = jnp.clip(idxs[t] // T, 0, NRB - 1)
                d = lax.dot_general(oh, h2c[n_t], NT, preferred_element_type=F32)
                xs = d if xs is None else xs + d
        cp_wg.wait(); cp_wu.wait(); cp_wd.wait()
        with scope('ffn'):
            xb = xs.astype(BF16)
            g = _r(jnp.dot(xb, wg_v[...], preferred_element_type=F32))
            u_ = _r(jnp.dot(xb, wu_v[...], preferred_element_type=F32))
            g = _r(g * jax.nn.sigmoid(g))
            a = (g * u_).astype(BF16)
            y = _r(lax.dot_general(a, wd_v[...], NT, preferred_element_type=F32))
            y = _r(y * _r(jax.nn.sigmoid(rsel[:, 0:1])))
        with scope('fix'):
            yT = jnp.concatenate([y, jnp.zeros((T - 8, D), F32)], axis=0).T.astype(BF16)
            rowk = lax.broadcasted_iota(jnp.int32, (T, T), 0)
            lanes = lax.broadcasted_iota(jnp.int32, (T, T), 1)
            for rb in range(NRB):
                cp_o(rb).wait()
            tiles = [jnp.clip(idxs[t] // T, 0, NRB - 1) for t in range(C)]
            for t in range(C):
                sel = jnp.where((rowk == t) & (lanes == (idxs[t] & (T - 1))), 1.0, 0.0).astype(BF16)
                for p_ in range(4):
                    rows = slice(p_ * 144, (p_ + 1) * 144)
                    upd = jnp.dot(yT[rows, :], sel, preferred_element_type=F32)
                    out_c[tiles[t], rows, :] = (out_c[tiles[t], rows, :].astype(F32) + modc[3, rows, :] * upd).astype(BF16)
        with scope('wout'):
            fresh = []
            for t in range(C):
                f_ = jnp.bool_(True)
                for s_ in range(t):
                    f_ = jnp.logical_and(f_, tiles[s_] != tiles[t])
                fresh.append(f_)
                @pl.when(f_)
                def _(t=t):
                    cp_o(tiles[t]).start()
            for t in range(C):
                @pl.when(fresh[t])
                def _(t=t):
                    cp_o(tiles[t]).wait()

    @jax.jit
    def fn(A_x, A_k_cache, A_v_cache, A_wq, A_wo, B_x, B_w_r, B_w_gate, B_w_up, B_w_down, c, w_mod):
        del B_x
        xT = A_x.reshape(S, D).T
        woT = A_wo.T
        wdT = B_w_down.T
        any_spec = pl.BlockSpec(memory_space=pl.ANY)
        outT = pl.pallas_call(
            kernel,
            in_specs=[any_spec] * 11,
            out_specs=any_spec,
            out_shape=jax.ShapeDtypeStruct((D, S), BF16),
            scratch_shapes=[
                pltpu.VMEM((NRB, D, T), BF16),
                pltpu.VMEM((NKV, S, DH), BF16),
                pltpu.VMEM((NKV, S, DH), BF16),
                pltpu.VMEM((2 * NW, D, T), BF16),
                pltpu.VMEM((2 * NW, D, T), BF16),
                pltpu.VMEM((D,), BF16),
                pltpu.VMEM((1, D), BF16),
                pltpu.VMEM((D, M1), BF16),
                pltpu.VMEM((D, 4 * D), BF16),
                pltpu.VMEM((D, FF), BF16),
                pltpu.VMEM((D, FF), BF16),
                pltpu.VMEM((D, FF), BF16),
                pltpu.VMEM((8, D), F32),
                pltpu.VMEM((5, D, T), F32),
                pltpu.VMEM((5, S, T), BF16),
                pltpu.VMEM((NRB, D, T), F32),
                pltpu.VMEM((NRB, D, T), F32),
                pltpu.VMEM((T, DH), BF16), pltpu.VMEM((T, DH), BF16),
                pltpu.VMEM((T, DH), BF16), pltpu.VMEM((T, DH), BF16),
                pltpu.VMEM((NRB, D, T), BF16),
                pltpu.VMEM((NRB, D, T), BF16),
                pltpu.VMEM((NRB, T), F32),
                pltpu.VMEM((D, T), F32),
                pltpu.VMEM((T, DH), BF16),
                pltpu.VMEM((S // T, T, T), F32),
                pltpu.VMEM((T, T), F32), pltpu.VMEM((T, T), F32), pltpu.VMEM((T, T), F32),
                pltpu.VMEM((16, T), F32),
                pltpu.SemaphoreType.DMA((NRB,)),
                pltpu.SemaphoreType.DMA((14,)),
            ],
            compiler_params=pltpu.CompilerParams(vmem_limit_bytes=110 * 1024 * 1024, flags=flags),
        )(xT, A_k_cache.reshape(HKV, S, DH), A_v_cache.reshape(HKV, S, DH), A_wq, woT,
          B_w_r, B_w_gate, B_w_up, wdT, c, w_mod)
        return outT.T.reshape(1, S, D)
    return fn


_KW = {'lag':7,'oppos':28,'qppos':7,'h_op':14,'f_ord':[[8,14,7],[7,28,7],[8,23,14],[7,'end',7]],'l_ord':[[7,14,0],[8,23,7],[8,14,14],[9,24,14]],'w1':'wm1 c x0 wq0 k0','w2':'v0','w3':'x1 wq1 wo0'}
_impl = make(**_KW)


@jax.jit
def pallas_adaLN_cond__gqa_block_cached__moe_arch_mod__prompt_kernel(
    A_x: jax.Array,
    A_k_cache: jax.Array,
    A_v_cache: jax.Array,
    A_wq: jax.Array,
    A_wo: jax.Array,
    B_x: jax.Array,
    B_w_r: jax.Array,
    B_w_gate: jax.Array,
    B_w_up: jax.Array,
    B_w_down: jax.Array,
    c: jax.Array,
    w_mod: jax.Array,
):
    return _impl(A_x, A_k_cache, A_v_cache, A_wq, A_wo, B_x, B_w_r, B_w_gate, B_w_up, B_w_down, c, w_mod)
```

```python
import contextlib
import jax
import jax.numpy as jnp
from jax import lax
import numpy as np
import jax.experimental.pallas as pl
import jax.experimental.pallas.tpu as pltpu

D = 576
S = 2048
HKV = 16
DH = 128
FF = 4608
C = 8
EPS = 1e-5
T = 128
NRB = S // T
NPER = 2 * NRB
F32 = jnp.float32
BF16 = jnp.bfloat16
NT = (((1,), (1,)), ((), ()))
QSCALE = float(DH ** -0.5 * np.log2(np.e))
LMIN = float(2.0 ** -90)
KT = [(0, 128), (128, 256), (256, 384), (384, 512), (512, 576)]
M1 = 2 * D


def _r(x):
    return x.astype(BF16).astype(F32)


def _col(row):
    return jnp.broadcast_to(row, (T, D)).T


def _sum8(x):
    return jnp.sum(x.reshape(x.shape[0] // 8, 8, x.shape[1]), axis=0)


def base_order(lag, oppos, qppos):
    toks = []
    for t in range(16 + lag):
        if t < 16: toks.append(('QK', t))
        if t - lag >= 0: toks.append(('PV', t - lag))
    assert oppos < len(toks) and qppos < len(toks)
    out = []
    for i, tk in enumerate(toks):
        if i == oppos: out += [('OP', j) for j in range(4)]
        if i == qppos: out += [('QP', j) for j in range(5)]
        out.append(tk)
    return out


def make(lag=8, oppos=30, qppos=8, flags=None, nb=18, **kw):
    seq_mid = kw.get('seq') or base_order(lag, oppos, qppos)
    seq_head = base_order(lag, kw.get('h_op', oppos), kw.get('h_qp', 0))
    seq_tail = [tk for tk in base_order(lag, oppos, kw.get('t_qp', qppos)) if tk[0] != 'OP'] + [('OP', j_) for j_ in range(4)]
    if not kw.get('ht', True):
        seq_head = seq_tail = seq_mid
    NKV, NW = 2, 3

    def mk(o):
        lg, op_, qp_ = o
        if op_ == 'end':
            return [tk for tk in base_order(lg, 0, qp_) if tk[0] != 'OP'] + [('OP', j_) for j_ in range(4)]
        return base_order(lg, op_, qp_)

    def edge_seq(kind, c):
        o = kw.get('f_ord' if kind == 'first' else 'l_ord')
        if o is not None:
            return mk(o[c])
        return seq_head if c == 0 else seq_tail if c == 3 else seq_mid

    def kernel(xT_hbm, k_hbm, v_hbm, wq_hbm, woT_hbm, wr_hbm, wg_hbm, wu_hbm, wdT_hbm, c_hbm, wmod_hbm, outT_hbm,
               x_c, k_v, v_v, wq_v, wo_v, wr_v, c_v, wm1_v, wm2_v, wg_v, wu_v, wd_v,
               modr, modc, h_v, acc, dlt, q0, q1, o0, o1, h2c, out_c, r_v, x1s,
               qs, ss, ms, ls, os_, chk_v, xsem, sems):
        q_scr = (q0, q1)
        o_scr = (o0, o1)
        (S_K, S_V, S_WQ, S_WO, S_WR, S_C, S_WM1, S_WM2, S_WG, S_WU, S_WD, S_WO0, S_WQ0, S_WQ1) = range(14)

        def scope(name):
            return jax.named_scope(name) if kw.get('scopes') else contextlib.nullcontext()

        class Two:
            def __init__(self, a, b): self.a, self.b = a, b
            def start(self): self.a.start(); self.b.start()
            def wait(self): self.a.wait(); self.b.wait()

        def cp_k(j): return pltpu.make_async_copy(k_hbm.at[j], k_v.at[j % NKV], sems.at[S_K])
        def cp_v(j): return pltpu.make_async_copy(v_hbm.at[j], v_v.at[j % NKV], sems.at[S_V])
        def cp_w1(src, dst, sem, j, hb):
            return pltpu.make_async_copy(src.at[:, pl.ds(pl.multiple_of(j * 256 + hb * T, T), T)],
                                         dst.at[2 * (j % NW) + hb], sems.at[sem])
        def cp_w(src, dst, sem, j): return Two(cp_w1(src, dst, sem, j, 0), cp_w1(src, dst, sem, j, 1))
        def cp_wq(j): return cp_w(wq_hbm, wq_v, S_WQ, j)
        def cp_wo(j): return cp_w(woT_hbm, wo_v, S_WO, j)
        cp_wo0 = cp_w(woT_hbm, wo_v, S_WO0, 0)
        def cp_x(rb):
            cols = slice(rb * T, (rb + 1) * T) if isinstance(rb, int) else pl.ds(pl.multiple_of(rb * T, T), T)
            return pltpu.make_async_copy(xT_hbm.at[:, cols], x_c.at[rb], xsem.at[rb])
        def cp_o(rb):
            cols = slice(rb * T, (rb + 1) * T) if isinstance(rb, int) else pl.ds(pl.multiple_of(rb * T, T), T)
            return pltpu.make_async_copy(out_c.at[rb], outT_hbm.at[:, cols], xsem.at[rb])
        cp_wr = pltpu.make_async_copy(wr_hbm, wr_v, sems.at[S_WR])
        cp_c = pltpu.make_async_copy(c_hbm, c_v, sems.at[S_C])
        cp_wm1 = pltpu.make_async_copy(wmod_hbm.at[:, 0:M1], wm1_v, sems.at[S_WM1])
        cp_wm2 = pltpu.make_async_copy(wmod_hbm.at[:, M1:6 * D], wm2_v, sems.at[S_WM2])
        cp_wg = pltpu.make_async_copy(wg_hbm, wg_v, sems.at[S_WG])
        cp_wu = pltpu.make_async_copy(wu_hbm, wu_v, sems.at[S_WU])
        cp_wd = pltpu.make_async_copy(wdT_hbm, wd_v, sems.at[S_WD])

        def wsl(ref, j, rows, hb):
            return ref[2 * (j % NW) + hb, rows, :]

        RBK = D // nb

        def ln1_thunks(rb, chain=True):
            st = {}
            th = []
            def ph_a(b):
                x = x_c[rb, b * RBK:(b + 1) * RBK, :].astype(F32)
                if b > 0 and chain:
                    x = (x.reshape(RBK // 8, 8, T) + (st['s'] * 0.0)[None]).reshape(RBK, T)
                t = _sum8(x)
                st['s'] = t if b == 0 else st['s'] + t
                if b == nb - 1:
                    st['m'] = jnp.broadcast_to(jnp.sum(st['s'], axis=0, keepdims=True) * (1.0 / D), (8, T))
            def ph_b(b):
                m = st['m']
                if b > 0 and chain: m = m + st['v'] * 0.0
                xc = x_c[rb, b * RBK:(b + 1) * RBK, :].astype(F32).reshape(RBK // 8, 8, T) - m[None]
                t = jnp.sum(xc * xc, axis=0)
                st['v'] = t if b == 0 else st['v'] + t
                if b == nb - 1:
                    st['rs'] = lax.rsqrt(jnp.sum(st['v'], axis=0, keepdims=True) * (1.0 / D) + EPS)
            def ph_c(k):
                k0, k1 = KT[k]
                m = st['m']
                if k > 0 and chain: m = m + st['z'] * 0.0
                n8 = (k1 - k0) // 8
                xc = (x_c[rb, k0:k1, :].astype(F32).reshape(n8, 8, T) - m[None]).reshape(k1 - k0, T)
                xh = xc * st['rs']
                st['z'] = xh[0:8, :]
                h = xh.T * modr[0:1, k0:k1] + modr[1:2, k0:k1]
                h_v[k, slice(rb * T, (rb + 1) * T) if isinstance(rb, int) else pl.ds(pl.multiple_of(rb * T, T), T), 0:k1 - k0] = h.astype(BF16)
            for b in range(nb): th.append(lambda b=b: ph_a(b))
            for b in range(nb): th.append(lambda b=b: ph_b(b))
            for k in range(5): th.append(lambda k=k: ph_c(k))
            return th

        def ln2_thunks(rb, chain=True):
            st = {}
            th = []
            def ph_a(b):
                rows = slice(b * RBK, (b + 1) * RBK)
                xin = x_c[rb, rows, :].astype(F32)
                a = acc[rb, rows, :] + dlt[rb, rows, :]
                if b > 0 and chain:
                    a = (a.reshape(RBK // 8, 8, T) + (st['s'] * 0.0)[None]).reshape(RBK, T)
                x1 = xin + modc[0, rows, :] * a
                x1s[rows, :] = x1
                t = _sum8(x1)
                st['s'] = t if b == 0 else st['s'] + t
                if b == nb - 1:
                    st['m'] = jnp.broadcast_to(jnp.sum(st['s'], axis=0, keepdims=True) * (1.0 / D), (8, T))
            def ph_b(b):
                m = st['m']
                if b > 0 and chain: m = m + st['v'] * 0.0
                xm = x1s[b * RBK:(b + 1) * RBK, :].reshape(RBK // 8, 8, T) - m[None]
                t = jnp.sum(xm * xm, axis=0)
                st['v'] = t if b == 0 else st['v'] + t
                if b == nb - 1:
                    v = _r(jnp.sum(st['v'], axis=0, keepdims=True) * (1.0 / D))
                    st['rd'] = 1.0 / _r(jnp.sqrt(_r(v + EPS)))
                    st['mr'] = _r(st['m'])
            def ph_c(b):
                rows = slice(b * RBK, (b + 1) * RBK)
                x1 = x1s[rows, :]
                mr = st['mr']
                if b > 0 and chain: mr = mr + st['r'] * 0.0
                xc = (x1.reshape(RBK // 8, 8, T) - mr[None]).reshape(RBK, T)
                h2 = xc * st['rd'] * modc[2, rows, :] + modc[1, rows, :]
                t = _sum8(h2 * modc[4, rows, :])
                st['r'] = t if b == 0 else st['r'] + t
                h2c[rb, rows, :] = h2.astype(BF16)
                out_c[rb, rows, :] = (x1 + modc[3, rows, :] * h2).astype(BF16)
                if b == nb - 1:
                    r_v[pl.ds(rb, 1), :] = _r(jnp.sum(st['r'], axis=0, keepdims=True))
            for b in range(nb): th.append(lambda b=b: ph_a(b))
            for b in range(nb): th.append(lambda b=b: ph_b(b))
            for b in range(nb): th.append(lambda b=b: ph_c(b))
            return th

        def mod2():
            cc = c_v[...].astype(F32)
            sc8 = jnp.broadcast_to(cc * jax.nn.sigmoid(cc), (8, D)).astype(BF16)
            mod = _r(jnp.dot(sc8, wm2_v[...], preferred_element_type=F32))
            for t in range(4):
                row = mod[0:1, t * D:(t + 1) * D]
                if t == 2: row = _r(1.0 + row)
                modc[t] = _col(row)
            modc[4] = _col(wr_v[...].reshape(1, D).astype(F32))

        def qp_tile(j, hb, rows, t):
            k0, k1 = KT[t]
            return jnp.dot(h_v[t, rows, 0:k1 - k0], wsl(wq_v, j, slice(k0, k1), hb), preferred_element_type=F32)

        def op_piece(j, hb, o_ref, rb, t, mode):
            rows = slice(t * 144, (t + 1) * 144)
            u = lax.dot_general(wsl(wo_v, j, rows, hb), o_ref[...], NT, preferred_element_type=F32)
            if mode == 'zero':
                acc[rb, rows, :] = jnp.zeros((144, T), F32)
            elif mode == 'commit':
                acc[rb, rows, :] += dlt[rb, rows, :]
            else:
                u = dlt[rb, rows, :] + u
            dlt[rb, rows, :] = u

        def period(j, par, chk, opspec, qpspec, th, seq):
            st = dict(l=None, o=None, q=None)
            ps = {}
            extra = {}
            n = len(seq)
            for i_, f_ in enumerate(th):
                extra.setdefault((i_ * n) // max(len(th), 1), []).append(f_)
            for i, (name, t) in enumerate(seq):
                for f_ in extra.get(i, []):
                    f_()
                if name == 'QK':
                    s = lax.dot_general(q_scr[par][...], k_v[j % NKV, t * T:(t + 1) * T, :], NT, preferred_element_type=F32)
                    p = jnp.exp2(s)
                    st['l'] = p if st['l'] is None else st['l'] + p
                    ps[t] = p.astype(BF16)
                elif name == 'PV':
                    o = jnp.dot(ps[t], v_v[j % NKV, t * T:(t + 1) * T, :], preferred_element_type=F32)
                    st['o'] = o if st['o'] is None else st['o'] + o
                    if t == 15:
                        l = jnp.sum(st['l'], axis=1, keepdims=True)
                        on = st['o'] * (1.0 / l)
                        o_scr[par][...] = on.astype(BF16)
                        lb = jnp.broadcast_to(l, (T, T))
                        chk['lmin'] = jnp.minimum(chk['lmin'], jnp.min(lb.reshape(T // 8, 8, T), axis=0))
                        chk['z'] = chk['z'] + _sum8(on + lb)
                elif name == 'OP':
                    op_piece(opspec[0], opspec[1], o_scr[1 - par], opspec[2], t, opspec[3])
                elif name == 'QP':
                    jq, hq, rbq = qpspec
                    rows = slice(rbq * T, (rbq + 1) * T) if isinstance(rbq, int) else pl.ds(pl.multiple_of(rbq * T, T), T)
                    d = qp_tile(jq, hq, rows, t)
                    st['q'] = d if st['q'] is None else st['q'] + d
                    if t == 4:
                        q_scr[1 - par][...] = (st['q'] * QSCALE).astype(BF16)

        def chk_new():
            return dict(lmin=jnp.full((8, T), 1.0, F32), z=jnp.zeros((8, T), F32))

        def chk_flush(chk, first):
            if first:
                chk_v[0:8, :] = chk['lmin']
                chk_v[8:16, :] = chk['z']
            else:
                chk_v[0:8, :] = jnp.minimum(chk_v[0:8, :], chk['lmin'])
                chk_v[8:16, :] = chk_v[8:16, :] + chk['z']

        def mid_step(j):
            chk = chk_new()
            for c in range(NPER if not kw.get('tiny_mid') else 2):
                opspec = (j, (c - 1) % 2, (c - 1) // 2, 'add' if (c - 1) % 2 else 'commit') if c >= 1 else (j - 1, 1, NRB - 1, 'add')
                qpspec = (j, (c + 1) % 2, (c + 1) // 2) if c + 1 < NPER else (j + 1, 0, 0)
                period(j, c % 2, chk, opspec, qpspec, [], seq_head if c == 0 else seq_tail if c == NPER - 1 else seq_mid)
            chk_flush(chk, True)

        def edge_step(j, kind):
            chk_flush(chk_new(), True)
            def body(it, carry):
                chk = chk_new()
                if kind == 'first':
                    edge_dma(it)
                    ra = jnp.minimum(2 * it + 2, NRB - 1)
                    rb_ = jnp.minimum(2 * it + 3, NRB - 1)
                    tha, thb = ln1_thunks(ra), ln1_thunks(rb_)
                else:
                    ra = jnp.maximum(2 * it - 2, 0)
                    rb_ = jnp.maximum(2 * it - 1, 0)
                    tha, thb = ln2_thunks(ra), ln2_thunks(rb_)
                ths = [tha[:len(tha) // 2], tha[len(tha) // 2:], thb[:len(thb) // 2], thb[len(thb) // 2:]]
                mode = 'zero' if kind == 'first' else 'commit'
                for c in range(4):
                    if c == 0:
                        if kind == 'first':
                            opspec = (j, 1, jnp.maximum(2 * it - 1, 0), 'add')
                        else:
                            opspec = (jnp.where(it == 0, j - 1, j), 1, (2 * it + NRB - 1) % NRB, 'add')
                    else:
                        opspec = (j, (c - 1) % 2, 2 * it + (c - 1) // 2, 'add' if (c - 1) % 2 else mode)
                    if c < 3:
                        qpspec = (j, (c + 1) % 2, 2 * it + (c + 1) // 2)
                    elif kind == 'first':
                        qpspec = (jnp.where(it == 7, j + 1, j), 0, (2 * it + 2) % NRB)
                    else:
                        qpspec = (j, 0, jnp.minimum(2 * it + 2, NRB - 1))
                    period(j, c % 2, chk, opspec, qpspec, ths[c], edge_seq(kind, c))
                chk_flush(chk, False)
                if kind == 'last':
                    @pl.when(it >= 1)
                    def _():
                        cp_o(2 * it - 2).start(); cp_o(2 * it - 1).start()
                return carry
            lax.fori_loop(0, NRB // 2, body, 0)

        def edge_dma(it):
            @pl.when(it < 6)
            def _():
                cp_x(2 * it + 4).start(); cp_x(2 * it + 5).start()
            @pl.when(it < 7)
            def _():
                cp_x(2 * it + 2).wait(); cp_x(2 * it + 3).wait()
            @pl.when(it == 1)
            def _():
                cp_wq(1).start(); cp_wr.start()
            @pl.when(it == 2)
            def _():
                cp_k(1).start(); cp_v(1).start()
            @pl.when(it == 3)
            def _():
                cp_wq(1).wait()
                cp_wo(1).start(); cp_wq(2).start()
            @pl.when(it == 4)
            def _():
                cp_wm2.start()

        def slow_step(j):
            def body(c, carry):
                rb = c // 2
                hb = c % 2
                rows = pl.ds(pl.multiple_of(rb * T, T), T)
                q = None
                for t_ in range(5):
                    d = qp_tile(j, hb, rows, t_)
                    q = d if q is None else q + d
                qs[...] = (q * QSCALE).astype(BF16)
                ms[...] = jnp.full((T, T), -jnp.inf, F32)
                def p1(t, carry_):
                    keys = pl.ds(pl.multiple_of(t * T, T), T)
                    s_ = lax.dot_general(qs[...], k_v[j % NKV, keys, :], NT, preferred_element_type=F32)
                    ss[t] = s_
                    ms[...] = jnp.maximum(ms[...], s_)
                    return carry_
                lax.fori_loop(0, S // T, p1, 0)
                ms[...] = jnp.broadcast_to(jnp.max(ms[...], axis=1, keepdims=True), (T, T))
                ls[...] = jnp.zeros((T, T), F32)
                os_[...] = jnp.zeros((T, T), F32)
                def p2(t, carry_):
                    keys = pl.ds(pl.multiple_of(t * T, T), T)
                    p = jnp.exp2(ss[t] - ms[...])
                    ls[...] += p
                    os_[...] += jnp.dot(p.astype(BF16), v_v[j % NKV, keys, :], preferred_element_type=F32)
                    return carry_
                lax.fori_loop(0, S // T, p2, 0)
                l = jnp.sum(ls[...], axis=1, keepdims=True)
                o1[...] = (os_[...] * (1.0 / l)).astype(BF16)
                @pl.when(c < NPER - 1)
                def _():
                    def po(t, carry_):
                        r_ = pl.ds(pl.multiple_of(t * 144, 16), 144)
                        u = lax.dot_general(wsl(wo_v, j, r_, hb), o1[...], NT, preferred_element_type=F32)
                        dlt[rb, r_, :] = jnp.where(hb == 0, 0.0, dlt[rb, r_, :]) + u
                        return carry_
                    lax.fori_loop(0, 4, po, 0)
                    @pl.when(jnp.logical_and(j == HKV - 1, hb == 1))
                    def _():
                        for f_ in ln2_thunks(rb, False):
                            f_()
                return carry
            with scope('SLOW'):
                lax.fori_loop(0, NPER, body, 0)

        W1 = kw.get('w1', 'c x0 wm1 wq0')
        W2 = kw.get('w2', 'k0 v0 x1 wq1 wo0')
        W3 = kw.get('w3', '')
        dm = dict(c=cp_c, x0=cp_x(0), wm1=cp_wm1, wq0=cp_w1(wq_hbm, wq_v, S_WQ0, 0, 0), k0=cp_k(0), v0=cp_v(0), x1=cp_x(1),
                  wq1=cp_w1(wq_hbm, wq_v, S_WQ1, 0, 1), wo0=cp_wo0)
        def wave(names):
            for n_ in names.split():
                dm[n_].start()
        wave(W1)
        o1[...] = jnp.zeros((T, DH), BF16)
        dlt[0] = jnp.zeros((D, T), F32)
        with scope('pro0'):
            cp_x(0).wait()
            th0 = ln1_thunks(0, False)
            for f_ in th0[:2 * nb]:
                f_()
            wave(W2)
            cp_c.wait(); cp_wm1.wait()
            wave(W3)
            cc = c_v[...].astype(F32)
            sc8 = jnp.broadcast_to(cc * jax.nn.sigmoid(cc), (8, D)).astype(BF16)
            mod = _r(jnp.dot(sc8, wm1_v[...], preferred_element_type=F32))
            modr[0:1, :] = 1.0 + mod[0:1, D:2 * D]
            modr[1:2, :] = mod[0:1, 0:D]
            for f_ in th0[2 * nb:]:
                f_()
            cp_w1(wq_hbm, wq_v, S_WQ0, 0, 0).wait()
            q = None
            for t in range(5):
                d = qp_tile(0, 0, slice(0, T), t)
                q = d if q is None else q + d
            q0[...] = (q * QSCALE).astype(BF16)
        cp_x(2).start(); cp_x(3).start()
        with scope('pro1'):
            cp_x(1).wait()
            for f_ in ln1_thunks(1, False):
                f_()
            cp_w1(wq_hbm, wq_v, S_WQ1, 0, 1).wait(); cp_k(0).wait(); cp_v(0).wait(); cp_wo0.wait()

        def step(j, carry):
            @pl.when(j == 0)
            def _():
                with scope('first'):
                    edge_step(0, 'first')
            @pl.when(jnp.logical_and(j > 0, j < HKV - 1))
            def _():
                with scope('wait'):
                    cp_k(j).wait(); cp_v(j).wait(); cp_wo(j).wait(); cp_wq(j + 1).wait()
                @pl.when(j + 2 < HKV)
                def _(): cp_wq(j + 2).start()
                @pl.when(j == 1)
                def _():
                    cp_wm2.wait(); cp_wr.wait()
                    mod2()
                    cp_wg.start()
                @pl.when(j == 2)
                def _(): cp_wu.start()
                @pl.when(j == 3)
                def _(): cp_wd.start()
                cp_k(j + 1).start(); cp_v(j + 1).start(); cp_wo(j + 1).start()
                with scope('midbody'):
                    mid_step(j)
            @pl.when(j == HKV - 1)
            def _():
                cp_k(HKV - 1).wait(); cp_v(HKV - 1).wait(); cp_wo(HKV - 1).wait()
                with scope('last'):
                    edge_step(HKV - 1, 'last')
                    for f_ in ln2_thunks(NRB - 2, False):
                        f_()
            ok = jnp.where((chk_v[0:8, :] >= LMIN) & (jnp.abs(chk_v[8:16, :]) < jnp.inf), 1.0, 0.0)
            @pl.when(jnp.min(ok) < (2.0 if kw.get('forceslow') else 0.5))
            def _():
                @pl.when(j == HKV - 1)
                def _():
                    for rb in range(NRB - 2):
                        cp_o(rb).wait()
                slow_step(j)
                @pl.when(j == HKV - 1)
                def _():
                    for rb in range(NRB - 2):
                        cp_o(rb).start()
            return carry
        lax.fori_loop(0, HKV, step, 0)
        jl = HKV - 1

        with scope('tail0'):
            cp_o(NRB - 2).start()
            for t in range(4):
                op_piece(jl, 1, o1, NRB - 1, t, 'add')
            for f_ in ln2_thunks(NRB - 1, False):
                f_()
            cp_o(NRB - 1).start()
        with scope('topk'):
            rb_ = pltpu.bitcast(r_v[...], jnp.int32) >> 16
            u = jnp.where(rb_ < 0, ~rb_, rb_ | 0x8000) & 0xFFFF
            tok = lax.broadcasted_iota(jnp.int32, (NRB, T), 0) * T + lax.broadcasted_iota(jnp.int32, (NRB, T), 1)
            key = pltpu.bitcast(((u << 11) | (S - 1 - tok)) + (1 << 27), F32)
            subs = lax.broadcasted_iota(jnp.int32, (8, T), 0)
            lane = lax.broadcasted_iota(jnp.int32, (8, T), 1)
            ksel = jnp.zeros((8, T), jnp.int32)
            for t in range(C):
                mx = jnp.max(jnp.max(key, axis=0, keepdims=True), axis=1, keepdims=True)
                key = jnp.where(key == mx, 0.0, key)
                ksel = jnp.where(subs == t, pltpu.bitcast(jnp.broadcast_to(mx, (8, T)), jnp.int32), ksel)
            ksel = ksel - (1 << 27)
            idxv = (S - 1) - (ksel & (S - 1))
            uu = ksel >> 11
            rbits = jnp.where((uu & 0x8000) != 0, uu & 0x7FFF, (~uu) & 0xFFFF) << 16
            rsel = pltpu.bitcast(rbits, F32)
            idxs = [jnp.max(jnp.where(subs == t, idxv, 0).astype(F32)).astype(jnp.int32) for t in range(C)]
        with scope('gather'):
            xs = None
            for t in range(C):
                oh = jnp.where((subs == t) & (lane == (idxv & (T - 1))), 1.0, 0.0).astype(BF16)
                n_t = jnp.clip(idxs[t] // T, 0, NRB - 1)
                d = lax.dot_general(oh, h2c[n_t], NT, preferred_element_type=F32)
                xs = d if xs is None else xs + d
        cp_wg.wait(); cp_wu.wait(); cp_wd.wait()
        with scope('ffn'):
            xb = xs.astype(BF16)
            g = _r(jnp.dot(xb, wg_v[...], preferred_element_type=F32))
            u_ = _r(jnp.dot(xb, wu_v[...], preferred_element_type=F32))
            g = _r(g * jax.nn.sigmoid(g))
            a = (g * u_).astype(BF16)
            y = _r(lax.dot_general(a, wd_v[...], NT, preferred_element_type=F32))
            y = _r(y * _r(jax.nn.sigmoid(rsel[:, 0:1])))
        with scope('fix'):
            for rb in range(NRB):
                cp_o(rb).wait()
            tiles = [jnp.clip(idxs[t] // T, 0, NRB - 1) for t in range(C)]
            if kw.get('fixmode', 'mxu') == 'mxu':
                yT = jnp.concatenate([y, jnp.zeros((T - 8, D), F32)], axis=0).T.astype(BF16)
                rowk = lax.broadcasted_iota(jnp.int32, (T, T), 0)
                lanes = lax.broadcasted_iota(jnp.int32, (T, T), 1)
            else:
                yT = jnp.concatenate([y, jnp.zeros((T - 8, D), F32)], axis=0).T * modc[3]
                lane1 = lax.broadcasted_iota(jnp.int32, (1, T), 1)
            def fix(t):
                if kw.get('fixmode', 'mxu') == 'mxu':
                    sel = jnp.where((rowk == t) & (lanes == (idxs[t] & (T - 1))), 1.0, 0.0).astype(BF16)
                    for p_ in range(4):
                        rows = slice(p_ * 144, (p_ + 1) * 144)
                        upd = jnp.dot(yT[rows, :], sel, preferred_element_type=F32)
                        out_c[tiles[t], rows, :] = (out_c[tiles[t], rows, :].astype(F32) + modc[3, rows, :] * upd).astype(BF16)
                else:
                    col = jnp.broadcast_to(yT[:, t:t + 1], (D, T))
                    hit = lane1 == (idxs[t] & (T - 1))
                    out_c[tiles[t]] = (out_c[tiles[t]].astype(F32) + jnp.where(hit, col, 0.0)).astype(BF16)
            final = []
            for t in range(C):
                f_ = jnp.bool_(True)
                for s_ in range(t + 1, C):
                    f_ = jnp.logical_and(f_, tiles[s_] != tiles[t])
                final.append(f_)
            GRP = kw.get('fixgrp', 4)
            for g0 in range(0, C, GRP):
                for t in range(g0, g0 + GRP):
                    fix(t)
                for t in range(g0, g0 + GRP):
                    @pl.when(final[t])
                    def _(t=t):
                        cp_o(tiles[t]).start()
        with scope('wout'):
            for t in range(C):
                @pl.when(final[t])
                def _(t=t):
                    cp_o(tiles[t]).wait()

    @jax.jit
    def fn(A_x, A_k_cache, A_v_cache, A_wq, A_wo, B_x, B_w_r, B_w_gate, B_w_up, B_w_down, c, w_mod):
        del B_x
        xT = A_x.reshape(S, D).T
        woT = A_wo.T
        wdT = B_w_down.T
        any_spec = pl.BlockSpec(memory_space=pl.ANY)
        outT = pl.pallas_call(
            kernel,
            in_specs=[any_spec] * 11,
            out_specs=any_spec,
            out_shape=jax.ShapeDtypeStruct((D, S), BF16),
            scratch_shapes=[
                pltpu.VMEM((NRB, D, T), BF16),
                pltpu.VMEM((NKV, S, DH), BF16),
                pltpu.VMEM((NKV, S, DH), BF16),
                pltpu.VMEM((2 * NW, D, T), BF16),
                pltpu.VMEM((2 * NW, D, T), BF16),
                pltpu.VMEM((D,), BF16),
                pltpu.VMEM((1, D), BF16),
                pltpu.VMEM((D, M1), BF16),
                pltpu.VMEM((D, 4 * D), BF16),
                pltpu.VMEM((D, FF), BF16),
                pltpu.VMEM((D, FF), BF16),
                pltpu.VMEM((D, FF), BF16),
                pltpu.VMEM((8, D), F32),
                pltpu.VMEM((5, D, T), F32),
                pltpu.VMEM((5, S, T), BF16),
                pltpu.VMEM((NRB, D, T), F32),
                pltpu.VMEM((NRB, D, T), F32),
                pltpu.VMEM((T, DH), BF16), pltpu.VMEM((T, DH), BF16),
                pltpu.VMEM((T, DH), BF16), pltpu.VMEM((T, DH), BF16),
                pltpu.VMEM((NRB, D, T), BF16),
                pltpu.VMEM((NRB, D, T), BF16),
                pltpu.VMEM((NRB, T), F32),
                pltpu.VMEM((D, T), F32),
                pltpu.VMEM((T, DH), BF16),
                pltpu.VMEM((S // T, T, T), F32),
                pltpu.VMEM((T, T), F32), pltpu.VMEM((T, T), F32), pltpu.VMEM((T, T), F32),
                pltpu.VMEM((16, T), F32),
                pltpu.SemaphoreType.DMA((NRB,)),
                pltpu.SemaphoreType.DMA((14,)),
            ],
            compiler_params=pltpu.CompilerParams(vmem_limit_bytes=110 * 1024 * 1024, flags=flags),
        )(xT, A_k_cache.reshape(HKV, S, DH), A_v_cache.reshape(HKV, S, DH), A_wq, woT,
          B_w_r, B_w_gate, B_w_up, wdT, c, w_mod)
        return outT.T.reshape(1, S, D)
    return fn


_KW = {'lag':7,'oppos':28,'qppos':7,'h_op':14,'f_ord':[[8,14,7],[7,28,7],[8,23,14],[7,'end',7]],'l_ord':[[7,14,0],[8,23,7],[8,14,14],[9,24,14]],'w1':'wm1 c x0 wq0 k0','w2':'v0','w3':'x1 wq1 wo0','fixgrp':2}
_impl = make(**_KW)


@jax.jit
def pallas_adaLN_cond__gqa_block_cached__moe_arch_mod__prompt_kernel(
    A_x: jax.Array,
    A_k_cache: jax.Array,
    A_v_cache: jax.Array,
    A_wq: jax.Array,
    A_wo: jax.Array,
    B_x: jax.Array,
    B_w_r: jax.Array,
    B_w_gate: jax.Array,
    B_w_up: jax.Array,
    B_w_down: jax.Array,
    c: jax.Array,
    w_mod: jax.Array,
):
    return _impl(A_x, A_k_cache, A_v_cache, A_wq, A_wo, B_x, B_w_r, B_w_gate, B_w_up, B_w_down, c, w_mod)
```

```python
import jax
import jax.numpy as jnp
from jax import lax
import numpy as np
import jax.experimental.pallas as pl
import jax.experimental.pallas.tpu as pltpu

D = 576
S = 2048
HKV = 16
DH = 128
FF = 4608
C = 8
EPS = 1e-5
T = 128
NRB = S // T
NPER = 2 * NRB
NB = 18
RBK = D // NB
NKV, NW = 2, 3
F32 = jnp.float32
BF16 = jnp.bfloat16
NT = (((1,), (1,)), ((), ()))
QSCALE = float(DH ** -0.5 * np.log2(np.e))
LMIN = float(2.0 ** -90)
KT = [(0, 128), (128, 256), (256, 384), (384, 512), (512, 576)]
M1 = 2 * D


def _r(x):
    return x.astype(BF16).astype(F32)


def _col(row):
    return jnp.broadcast_to(row, (T, D)).T


def _sum8(x):
    return jnp.sum(x.reshape(x.shape[0] // 8, 8, x.shape[1]), axis=0)


def _order(lag, oppos, qppos):
    toks = []
    for t in range(16 + lag):
        if t < 16:
            toks.append(('QK', t))
        if t >= lag:
            toks.append(('PV', t - lag))
    out = []
    for i, tk in enumerate(toks):
        if i == oppos:
            out += [('OP', p) for p in range(4)]
        if i == qppos:
            out += [('QP', p) for p in range(5)]
        out.append(tk)
    if oppos is None:
        out += [('OP', p) for p in range(4)]
    return out


SEQ_HEAD, SEQ_MID, SEQ_TAIL = _order(7, 14, 0), _order(7, 28, 7), _order(7, None, 7)
SEQ_FIRST = [_order(8, 14, 7), _order(7, 28, 7), _order(8, 23, 14), _order(7, None, 7)]
SEQ_LAST = [_order(7, 14, 0), _order(8, 23, 7), _order(8, 14, 14), _order(9, 24, 14)]


class _Pair:
    def __init__(self, a, b):
        self.a, self.b = a, b

    def start(self):
        self.a.start()
        self.b.start()

    def wait(self):
        self.a.wait()
        self.b.wait()


def _chunk(rb):
    return slice(rb * T, (rb + 1) * T) if isinstance(rb, int) else pl.ds(pl.multiple_of(rb * T, T), T)


def _kernel(xT_hbm, k_hbm, v_hbm, wq_hbm, woT_hbm, wr_hbm, wg_hbm, wu_hbm, wdT_hbm, c_hbm, wmod_hbm, outT_hbm,
            x_c, k_v, v_v, wq_v, wo_v, wr_v, c_v, wm1_v, wm2_v, wg_v, wu_v, wd_v,
            modr, modc, h_v, acc, dlt, q0, q1, o0, o1, h2c, out_c, r_v, x1s,
            qs, ss, ms, ls, os_, chk_v, xsem, sems):
    q_scr = (q0, q1)
    o_scr = (o0, o1)
    (S_K, S_V, S_WQ, S_WO, S_WR, S_C, S_WM1, S_WM2, S_WG, S_WU, S_WD, S_WO0, S_WQ0, S_WQ1) = range(14)

    def cp_k(j): return pltpu.make_async_copy(k_hbm.at[j], k_v.at[j % NKV], sems.at[S_K])
    def cp_v(j): return pltpu.make_async_copy(v_hbm.at[j], v_v.at[j % NKV], sems.at[S_V])
    def cp_w1(src, dst, sem, j, hb):
        return pltpu.make_async_copy(src.at[:, pl.ds(pl.multiple_of(j * 2 * T + hb * T, T), T)],
                                     dst.at[2 * (j % NW) + hb], sems.at[sem])
    def cp_w(src, dst, sem, j): return _Pair(cp_w1(src, dst, sem, j, 0), cp_w1(src, dst, sem, j, 1))
    def cp_wq(j): return cp_w(wq_hbm, wq_v, S_WQ, j)
    def cp_wo(j): return cp_w(woT_hbm, wo_v, S_WO, j)
    def cp_x(rb): return pltpu.make_async_copy(xT_hbm.at[:, _chunk(rb)], x_c.at[rb], xsem.at[rb])
    def cp_o(rb): return pltpu.make_async_copy(out_c.at[rb], outT_hbm.at[:, _chunk(rb)], xsem.at[rb])
    cp_wq00 = cp_w1(wq_hbm, wq_v, S_WQ0, 0, 0)
    cp_wq01 = cp_w1(wq_hbm, wq_v, S_WQ1, 0, 1)
    cp_wo0 = cp_w(woT_hbm, wo_v, S_WO0, 0)
    cp_wr = pltpu.make_async_copy(wr_hbm, wr_v, sems.at[S_WR])
    cp_c = pltpu.make_async_copy(c_hbm, c_v, sems.at[S_C])
    cp_wm1 = pltpu.make_async_copy(wmod_hbm.at[:, 0:M1], wm1_v, sems.at[S_WM1])
    cp_wm2 = pltpu.make_async_copy(wmod_hbm.at[:, M1:6 * D], wm2_v, sems.at[S_WM2])
    cp_wg = pltpu.make_async_copy(wg_hbm, wg_v, sems.at[S_WG])
    cp_wu = pltpu.make_async_copy(wu_hbm, wu_v, sems.at[S_WU])
    cp_wd = pltpu.make_async_copy(wdT_hbm, wd_v, sems.at[S_WD])

    def wsl(ref, j, rows, hb):
        return ref[2 * (j % NW) + hb, rows, :]

    def ln1_pieces(rb, pace):
        st = {}
        def mean(b):
            x = x_c[rb, b * RBK:(b + 1) * RBK, :].astype(F32)
            if b > 0 and pace:
                x = (x.reshape(RBK // 8, 8, T) + (st['s'] * 0.0)[None]).reshape(RBK, T)
            t = _sum8(x)
            st['s'] = t if b == 0 else st['s'] + t
            if b == NB - 1:
                st['m'] = jnp.broadcast_to(jnp.sum(st['s'], axis=0, keepdims=True) * (1.0 / D), (8, T))
        def var(b):
            m = st['m'] + st['v'] * 0.0 if (b > 0 and pace) else st['m']
            xc = x_c[rb, b * RBK:(b + 1) * RBK, :].astype(F32).reshape(RBK // 8, 8, T) - m[None]
            t = jnp.sum(xc * xc, axis=0)
            st['v'] = t if b == 0 else st['v'] + t
            if b == NB - 1:
                st['rs'] = lax.rsqrt(jnp.sum(st['v'], axis=0, keepdims=True) * (1.0 / D) + EPS)
        def norm(k):
            k0, k1 = KT[k]
            m = st['m'] + st['z'] * 0.0 if (k > 0 and pace) else st['m']
            xc = (x_c[rb, k0:k1, :].astype(F32).reshape((k1 - k0) // 8, 8, T) - m[None]).reshape(k1 - k0, T)
            xh = xc * st['rs']
            st['z'] = xh[0:8, :]
            h = xh.T * modr[0:1, k0:k1] + modr[1:2, k0:k1]
            h_v[k, _chunk(rb), 0:k1 - k0] = h.astype(BF16)
        return ([lambda b=b: mean(b) for b in range(NB)] + [lambda b=b: var(b) for b in range(NB)]
                + [lambda k=k: norm(k) for k in range(5)])

    def ln2_pieces(rb, pace):
        st = {}
        def resid(b):
            rows = slice(b * RBK, (b + 1) * RBK)
            a = acc[rb, rows, :] + dlt[rb, rows, :]
            if b > 0 and pace:
                a = (a.reshape(RBK // 8, 8, T) + (st['s'] * 0.0)[None]).reshape(RBK, T)
            x1 = x_c[rb, rows, :].astype(F32) + modc[0, rows, :] * a
            x1s[rows, :] = x1
            t = _sum8(x1)
            st['s'] = t if b == 0 else st['s'] + t
            if b == NB - 1:
                st['m'] = jnp.broadcast_to(jnp.sum(st['s'], axis=0, keepdims=True) * (1.0 / D), (8, T))
        def var(b):
            m = st['m'] + st['v'] * 0.0 if (b > 0 and pace) else st['m']
            xm = x1s[b * RBK:(b + 1) * RBK, :].reshape(RBK // 8, 8, T) - m[None]
            t = jnp.sum(xm * xm, axis=0)
            st['v'] = t if b == 0 else st['v'] + t
            if b == NB - 1:
                v = _r(jnp.sum(st['v'], axis=0, keepdims=True) * (1.0 / D))
                st['rd'] = 1.0 / _r(jnp.sqrt(_r(v + EPS)))
                st['mr'] = _r(st['m'])
        def norm(b):
            rows = slice(b * RBK, (b + 1) * RBK)
            x1 = x1s[rows, :]
            mr = st['mr'] + st['r'] * 0.0 if (b > 0 and pace) else st['mr']
            xc = (x1.reshape(RBK // 8, 8, T) - mr[None]).reshape(RBK, T)
            h2 = xc * st['rd'] * modc[2, rows, :] + modc[1, rows, :]
            t = _sum8(h2 * modc[4, rows, :])
            st['r'] = t if b == 0 else st['r'] + t
            h2c[rb, rows, :] = h2.astype(BF16)
            out_c[rb, rows, :] = (x1 + modc[3, rows, :] * h2).astype(BF16)
            if b == NB - 1:
                r_v[pl.ds(rb, 1), :] = _r(jnp.sum(st['r'], axis=0, keepdims=True))
        return ([lambda b=b: resid(b) for b in range(NB)] + [lambda b=b: var(b) for b in range(NB)]
                + [lambda b=b: norm(b) for b in range(NB)])

    def run(pieces):
        for f in pieces:
            f()

    def silu_c8():
        cc = c_v[...].astype(F32)
        return jnp.broadcast_to(cc * jax.nn.sigmoid(cc), (8, D)).astype(BF16)

    def mod_b():
        mod = _r(jnp.dot(silu_c8(), wm2_v[...], preferred_element_type=F32))
        for t in range(4):
            row = mod[0:1, t * D:(t + 1) * D]
            modc[t] = _col(_r(1.0 + row) if t == 2 else row)
        modc[4] = _col(wr_v[...].reshape(1, D).astype(F32))

    def qp_tile(j, hb, rows, t):
        k0, k1 = KT[t]
        return jnp.dot(h_v[t, rows, 0:k1 - k0], wsl(wq_v, j, slice(k0, k1), hb), preferred_element_type=F32)

    def op_piece(j, hb, o_ref, rb, t, mode):
        rows = slice(t * 144, (t + 1) * 144)
        u = lax.dot_general(wsl(wo_v, j, rows, hb), o_ref[...], NT, preferred_element_type=F32)
        if mode == 'zero':
            acc[rb, rows, :] = jnp.zeros((144, T), F32)
        elif mode == 'commit':
            acc[rb, rows, :] += dlt[rb, rows, :]
        else:
            u = dlt[rb, rows, :] + u
        dlt[rb, rows, :] = u

    def unit(j, par, chk, opspec, qpspec, pieces, seq):
        st = dict(l=None, o=None, q=None)
        ps = {}
        extra = {}
        for i, f in enumerate(pieces):
            extra.setdefault((i * len(seq)) // len(pieces), []).append(f)
        for i, (name, t) in enumerate(seq):
            run(extra.get(i, []))
            if name == 'QK':
                s = lax.dot_general(q_scr[par][...], k_v[j % NKV, t * T:(t + 1) * T, :], NT, preferred_element_type=F32)
                p = jnp.exp2(s)
                st['l'] = p if st['l'] is None else st['l'] + p
                ps[t] = p.astype(BF16)
            elif name == 'PV':
                o = jnp.dot(ps[t], v_v[j % NKV, t * T:(t + 1) * T, :], preferred_element_type=F32)
                st['o'] = o if st['o'] is None else st['o'] + o
                if t == 15:
                    l = jnp.sum(st['l'], axis=1, keepdims=True)
                    on = st['o'] * (1.0 / l)
                    o_scr[par][...] = on.astype(BF16)
                    lb = jnp.broadcast_to(l, (T, T))
                    chk['lmin'] = jnp.minimum(chk['lmin'], jnp.min(lb.reshape(T // 8, 8, T), axis=0))
                    chk['z'] = chk['z'] + _sum8(on + lb)
            elif name == 'OP':
                op_piece(opspec[0], opspec[1], o_scr[1 - par], opspec[2], t, opspec[3])
            else:
                d = qp_tile(qpspec[0], qpspec[1], _chunk(qpspec[2]), t)
                st['q'] = d if st['q'] is None else st['q'] + d
                if t == 4:
                    q_scr[1 - par][...] = (st['q'] * QSCALE).astype(BF16)

    def chk_new():
        return dict(lmin=jnp.full((8, T), 1.0, F32), z=jnp.zeros((8, T), F32))

    def chk_put(chk, first):
        if first:
            chk_v[0:8, :] = chk['lmin']
            chk_v[8:16, :] = chk['z']
        else:
            chk_v[0:8, :] = jnp.minimum(chk_v[0:8, :], chk['lmin'])
            chk_v[8:16, :] = chk_v[8:16, :] + chk['z']

    def mid_step(j):
        chk = chk_new()
        for c in range(NPER):
            if c >= 1:
                opspec = (j, (c - 1) % 2, (c - 1) // 2, 'add' if (c - 1) % 2 else 'commit')
            else:
                opspec = (j - 1, 1, NRB - 1, 'add')
            qpspec = (j, (c + 1) % 2, (c + 1) // 2) if c + 1 < NPER else (j + 1, 0, 0)
            unit(j, c % 2, chk, opspec, qpspec, [], SEQ_HEAD if c == 0 else SEQ_TAIL if c == NPER - 1 else SEQ_MID)
        chk_put(chk, True)

    def start_up_copies(it):
        @pl.when(it < 6)
        def _():
            cp_x(2 * it + 4).start(); cp_x(2 * it + 5).start()
        @pl.when(it < 7)
        def _():
            cp_x(2 * it + 2).wait(); cp_x(2 * it + 3).wait()
        @pl.when(it == 1)
        def _():
            cp_wq(1).start(); cp_wr.start()
        @pl.when(it == 2)
        def _():
            cp_k(1).start(); cp_v(1).start()
        @pl.when(it == 3)
        def _():
            cp_wq(1).wait()
            cp_wo(1).start(); cp_wq(2).start()
        @pl.when(it == 4)
        def _():
            cp_wm2.start()

    def edge_step(j, first):
        chk_put(chk_new(), True)
        def body(it, carry):
            chk = chk_new()
            if first:
                start_up_copies(it)
                pa = ln1_pieces(jnp.minimum(2 * it + 2, NRB - 1), True)
                pb = ln1_pieces(jnp.minimum(2 * it + 3, NRB - 1), True)
            else:
                pa = ln2_pieces(jnp.maximum(2 * it - 2, 0), True)
                pb = ln2_pieces(jnp.maximum(2 * it - 1, 0), True)
            pcs = [pa[:len(pa) // 2], pa[len(pa) // 2:], pb[:len(pb) // 2], pb[len(pb) // 2:]]
            for c in range(4):
                if c > 0:
                    mode = 'add' if (c - 1) % 2 else ('zero' if first else 'commit')
                    opspec = (j, (c - 1) % 2, 2 * it + (c - 1) // 2, mode)
                elif first:
                    opspec = (j, 1, jnp.maximum(2 * it - 1, 0), 'add')
                else:
                    opspec = (jnp.where(it == 0, j - 1, j), 1, (2 * it + NRB - 1) % NRB, 'add')
                if c < 3:
                    qpspec = (j, (c + 1) % 2, 2 * it + (c + 1) // 2)
                elif first:
                    qpspec = (jnp.where(it == 7, j + 1, j), 0, (2 * it + 2) % NRB)
                else:
                    qpspec = (j, 0, jnp.minimum(2 * it + 2, NRB - 1))
                unit(j, c % 2, chk, opspec, qpspec, pcs[c], (SEQ_FIRST if first else SEQ_LAST)[c])
            chk_put(chk, False)
            if not first:
                @pl.when(it >= 1)
                def _():
                    cp_o(2 * it - 2).start(); cp_o(2 * it - 1).start()
            return carry
        lax.fori_loop(0, NRB // 2, body, 0)

    def slow_step(j):
        def body(c, carry):
            rb = c // 2
            hb = c % 2
            q = None
            for t in range(5):
                d = qp_tile(j, hb, _chunk(rb), t)
                q = d if q is None else q + d
            qs[...] = (q * QSCALE).astype(BF16)
            ms[...] = jnp.full((T, T), -jnp.inf, F32)
            def scores(t, carry_):
                s = lax.dot_general(qs[...], k_v[j % NKV, _chunk(t), :], NT, preferred_element_type=F32)
                ss[t] = s
                ms[...] = jnp.maximum(ms[...], s)
                return carry_
            lax.fori_loop(0, S // T, scores, 0)
            ms[...] = jnp.broadcast_to(jnp.max(ms[...], axis=1, keepdims=True), (T, T))
            ls[...] = jnp.zeros((T, T), F32)
            os_[...] = jnp.zeros((T, T), F32)
            def weights(t, carry_):
                p = jnp.exp2(ss[t] - ms[...])
                ls[...] += p
                os_[...] += jnp.dot(p.astype(BF16), v_v[j % NKV, _chunk(t), :], preferred_element_type=F32)
                return carry_
            lax.fori_loop(0, S // T, weights, 0)
            l = jnp.sum(ls[...], axis=1, keepdims=True)
            o1[...] = (os_[...] * (1.0 / l)).astype(BF16)
            @pl.when(c < NPER - 1)
            def _():
                def proj(t, carry_):
                    rows = pl.ds(pl.multiple_of(t * 144, 16), 144)
                    u = lax.dot_general(wsl(wo_v, j, rows, hb), o1[...], NT, preferred_element_type=F32)
                    dlt[rb, rows, :] = jnp.where(hb == 0, 0.0, dlt[rb, rows, :]) + u
                    return carry_
                lax.fori_loop(0, 4, proj, 0)
                @pl.when(jnp.logical_and(j == HKV - 1, hb == 1))
                def _():
                    run(ln2_pieces(rb, False))
            return carry
        lax.fori_loop(0, NPER, body, 0)

    cp_wm1.start(); cp_c.start(); cp_x(0).start(); cp_wq00.start(); cp_k(0).start()
    o1[...] = jnp.zeros((T, DH), BF16)
    dlt[0] = jnp.zeros((D, T), F32)
    cp_x(0).wait()
    p0 = ln1_pieces(0, False)
    run(p0[:2 * NB])
    cp_v(0).start()
    cp_c.wait(); cp_wm1.wait()
    cp_x(1).start(); cp_wq01.start(); cp_wo0.start()
    mod = _r(jnp.dot(silu_c8(), wm1_v[...], preferred_element_type=F32))
    modr[0:1, :] = 1.0 + mod[0:1, D:2 * D]
    modr[1:2, :] = mod[0:1, 0:D]
    run(p0[2 * NB:])
    cp_wq00.wait()
    q = None
    for t in range(5):
        d = qp_tile(0, 0, _chunk(0), t)
        q = d if q is None else q + d
    q0[...] = (q * QSCALE).astype(BF16)
    cp_x(2).start(); cp_x(3).start()
    cp_x(1).wait()
    run(ln1_pieces(1, False))
    cp_wq01.wait(); cp_k(0).wait(); cp_v(0).wait(); cp_wo0.wait()

    def step(j, carry):
        @pl.when(j == 0)
        def _():
            edge_step(0, True)

        @pl.when(jnp.logical_and(j > 0, j < HKV - 1))
        def _():
            cp_k(j).wait(); cp_v(j).wait(); cp_wo(j).wait(); cp_wq(j + 1).wait()
            @pl.when(j + 2 < HKV)
            def _():
                cp_wq(j + 2).start()
            @pl.when(j == 1)
            def _():
                cp_wm2.wait(); cp_wr.wait()
                mod_b()
                cp_wg.start()
            @pl.when(j == 2)
            def _():
                cp_wu.start()
            @pl.when(j == 3)
            def _():
                cp_wd.start()
            cp_k(j + 1).start(); cp_v(j + 1).start(); cp_wo(j + 1).start()
            mid_step(j)

        @pl.when(j == HKV - 1)
        def _():
            cp_k(HKV - 1).wait(); cp_v(HKV - 1).wait(); cp_wo(HKV - 1).wait()
            edge_step(HKV - 1, False)
            run(ln2_pieces(NRB - 2, False))

        ok = jnp.where((chk_v[0:8, :] >= LMIN) & (jnp.abs(chk_v[8:16, :]) < jnp.inf), 1.0, 0.0)
        @pl.when(jnp.min(ok) < 0.5)
        def _():
            @pl.when(j == HKV - 1)
            def _():
                for rb in range(NRB - 2):
                    cp_o(rb).wait()
            slow_step(j)
            @pl.when(j == HKV - 1)
            def _():
                for rb in range(NRB - 2):
                    cp_o(rb).start()
        return carry
    lax.fori_loop(0, HKV, step, 0)

    cp_o(NRB - 2).start()
    for t in range(4):
        op_piece(HKV - 1, 1, o1, NRB - 1, t, 'add')
    run(ln2_pieces(NRB - 1, False))
    cp_o(NRB - 1).start()

    bits = pltpu.bitcast(r_v[...], jnp.int32) >> 16
    u = jnp.where(bits < 0, ~bits, bits | 0x8000) & 0xFFFF
    tok = lax.broadcasted_iota(jnp.int32, (NRB, T), 0) * T + lax.broadcasted_iota(jnp.int32, (NRB, T), 1)
    key = pltpu.bitcast(((u << 11) | (S - 1 - tok)) + (1 << 27), F32)
    subs = lax.broadcasted_iota(jnp.int32, (8, T), 0)
    lane = lax.broadcasted_iota(jnp.int32, (8, T), 1)
    ksel = jnp.zeros((8, T), jnp.int32)
    for t in range(C):
        mx = jnp.max(jnp.max(key, axis=0, keepdims=True), axis=1, keepdims=True)
        key = jnp.where(key == mx, 0.0, key)
        ksel = jnp.where(subs == t, pltpu.bitcast(jnp.broadcast_to(mx, (8, T)), jnp.int32), ksel)
    ksel = ksel - (1 << 27)
    idxv = (S - 1) - (ksel & (S - 1))
    uu = ksel >> 11
    rsel = pltpu.bitcast(jnp.where((uu & 0x8000) != 0, uu & 0x7FFF, (~uu) & 0xFFFF) << 16, F32)
    idxs = [jnp.max(jnp.where(subs == t, idxv, 0).astype(F32)).astype(jnp.int32) for t in range(C)]
    tiles = [jnp.clip(idxs[t] // T, 0, NRB - 1) for t in range(C)]

    xs = None
    for t in range(C):
        oh = jnp.where((subs == t) & (lane == (idxv & (T - 1))), 1.0, 0.0).astype(BF16)
        d = lax.dot_general(oh, h2c[tiles[t]], NT, preferred_element_type=F32)
        xs = d if xs is None else xs + d

    cp_wg.wait(); cp_wu.wait(); cp_wd.wait()
    xb = xs.astype(BF16)
    g = _r(jnp.dot(xb, wg_v[...], preferred_element_type=F32))
    up = _r(jnp.dot(xb, wu_v[...], preferred_element_type=F32))
    g = _r(g * jax.nn.sigmoid(g))
    a = (g * up).astype(BF16)
    y = _r(lax.dot_general(a, wd_v[...], NT, preferred_element_type=F32))
    y = _r(y * _r(jax.nn.sigmoid(rsel[:, 0:1])))

    for rb in range(NRB):
        cp_o(rb).wait()
    yT = jnp.concatenate([y, jnp.zeros((T - C, D), F32)], axis=0).T.astype(BF16)
    rowk = lax.broadcasted_iota(jnp.int32, (T, T), 0)
    lanes = lax.broadcasted_iota(jnp.int32, (T, T), 1)
    final = []
    for t in range(C):
        f = jnp.bool_(True)
        for s in range(t + 1, C):
            f = jnp.logical_and(f, tiles[s] != tiles[t])
        final.append(f)
    for g0 in range(0, C, 2):
        for t in range(g0, g0 + 2):
            sel = jnp.where((rowk == t) & (lanes == (idxs[t] & (T - 1))), 1.0, 0.0).astype(BF16)
            for p in range(4):
                rows = slice(p * 144, (p + 1) * 144)
                upd = jnp.dot(yT[rows, :], sel, preferred_element_type=F32)
                out_c[tiles[t], rows, :] = (out_c[tiles[t], rows, :].astype(F32) + modc[3, rows, :] * upd).astype(BF16)
        for t in range(g0, g0 + 2):
            @pl.when(final[t])
            def _(t=t):
                cp_o(tiles[t]).start()
    for t in range(C):
        @pl.when(final[t])
        def _(t=t):
            cp_o(tiles[t]).wait()


@jax.jit
def pallas_adaLN_cond__gqa_block_cached__moe_arch_mod__prompt_kernel(
    A_x: jax.Array,
    A_k_cache: jax.Array,
    A_v_cache: jax.Array,
    A_wq: jax.Array,
    A_wo: jax.Array,
    B_x: jax.Array,
    B_w_r: jax.Array,
    B_w_gate: jax.Array,
    B_w_up: jax.Array,
    B_w_down: jax.Array,
    c: jax.Array,
    w_mod: jax.Array,
):
    del B_x
    any_spec = pl.BlockSpec(memory_space=pl.ANY)
    tile = pltpu.VMEM((T, DH), BF16)
    outT = pl.pallas_call(
        _kernel,
        in_specs=[any_spec] * 11,
        out_specs=any_spec,
        out_shape=jax.ShapeDtypeStruct((D, S), BF16),
        scratch_shapes=[
            pltpu.VMEM((NRB, D, T), BF16),
            pltpu.VMEM((NKV, S, DH), BF16),
            pltpu.VMEM((NKV, S, DH), BF16),
            pltpu.VMEM((2 * NW, D, T), BF16),
            pltpu.VMEM((2 * NW, D, T), BF16),
            pltpu.VMEM((D,), BF16),
            pltpu.VMEM((1, D), BF16),
            pltpu.VMEM((D, M1), BF16),
            pltpu.VMEM((D, 4 * D), BF16),
            pltpu.VMEM((D, FF), BF16),
            pltpu.VMEM((D, FF), BF16),
            pltpu.VMEM((D, FF), BF16),
            pltpu.VMEM((8, D), F32),
            pltpu.VMEM((5, D, T), F32),
            pltpu.VMEM((5, S, T), BF16),
            pltpu.VMEM((NRB, D, T), F32),
            pltpu.VMEM((NRB, D, T), F32),
            tile, tile, tile, tile,
            pltpu.VMEM((NRB, D, T), BF16),
            pltpu.VMEM((NRB, D, T), BF16),
            pltpu.VMEM((NRB, T), F32),
            pltpu.VMEM((D, T), F32),
            tile,
            pltpu.VMEM((S // T, T, T), F32),
            pltpu.VMEM((T, T), F32), pltpu.VMEM((T, T), F32), pltpu.VMEM((T, T), F32),
            pltpu.VMEM((16, T), F32),
            pltpu.SemaphoreType.DMA((NRB,)),
            pltpu.SemaphoreType.DMA((14,)),
        ],
        compiler_params=pltpu.CompilerParams(vmem_limit_bytes=100 * 1024 * 1024),
    )(A_x.reshape(S, D).T, A_k_cache.reshape(HKV, S, DH), A_v_cache.reshape(HKV, S, DH), A_wq, A_wo.T,
      B_w_r, B_w_gate, B_w_up, B_w_down.T, c, w_mod)
    return outT.T.reshape(1, S, D)
```

```python
import jax
import jax.numpy as jnp
from jax import lax
import numpy as np
import jax.experimental.pallas as pl
import jax.experimental.pallas.tpu as pltpu

D = 576
S = 2048
HKV = 16
DH = 128
FF = 4608
C = 8
EPS = 1e-5
T = 128
NRB = S // T
NPER = 2 * NRB
NB = 18
RBK = D // NB
NKV, NW = 2, 3
F32 = jnp.float32
BF16 = jnp.bfloat16
NT = (((1,), (1,)), ((), ()))
QSCALE = float(DH ** -0.5 * np.log2(np.e))
LMIN = float(2.0 ** -90)
KT = [(0, 128), (128, 256), (256, 384), (384, 512), (512, 576)]
M1 = 2 * D


def _r(x):
    return x.astype(BF16).astype(F32)


def _col(row):
    return jnp.broadcast_to(row, (T, D)).T


def _sum8(x):
    return jnp.sum(x.reshape(x.shape[0] // 8, 8, x.shape[1]), axis=0)


def _order(lag, oppos, qppos):
    toks = []
    for t in range(16 + lag):
        if t < 16:
            toks.append(('QK', t))
        if t >= lag:
            toks.append(('PV', t - lag))
    out = []
    for i, tk in enumerate(toks):
        if i == oppos:
            out += [('OP', p) for p in range(4)]
        if i == qppos:
            out += [('QP', p) for p in range(5)]
        out.append(tk)
    if oppos is None:
        out += [('OP', p) for p in range(4)]
    return out


SEQ_HEAD, SEQ_MID, SEQ_TAIL = _order(7, 14, 0), _order(7, 28, 7), _order(7, None, 7)
SEQ_FIRST = [_order(8, 14, 7), _order(7, 28, 7), _order(8, 23, 14), _order(7, None, 7)]
SEQ_LAST = [_order(7, 14, 0), _order(8, 23, 7), _order(8, 14, 14), _order(9, 24, 14)]


class _Pair:
    def __init__(self, a, b):
        self.a, self.b = a, b

    def start(self):
        self.a.start()
        self.b.start()

    def wait(self):
        self.a.wait()
        self.b.wait()


def _chunk(rb):
    return slice(rb * T, (rb + 1) * T) if isinstance(rb, int) else pl.ds(pl.multiple_of(rb * T, T), T)


def _kernel(xT_hbm, k_hbm, v_hbm, wq_hbm, woT_hbm, wr_hbm, wg_hbm, wu_hbm, wdT_hbm, c_hbm, wmod_hbm, outT_hbm,
            x_c, k_v, v_v, wq_v, wo_v, wr_v, c_v, wm1_v, wm2_v, wg_v, wu_v, wd_v,
            modr, modc, h_v, acc, dlt, q0, q1, o0, o1, h2c, out_c, r_v, x1s,
            qs, ss, ms, ls, os_, chk_v, ok_s, xsem, sems):
    q_scr = (q0, q1)
    o_scr = (o0, o1)
    (S_K, S_V, S_WQ, S_WO, S_WR, S_C, S_WM1, S_WM2, S_WG, S_WU, S_WD, S_WO0, S_WQ0, S_WQ1) = range(14)

    def cp_k(j): return pltpu.make_async_copy(k_hbm.at[j], k_v.at[j % NKV], sems.at[S_K])
    def cp_v(j): return pltpu.make_async_copy(v_hbm.at[j], v_v.at[j % NKV], sems.at[S_V])
    def cp_w1(src, dst, sem, j, hb):
        return pltpu.make_async_copy(src.at[:, pl.ds(pl.multiple_of(j * 2 * T + hb * T, T), T)],
                                     dst.at[2 * (j % NW) + hb], sems.at[sem])
    def cp_w(src, dst, sem, j): return _Pair(cp_w1(src, dst, sem, j, 0), cp_w1(src, dst, sem, j, 1))
    def cp_wq(j): return cp_w(wq_hbm, wq_v, S_WQ, j)
    def cp_wo(j): return cp_w(woT_hbm, wo_v, S_WO, j)
    def cp_x(rb): return pltpu.make_async_copy(xT_hbm.at[:, _chunk(rb)], x_c.at[rb], xsem.at[rb])
    def cp_o(rb): return pltpu.make_async_copy(out_c.at[rb], outT_hbm.at[:, _chunk(rb)], xsem.at[rb])
    cp_wq00 = cp_w1(wq_hbm, wq_v, S_WQ0, 0, 0)
    cp_wq01 = cp_w1(wq_hbm, wq_v, S_WQ1, 0, 1)
    cp_wo0 = cp_w(woT_hbm, wo_v, S_WO0, 0)
    cp_wr = pltpu.make_async_copy(wr_hbm, wr_v, sems.at[S_WR])
    cp_c = pltpu.make_async_copy(c_hbm, c_v, sems.at[S_C])
    cp_wm1 = pltpu.make_async_copy(wmod_hbm.at[:, 0:M1], wm1_v, sems.at[S_WM1])
    cp_wm2 = pltpu.make_async_copy(wmod_hbm.at[:, M1:6 * D], wm2_v, sems.at[S_WM2])
    cp_wg = pltpu.make_async_copy(wg_hbm, wg_v, sems.at[S_WG])
    cp_wu = pltpu.make_async_copy(wu_hbm, wu_v, sems.at[S_WU])
    cp_wd = pltpu.make_async_copy(wdT_hbm, wd_v, sems.at[S_WD])

    def wsl(ref, j, rows, hb):
        return ref[2 * (j % NW) + hb, rows, :]

    def ln1_pieces(rb, pace):
        st = {}
        def mean(b):
            x = x_c[rb, b * RBK:(b + 1) * RBK, :].astype(F32)
            if b > 0 and pace:
                x = (x.reshape(RBK // 8, 8, T) + (st['s'] * 0.0)[None]).reshape(RBK, T)
            t = _sum8(x)
            st['s'] = t if b == 0 else st['s'] + t
            if b == NB - 1:
                st['m'] = jnp.broadcast_to(jnp.sum(st['s'], axis=0, keepdims=True) * (1.0 / D), (8, T))
        def var(b):
            m = st['m'] + st['v'] * 0.0 if (b > 0 and pace) else st['m']
            xc = x_c[rb, b * RBK:(b + 1) * RBK, :].astype(F32).reshape(RBK // 8, 8, T) - m[None]
            t = jnp.sum(xc * xc, axis=0)
            st['v'] = t if b == 0 else st['v'] + t
            if b == NB - 1:
                st['rs'] = lax.rsqrt(jnp.sum(st['v'], axis=0, keepdims=True) * (1.0 / D) + EPS)
        def norm(k):
            k0, k1 = KT[k]
            m = st['m'] + st['z'] * 0.0 if (k > 0 and pace) else st['m']
            xc = (x_c[rb, k0:k1, :].astype(F32).reshape((k1 - k0) // 8, 8, T) - m[None]).reshape(k1 - k0, T)
            xh = xc * st['rs']
            st['z'] = xh[0:8, :]
            h = xh.T * modr[0:1, k0:k1] + modr[1:2, k0:k1]
            h_v[k, _chunk(rb), 0:k1 - k0] = h.astype(BF16)
        return ([lambda b=b: mean(b) for b in range(NB)] + [lambda b=b: var(b) for b in range(NB)]
                + [lambda k=k: norm(k) for k in range(5)])

    def ln2_pieces(rb, pace):
        st = {}
        def resid(b):
            rows = slice(b * RBK, (b + 1) * RBK)
            a = acc[rb, rows, :] + dlt[rb, rows, :]
            if b > 0 and pace:
                a = (a.reshape(RBK // 8, 8, T) + (st['s'] * 0.0)[None]).reshape(RBK, T)
            x1 = x_c[rb, rows, :].astype(F32) + modc[0, rows, :] * a
            x1s[rows, :] = x1
            t = _sum8(x1)
            st['s'] = t if b == 0 else st['s'] + t
            if b == NB - 1:
                st['m'] = jnp.broadcast_to(jnp.sum(st['s'], axis=0, keepdims=True) * (1.0 / D), (8, T))
        def var(b):
            m = st['m'] + st['v'] * 0.0 if (b > 0 and pace) else st['m']
            xm = x1s[b * RBK:(b + 1) * RBK, :].reshape(RBK // 8, 8, T) - m[None]
            t = jnp.sum(xm * xm, axis=0)
            st['v'] = t if b == 0 else st['v'] + t
            if b == NB - 1:
                v = _r(jnp.sum(st['v'], axis=0, keepdims=True) * (1.0 / D))
                st['rd'] = 1.0 / _r(jnp.sqrt(_r(v + EPS)))
                st['mr'] = _r(st['m'])
        def norm(b):
            rows = slice(b * RBK, (b + 1) * RBK)
            x1 = x1s[rows, :]
            mr = st['mr'] + st['r'] * 0.0 if (b > 0 and pace) else st['mr']
            xc = (x1.reshape(RBK // 8, 8, T) - mr[None]).reshape(RBK, T)
            h2 = xc * st['rd'] * modc[2, rows, :] + modc[1, rows, :]
            t = _sum8(h2 * modc[4, rows, :])
            st['r'] = t if b == 0 else st['r'] + t
            h2c[rb, rows, :] = h2.astype(BF16)
            out_c[rb, rows, :] = (x1 + modc[3, rows, :] * h2).astype(BF16)
            if b == NB - 1:
                r_v[pl.ds(rb, 1), :] = _r(jnp.sum(st['r'], axis=0, keepdims=True))
        return ([lambda b=b: resid(b) for b in range(NB)] + [lambda b=b: var(b) for b in range(NB)]
                + [lambda b=b: norm(b) for b in range(NB)])

    def run(pieces):
        for f in pieces:
            f()

    def silu_c8():
        cc = c_v[...].astype(F32)
        return jnp.broadcast_to(cc * jax.nn.sigmoid(cc), (8, D)).astype(BF16)

    def mod_b():
        mod = _r(jnp.dot(silu_c8(), wm2_v[...], preferred_element_type=F32))
        for t in range(4):
            row = mod[0:1, t * D:(t + 1) * D]
            modc[t] = _col(_r(1.0 + row) if t == 2 else row)
        modc[4] = _col(wr_v[...].reshape(1, D).astype(F32))

    def qp_tile(j, hb, rows, t):
        k0, k1 = KT[t]
        return jnp.dot(h_v[t, rows, 0:k1 - k0], wsl(wq_v, j, slice(k0, k1), hb), preferred_element_type=F32)

    def op_piece(j, hb, o_ref, rb, t, mode):
        rows = slice(t * 144, (t + 1) * 144)
        u = lax.dot_general(wsl(wo_v, j, rows, hb), o_ref[...], NT, preferred_element_type=F32)
        if mode == 'zero':
            acc[rb, rows, :] = jnp.zeros((144, T), F32)
        elif mode == 'commit':
            acc[rb, rows, :] += dlt[rb, rows, :]
        else:
            u = dlt[rb, rows, :] + u
        dlt[rb, rows, :] = u

    def unit(j, par, chk, opspec, qpspec, pieces, seq):
        st = dict(l=None, o=None, q=None)
        ps = {}
        extra = {}
        for i, f in enumerate(pieces):
            extra.setdefault((i * len(seq)) // len(pieces), []).append(f)
        for i, (name, t) in enumerate(seq):
            run(extra.get(i, []))
            if name == 'QK':
                s = lax.dot_general(q_scr[par][...], k_v[j % NKV, t * T:(t + 1) * T, :], NT, preferred_element_type=F32)
                p = jnp.exp2(s)
                st['l'] = p if st['l'] is None else st['l'] + p
                ps[t] = p.astype(BF16)
            elif name == 'PV':
                o = jnp.dot(ps[t], v_v[j % NKV, t * T:(t + 1) * T, :], preferred_element_type=F32)
                st['o'] = o if st['o'] is None else st['o'] + o
                if t == 15:
                    l = jnp.sum(st['l'], axis=1, keepdims=True)
                    on = st['o'] * (1.0 / l)
                    o_scr[par][...] = on.astype(BF16)
                    lb = jnp.broadcast_to(l, (T, T))
                    chk['lmin'] = jnp.minimum(chk['lmin'], jnp.min(lb.reshape(T // 8, 8, T), axis=0))
                    chk['z'] = chk['z'] + _sum8(on + lb)
            elif name == 'OP':
                op_piece(opspec[0], opspec[1], o_scr[1 - par], opspec[2], t, opspec[3])
            else:
                d = qp_tile(qpspec[0], qpspec[1], _chunk(qpspec[2]), t)
                st['q'] = d if st['q'] is None else st['q'] + d
                if t == 4:
                    q_scr[1 - par][...] = (st['q'] * QSCALE).astype(BF16)

    def chk_new():
        return dict(lmin=jnp.full((8, T), 1.0, F32), z=jnp.zeros((8, T), F32))

    def chk_put(chk, first):
        if first:
            chk_v[0:8, :] = chk['lmin']
            chk_v[8:16, :] = chk['z']
        else:
            chk_v[0:8, :] = jnp.minimum(chk_v[0:8, :], chk['lmin'])
            chk_v[8:16, :] = chk_v[8:16, :] + chk['z']

    def chk_ok(lmin, z):
        return jnp.min(jnp.where((lmin >= LMIN) & (jnp.abs(z) < jnp.inf), 1.0, 0.0))

    def mid_step(j):
        chk = chk_new()
        for c in range(NPER):
            if c >= 1:
                opspec = (j, (c - 1) % 2, (c - 1) // 2, 'add' if (c - 1) % 2 else 'commit')
            else:
                opspec = (j - 1, 1, NRB - 1, 'add')
            qpspec = (j, (c + 1) % 2, (c + 1) // 2) if c + 1 < NPER else (j + 1, 0, 0)
            unit(j, c % 2, chk, opspec, qpspec, [], SEQ_HEAD if c == 0 else SEQ_TAIL if c == NPER - 1 else SEQ_MID)
        ok_s[0] = chk_ok(chk['lmin'], chk['z'])

    def start_up_copies(it):
        @pl.when(it < 6)
        def _():
            cp_x(2 * it + 4).start(); cp_x(2 * it + 5).start()
        @pl.when(it < 7)
        def _():
            cp_x(2 * it + 2).wait(); cp_x(2 * it + 3).wait()
        @pl.when(it == 1)
        def _():
            cp_wq(1).start(); cp_wr.start()
        @pl.when(it == 2)
        def _():
            cp_k(1).start(); cp_v(1).start()
        @pl.when(it == 3)
        def _():
            cp_wq(1).wait()
            cp_wo(1).start(); cp_wq(2).start()
        @pl.when(it == 4)
        def _():
            cp_wm2.start()

    def edge_step(j, first):
        chk_put(chk_new(), True)
        def body(it, carry):
            chk = chk_new()
            if first:
                start_up_copies(it)
                pa = ln1_pieces(jnp.minimum(2 * it + 2, NRB - 1), True)
                pb = ln1_pieces(jnp.minimum(2 * it + 3, NRB - 1), True)
            else:
                pa = ln2_pieces(jnp.maximum(2 * it - 2, 0), True)
                pb = ln2_pieces(jnp.maximum(2 * it - 1, 0), True)
            pcs = [pa[:len(pa) // 2], pa[len(pa) // 2:], pb[:len(pb) // 2], pb[len(pb) // 2:]]
            for c in range(4):
                if c > 0:
                    mode = 'add' if (c - 1) % 2 else ('zero' if first else 'commit')
                    opspec = (j, (c - 1) % 2, 2 * it + (c - 1) // 2, mode)
                elif first:
                    opspec = (j, 1, jnp.maximum(2 * it - 1, 0), 'add')
                else:
                    opspec = (jnp.where(it == 0, j - 1, j), 1, (2 * it + NRB - 1) % NRB, 'add')
                if c < 3:
                    qpspec = (j, (c + 1) % 2, 2 * it + (c + 1) // 2)
                elif first:
                    qpspec = (jnp.where(it == 7, j + 1, j), 0, (2 * it + 2) % NRB)
                else:
                    qpspec = (j, 0, jnp.minimum(2 * it + 2, NRB - 1))
                unit(j, c % 2, chk, opspec, qpspec, pcs[c], (SEQ_FIRST if first else SEQ_LAST)[c])
            chk_put(chk, False)
            if not first:
                @pl.when(it >= 1)
                def _():
                    cp_o(2 * it - 2).start(); cp_o(2 * it - 1).start()
            return carry
        lax.fori_loop(0, NRB // 2, body, 0)
        ok_s[0] = chk_ok(chk_v[0:8, :], chk_v[8:16, :])

    def slow_step(j):
        def body(c, carry):
            rb = c // 2
            hb = c % 2
            q = None
            for t in range(5):
                d = qp_tile(j, hb, _chunk(rb), t)
                q = d if q is None else q + d
            qs[...] = (q * QSCALE).astype(BF16)
            ms[...] = jnp.full((T, T), -jnp.inf, F32)
            def scores(t, carry_):
                s = lax.dot_general(qs[...], k_v[j % NKV, _chunk(t), :], NT, preferred_element_type=F32)
                ss[t] = s
                ms[...] = jnp.maximum(ms[...], s)
                return carry_
            lax.fori_loop(0, S // T, scores, 0)
            ms[...] = jnp.broadcast_to(jnp.max(ms[...], axis=1, keepdims=True), (T, T))
            ls[...] = jnp.zeros((T, T), F32)
            os_[...] = jnp.zeros((T, T), F32)
            def weights(t, carry_):
                p = jnp.exp2(ss[t] - ms[...])
                ls[...] += p
                os_[...] += jnp.dot(p.astype(BF16), v_v[j % NKV, _chunk(t), :], preferred_element_type=F32)
                return carry_
            lax.fori_loop(0, S // T, weights, 0)
            l = jnp.sum(ls[...], axis=1, keepdims=True)
            o1[...] = (os_[...] * (1.0 / l)).astype(BF16)
            @pl.when(c < NPER - 1)
            def _():
                def proj(t, carry_):
                    rows = pl.ds(pl.multiple_of(t * 144, 16), 144)
                    u = lax.dot_general(wsl(wo_v, j, rows, hb), o1[...], NT, preferred_element_type=F32)
                    dlt[rb, rows, :] = jnp.where(hb == 0, 0.0, dlt[rb, rows, :]) + u
                    return carry_
                lax.fori_loop(0, 4, proj, 0)
                @pl.when(jnp.logical_and(j == HKV - 1, hb == 1))
                def _():
                    run(ln2_pieces(rb, False))
            return carry
        lax.fori_loop(0, NPER, body, 0)

    cp_wm1.start(); cp_c.start(); cp_x(0).start(); cp_wq00.start(); cp_k(0).start()
    o1[...] = jnp.zeros((T, DH), BF16)
    dlt[0] = jnp.zeros((D, T), F32)
    cp_x(0).wait()
    p0 = ln1_pieces(0, False)
    run(p0[:2 * NB])
    cp_v(0).start()
    cp_c.wait(); cp_wm1.wait()
    cp_x(1).start(); cp_wq01.start(); cp_wo0.start()
    mod = _r(jnp.dot(silu_c8(), wm1_v[...], preferred_element_type=F32))
    modr[0:1, :] = 1.0 + mod[0:1, D:2 * D]
    modr[1:2, :] = mod[0:1, 0:D]
    run(p0[2 * NB:])
    cp_wq00.wait()
    q = None
    for t in range(5):
        d = qp_tile(0, 0, _chunk(0), t)
        q = d if q is None else q + d
    q0[...] = (q * QSCALE).astype(BF16)
    cp_x(2).start(); cp_x(3).start()
    cp_x(1).wait()
    run(ln1_pieces(1, False))
    cp_wq01.wait(); cp_k(0).wait(); cp_v(0).wait(); cp_wo0.wait()

    def step(j, carry):
        @pl.when(j == 0)
        def _():
            edge_step(0, True)

        @pl.when(jnp.logical_and(j > 0, j < HKV - 1))
        def _():
            cp_k(j).wait(); cp_v(j).wait(); cp_wo(j).wait(); cp_wq(j + 1).wait()
            @pl.when(j + 2 < HKV)
            def _():
                cp_wq(j + 2).start()
            @pl.when(j == 1)
            def _():
                cp_wm2.wait(); cp_wr.wait()
                mod_b()
                cp_wg.start()
            @pl.when(j == 2)
            def _():
                cp_wu.start()
            @pl.when(j == 3)
            def _():
                cp_wd.start()
            cp_k(j + 1).start(); cp_v(j + 1).start(); cp_wo(j + 1).start()
            mid_step(j)

        @pl.when(j == HKV - 1)
        def _():
            cp_k(HKV - 1).wait(); cp_v(HKV - 1).wait(); cp_wo(HKV - 1).wait()
            edge_step(HKV - 1, False)
            run(ln2_pieces(NRB - 2, False))

        @pl.when(ok_s[0] < 0.5)
        def _():
            @pl.when(j == HKV - 1)
            def _():
                for rb in range(NRB - 2):
                    cp_o(rb).wait()
            slow_step(j)
            @pl.when(j == HKV - 1)
            def _():
                for rb in range(NRB - 2):
                    cp_o(rb).start()
        return carry
    lax.fori_loop(0, HKV, step, 0)

    cp_o(NRB - 2).start()
    for t in range(4):
        op_piece(HKV - 1, 1, o1, NRB - 1, t, 'add')
    run(ln2_pieces(NRB - 1, False))
    cp_o(NRB - 1).start()

    bits = pltpu.bitcast(r_v[...], jnp.int32) >> 16
    u = jnp.where(bits < 0, ~bits, bits | 0x8000) & 0xFFFF
    tok = lax.broadcasted_iota(jnp.int32, (NRB, T), 0) * T + lax.broadcasted_iota(jnp.int32, (NRB, T), 1)
    key = pltpu.bitcast(((u << 11) | (S - 1 - tok)) + (1 << 27), F32)
    subs = lax.broadcasted_iota(jnp.int32, (8, T), 0)
    lane = lax.broadcasted_iota(jnp.int32, (8, T), 1)
    ksel = jnp.zeros((8, T), jnp.int32)
    for t in range(C):
        mx = jnp.max(jnp.max(key, axis=0, keepdims=True), axis=1, keepdims=True)
        key = jnp.where(key == mx, 0.0, key)
        ksel = jnp.where(subs == t, pltpu.bitcast(jnp.broadcast_to(mx, (8, T)), jnp.int32), ksel)
    ksel = ksel - (1 << 27)
    idxv = (S - 1) - (ksel & (S - 1))
    uu = ksel >> 11
    rsel = pltpu.bitcast(jnp.where((uu & 0x8000) != 0, uu & 0x7FFF, (~uu) & 0xFFFF) << 16, F32)
    idxs = [jnp.max(jnp.where(subs == t, idxv, 0).astype(F32)).astype(jnp.int32) for t in range(C)]
    tiles = [jnp.clip(idxs[t] // T, 0, NRB - 1) for t in range(C)]

    xs = None
    for t in range(C):
        oh = jnp.where((subs == t) & (lane == (idxv & (T - 1))), 1.0, 0.0).astype(BF16)
        d = lax.dot_general(oh, h2c[tiles[t]], NT, preferred_element_type=F32)
        xs = d if xs is None else xs + d

    cp_wg.wait(); cp_wu.wait(); cp_wd.wait()
    xb = xs.astype(BF16)
    g = _r(jnp.dot(xb, wg_v[...], preferred_element_type=F32))
    up = _r(jnp.dot(xb, wu_v[...], preferred_element_type=F32))
    g = _r(g * jax.nn.sigmoid(g))
    a = (g * up).astype(BF16)
    y = _r(lax.dot_general(a, wd_v[...], NT, preferred_element_type=F32))
    y = _r(y * _r(jax.nn.sigmoid(rsel[:, 0:1])))

    for rb in range(NRB):
        cp_o(rb).wait()
    yT = jnp.concatenate([y, jnp.zeros((T - C, D), F32)], axis=0).T.astype(BF16)
    rowk = lax.broadcasted_iota(jnp.int32, (T, T), 0)
    lanes = lax.broadcasted_iota(jnp.int32, (T, T), 1)
    final = []
    for t in range(C):
        f = jnp.bool_(True)
        for s in range(t + 1, C):
            f = jnp.logical_and(f, tiles[s] != tiles[t])
        final.append(f)
    for g0 in range(0, C, 2):
        for t in range(g0, g0 + 2):
            sel = jnp.where((rowk == t) & (lanes == (idxs[t] & (T - 1))), 1.0, 0.0).astype(BF16)
            for p in range(4):
                rows = slice(p * 144, (p + 1) * 144)
                upd = jnp.dot(yT[rows, :], sel, preferred_element_type=F32)
                out_c[tiles[t], rows, :] = (out_c[tiles[t], rows, :].astype(F32) + modc[3, rows, :] * upd).astype(BF16)
        for t in range(g0, g0 + 2):
            @pl.when(final[t])
            def _(t=t):
                cp_o(tiles[t]).start()
    for t in range(C):
        @pl.when(final[t])
        def _(t=t):
            cp_o(tiles[t]).wait()


@jax.jit
def pallas_adaLN_cond__gqa_block_cached__moe_arch_mod__prompt_kernel(
    A_x: jax.Array,
    A_k_cache: jax.Array,
    A_v_cache: jax.Array,
    A_wq: jax.Array,
    A_wo: jax.Array,
    B_x: jax.Array,
    B_w_r: jax.Array,
    B_w_gate: jax.Array,
    B_w_up: jax.Array,
    B_w_down: jax.Array,
    c: jax.Array,
    w_mod: jax.Array,
):
    del B_x
    any_spec = pl.BlockSpec(memory_space=pl.ANY)
    tile = pltpu.VMEM((T, DH), BF16)
    outT = pl.pallas_call(
        _kernel,
        in_specs=[any_spec] * 11,
        out_specs=any_spec,
        out_shape=jax.ShapeDtypeStruct((D, S), BF16),
        scratch_shapes=[
            pltpu.VMEM((NRB, D, T), BF16),
            pltpu.VMEM((NKV, S, DH), BF16),
            pltpu.VMEM((NKV, S, DH), BF16),
            pltpu.VMEM((2 * NW, D, T), BF16),
            pltpu.VMEM((2 * NW, D, T), BF16),
            pltpu.VMEM((D,), BF16),
            pltpu.VMEM((1, D), BF16),
            pltpu.VMEM((D, M1), BF16),
            pltpu.VMEM((D, 4 * D), BF16),
            pltpu.VMEM((D, FF), BF16),
            pltpu.VMEM((D, FF), BF16),
            pltpu.VMEM((D, FF), BF16),
            pltpu.VMEM((8, D), F32),
            pltpu.VMEM((5, D, T), F32),
            pltpu.VMEM((5, S, T), BF16),
            pltpu.VMEM((NRB, D, T), F32),
            pltpu.VMEM((NRB, D, T), F32),
            tile, tile, tile, tile,
            pltpu.VMEM((NRB, D, T), BF16),
            pltpu.VMEM((NRB, D, T), BF16),
            pltpu.VMEM((NRB, T), F32),
            pltpu.VMEM((D, T), F32),
            tile,
            pltpu.VMEM((S // T, T, T), F32),
            pltpu.VMEM((T, T), F32), pltpu.VMEM((T, T), F32), pltpu.VMEM((T, T), F32),
            pltpu.VMEM((16, T), F32),
            pltpu.SMEM((1,), F32),
            pltpu.SemaphoreType.DMA((NRB,)),
            pltpu.SemaphoreType.DMA((14,)),
        ],
        compiler_params=pltpu.CompilerParams(vmem_limit_bytes=100 * 1024 * 1024),
    )(A_x.reshape(S, D).T, A_k_cache.reshape(HKV, S, DH), A_v_cache.reshape(HKV, S, DH), A_wq, A_wo.T,
      B_w_r, B_w_gate, B_w_up, B_w_down.T, c, w_mod)
    return outT.T.reshape(1, S, D)
```

```python
import jax
import jax.numpy as jnp
from jax import lax
import numpy as np
import jax.experimental.pallas as pl
import jax.experimental.pallas.tpu as pltpu

D = 576
S = 2048
HKV = 16
DH = 128
FF = 4608
C = 8
EPS = 1e-5
T = 128
NRB = S // T
NPER = 2 * NRB
NB = 18
RBK = D // NB
NKV, NW = 2, 3
F32 = jnp.float32
BF16 = jnp.bfloat16
NT = (((1,), (1,)), ((), ()))
QSCALE = float(DH ** -0.5 * np.log2(np.e))
LMIN = float(2.0 ** -60)
KT = [(0, 128), (128, 256), (256, 384), (384, 512), (512, 576)]
M1 = 2 * D


def _r(x):
    return x.astype(BF16).astype(F32)


def _col(row):
    return jnp.broadcast_to(row, (T, D)).T


def _sum8(x):
    return jnp.sum(x.reshape(x.shape[0] // 8, 8, x.shape[1]), axis=0)


def _order(lag, oppos, qppos):
    toks = []
    for t in range(16 + lag):
        if t < 16:
            toks.append(('QK', t))
        if t >= lag:
            toks.append(('PV', t - lag))
    out = []
    for i, tk in enumerate(toks):
        if i == oppos:
            out += [('OP', p) for p in range(4)]
        if i == qppos:
            out += [('QP', p) for p in range(5)]
        out.append(tk)
    if oppos is None:
        out += [('OP', p) for p in range(4)]
    return out


SEQ_HEAD, SEQ_MID, SEQ_TAIL = _order(7, 14, 0), _order(7, 28, 7), _order(7, None, 7)
SEQ_FIRST = [_order(8, 14, 7), _order(7, 28, 7), _order(8, 23, 14), _order(7, None, 7)]
SEQ_LAST = [_order(7, 14, 0), _order(8, 23, 7), _order(8, 14, 14), _order(9, 24, 14)]


def _chunk(rb):
    return slice(rb * T, (rb + 1) * T) if isinstance(rb, int) else pl.ds(pl.multiple_of(rb * T, T), T)


def _kernel(xT_hbm, k_hbm, v_hbm, wq_hbm, woT_hbm, wr_hbm, wg_hbm, wu_hbm, wdT_hbm, c_hbm, wmod_hbm, outT_hbm,
            x_c, k_v, v_v, wq_v, wo_v, wr_v, c_v, wm1_v, wm2_v, wg_v, wu_v, wd_v,
            modr, modc, h_v, acc, dlt, q0, q1, o0, o1, h2c, out_c, r_v, x1s,
            qs, ss, ms, ls, os_, chk_v, ok_s, xsem, sems):
    q_scr = (q0, q1)
    o_scr = (o0, o1)
    (S_K, S_V, S_WQ, S_WO, S_WR, S_C, S_WM1, S_WM2, S_WG, S_WU, S_WD, S_WO0, S_WQ0, S_WQ1) = range(14)

    def cp_k(j): return pltpu.make_async_copy(k_hbm.at[j], k_v.at[j % NKV], sems.at[S_K])
    def cp_v(j): return pltpu.make_async_copy(v_hbm.at[j], v_v.at[j % NKV], sems.at[S_V])
    def cp_w(src, dst, sem, j):
        return pltpu.make_async_copy(src.at[:, pl.ds(pl.multiple_of(j * 2 * T, 2 * T), 2 * T)], dst.at[j % NW], sems.at[sem])
    def cp_wq(j): return cp_w(wq_hbm, wq_v, S_WQ, j)
    def cp_wo(j): return cp_w(woT_hbm, wo_v, S_WO, j)
    def cp_x(rb): return pltpu.make_async_copy(xT_hbm.at[:, _chunk(rb)], x_c.at[rb], xsem.at[rb])
    def cp_o(rb): return pltpu.make_async_copy(out_c.at[rb], outT_hbm.at[:, _chunk(rb)], xsem.at[rb])
    cp_wq00 = cp_w(wq_hbm, wq_v, S_WQ0, 0)
    cp_wo0 = cp_w(woT_hbm, wo_v, S_WO0, 0)
    cp_wr = pltpu.make_async_copy(wr_hbm, wr_v, sems.at[S_WR])
    cp_c = pltpu.make_async_copy(c_hbm, c_v, sems.at[S_C])
    cp_wm1 = pltpu.make_async_copy(wmod_hbm.at[:, 0:M1], wm1_v, sems.at[S_WM1])
    cp_wm2 = pltpu.make_async_copy(wmod_hbm.at[:, M1:6 * D], wm2_v, sems.at[S_WM2])
    cp_wg = pltpu.make_async_copy(wg_hbm, wg_v, sems.at[S_WG])
    cp_wu = pltpu.make_async_copy(wu_hbm, wu_v, sems.at[S_WU])
    cp_wd = pltpu.make_async_copy(wdT_hbm, wd_v, sems.at[S_WD])

    def wsl(ref, j, rows, hb):
        cols = slice(hb * T, (hb + 1) * T) if isinstance(hb, int) else pl.ds(pl.multiple_of(hb * T, T), T)
        return ref[j % NW, rows, cols]

    def ln1_pieces(rb, pace):
        st = {}
        def mean(b):
            x = x_c[rb, b * RBK:(b + 1) * RBK, :].astype(F32)
            if b > 0 and pace:
                x = (x.reshape(RBK // 8, 8, T) + (st['s'] * 0.0)[None]).reshape(RBK, T)
            t = _sum8(x)
            st['s'] = t if b == 0 else st['s'] + t
            if b == NB - 1:
                st['m'] = jnp.broadcast_to(jnp.sum(st['s'], axis=0, keepdims=True) * (1.0 / D), (8, T))
        def var(b):
            m = st['m'] + st['v'] * 0.0 if (b > 0 and pace) else st['m']
            xc = x_c[rb, b * RBK:(b + 1) * RBK, :].astype(F32).reshape(RBK // 8, 8, T) - m[None]
            t = jnp.sum(xc * xc, axis=0)
            st['v'] = t if b == 0 else st['v'] + t
            if b == NB - 1:
                st['rs'] = lax.rsqrt(jnp.sum(st['v'], axis=0, keepdims=True) * (1.0 / D) + EPS)
        def norm(k):
            k0, k1 = KT[k]
            m = st['m'] + st['z'] * 0.0 if (k > 0 and pace) else st['m']
            xc = (x_c[rb, k0:k1, :].astype(F32).reshape((k1 - k0) // 8, 8, T) - m[None]).reshape(k1 - k0, T)
            xh = xc * st['rs']
            st['z'] = xh[0:8, :]
            h = xh.T * modr[0:1, k0:k1] + modr[1:2, k0:k1]
            h_v[k, _chunk(rb), 0:k1 - k0] = h.astype(BF16)
        return ([lambda b=b: mean(b) for b in range(NB)] + [lambda b=b: var(b) for b in range(NB)]
                + [lambda k=k: norm(k) for k in range(5)])

    def ln2_pieces(rb, pace):
        st = {}
        def resid(b):
            rows = slice(b * RBK, (b + 1) * RBK)
            a = acc[rb, rows, :] + dlt[rb, rows, :]
            if b > 0 and pace:
                a = (a.reshape(RBK // 8, 8, T) + (st['s'] * 0.0)[None]).reshape(RBK, T)
            x1 = x_c[rb, rows, :].astype(F32) + modc[0, rows, :] * a
            x1s[rows, :] = x1
            t = _sum8(x1)
            st['s'] = t if b == 0 else st['s'] + t
            if b == NB - 1:
                st['m'] = jnp.broadcast_to(jnp.sum(st['s'], axis=0, keepdims=True) * (1.0 / D), (8, T))
        def var(b):
            m = st['m'] + st['v'] * 0.0 if (b > 0 and pace) else st['m']
            xm = x1s[b * RBK:(b + 1) * RBK, :].reshape(RBK // 8, 8, T) - m[None]
            t = jnp.sum(xm * xm, axis=0)
            st['v'] = t if b == 0 else st['v'] + t
            if b == NB - 1:
                v = _r(jnp.sum(st['v'], axis=0, keepdims=True) * (1.0 / D))
                st['rd'] = 1.0 / _r(jnp.sqrt(_r(v + EPS)))
                st['mr'] = _r(st['m'])
        def norm(b):
            rows = slice(b * RBK, (b + 1) * RBK)
            x1 = x1s[rows, :]
            mr = st['mr'] + st['r'] * 0.0 if (b > 0 and pace) else st['mr']
            xc = (x1.reshape(RBK // 8, 8, T) - mr[None]).reshape(RBK, T)
            h2 = xc * st['rd'] * modc[2, rows, :] + modc[1, rows, :]
            t = _sum8(h2 * modc[4, rows, :])
            st['r'] = t if b == 0 else st['r'] + t
            h2c[rb, rows, :] = h2.astype(BF16)
            out_c[rb, rows, :] = (x1 + modc[3, rows, :] * h2).astype(BF16)
            if b == NB - 1:
                r_v[pl.ds(rb, 1), :] = _r(jnp.sum(st['r'], axis=0, keepdims=True))
        return ([lambda b=b: resid(b) for b in range(NB)] + [lambda b=b: var(b) for b in range(NB)]
                + [lambda b=b: norm(b) for b in range(NB)])

    def run(pieces):
        for f in pieces:
            f()

    def silu_c8():
        cc = c_v[...].astype(F32)
        return jnp.broadcast_to(cc * jax.nn.sigmoid(cc), (8, D)).astype(BF16)

    def mod_b():
        mod = _r(jnp.dot(silu_c8(), wm2_v[...], preferred_element_type=F32))
        for t in range(4):
            row = mod[0:1, t * D:(t + 1) * D]
            modc[t] = _col(_r(1.0 + row) if t == 2 else row)
        modc[4] = _col(wr_v[...].reshape(1, D).astype(F32))

    def qp_tile(j, hb, rows, t):
        k0, k1 = KT[t]
        return jnp.dot(h_v[t, rows, 0:k1 - k0], wsl(wq_v, j, slice(k0, k1), hb), preferred_element_type=F32)

    def op_piece(j, hb, o_ref, rb, t, mode):
        rows = slice(t * 144, (t + 1) * 144)
        u = lax.dot_general(wsl(wo_v, j, rows, hb), o_ref[...], NT, preferred_element_type=F32)
        if mode == 'zero':
            acc[rb, rows, :] = jnp.zeros((144, T), F32)
        elif mode == 'commit':
            acc[rb, rows, :] += dlt[rb, rows, :]
        else:
            u = dlt[rb, rows, :] + u
        dlt[rb, rows, :] = u

    def unit(j, par, chk, opspec, qpspec, pieces, seq):
        st = dict(l=None, o=None, q=None)
        ps = {}
        extra = {}
        for i, f in enumerate(pieces):
            extra.setdefault((i * len(seq)) // len(pieces), []).append(f)
        for i, (name, t) in enumerate(seq):
            run(extra.get(i, []))
            if name == 'QK':
                s = lax.dot_general(q_scr[par][...], k_v[j % NKV, t * T:(t + 1) * T, :], NT, preferred_element_type=F32)
                p = jnp.exp2(s)
                st['l'] = p if st['l'] is None else st['l'] + p
                ps[t] = p.astype(BF16)
            elif name == 'PV':
                o = jnp.dot(ps[t], v_v[j % NKV, t * T:(t + 1) * T, :], preferred_element_type=F32)
                st['o'] = o if st['o'] is None else st['o'] + o
                if t == 15:
                    l = jnp.sum(st['l'], axis=1, keepdims=True)
                    on = st['o'] * (1.0 / l)
                    o_scr[par][...] = on.astype(BF16)
                    lb = jnp.broadcast_to(l, (T, T))
                    chk['lmin'] = jnp.minimum(chk['lmin'], jnp.min(lb.reshape(T // 8, 8, T), axis=0))
                    chk['z'] = chk['z'] + _sum8(on + lb)
            elif name == 'OP':
                op_piece(opspec[0], opspec[1], o_scr[1 - par], opspec[2], t, opspec[3])
            else:
                d = qp_tile(qpspec[0], qpspec[1], _chunk(qpspec[2]), t)
                st['q'] = d if st['q'] is None else st['q'] + d
                if t == 4:
                    q_scr[1 - par][...] = (st['q'] * QSCALE).astype(BF16)

    def chk_new():
        return dict(lmin=jnp.full((8, T), 1.0, F32), z=jnp.zeros((8, T), F32))

    def chk_put(chk, first):
        if first:
            chk_v[0:8, :] = chk['lmin']
            chk_v[8:16, :] = chk['z']
        else:
            chk_v[0:8, :] = jnp.minimum(chk_v[0:8, :], chk['lmin'])
            chk_v[8:16, :] = chk_v[8:16, :] + chk['z']

    def chk_ok(lmin, z):
        return jnp.min(jnp.where((lmin >= LMIN) & (jnp.abs(z) < jnp.inf), 1.0, 0.0))

    def mid_step(j):
        chk = chk_new()
        for c in range(NPER):
            if c >= 1:
                opspec = (j, (c - 1) % 2, (c - 1) // 2, 'add' if (c - 1) % 2 else 'commit')
            else:
                opspec = (j - 1, 1, NRB - 1, 'add')
            qpspec = (j, (c + 1) % 2, (c + 1) // 2) if c + 1 < NPER else (j + 1, 0, 0)
            unit(j, c % 2, chk, opspec, qpspec, [], SEQ_HEAD if c == 0 else SEQ_TAIL if c == NPER - 1 else SEQ_MID)
        ok_s[0] = chk_ok(chk['lmin'], chk['z'])

    def start_up_copies(it):
        @pl.when(it < 6)
        def _():
            cp_x(2 * it + 4).start(); cp_x(2 * it + 5).start()
        @pl.when(it < 7)
        def _():
            cp_x(2 * it + 2).wait(); cp_x(2 * it + 3).wait()
        @pl.when(it == 1)
        def _():
            cp_wq(1).start(); cp_wr.start()
        @pl.when(it == 2)
        def _():
            cp_k(1).start(); cp_v(1).start()
        @pl.when(it == 3)
        def _():
            cp_wq(1).wait()
            cp_wo(1).start(); cp_wq(2).start()
        @pl.when(it == 4)
        def _():
            cp_wm2.start()

    def edge_step(j, first):
        chk_put(chk_new(), True)
        def body(it, carry):
            chk = chk_new()
            if first:
                start_up_copies(it)
                pa = ln1_pieces(jnp.minimum(2 * it + 2, NRB - 1), True)
                pb = ln1_pieces(jnp.minimum(2 * it + 3, NRB - 1), True)
            else:
                pa = ln2_pieces(jnp.maximum(2 * it - 2, 0), True)
                pb = ln2_pieces(jnp.maximum(2 * it - 1, 0), True)
            pcs = [pa[:len(pa) // 2], pa[len(pa) // 2:], pb[:len(pb) // 2], pb[len(pb) // 2:]]
            for c in range(4):
                if c > 0:
                    mode = 'add' if (c - 1) % 2 else ('zero' if first else 'commit')
                    opspec = (j, (c - 1) % 2, 2 * it + (c - 1) // 2, mode)
                elif first:
                    opspec = (j, 1, jnp.maximum(2 * it - 1, 0), 'add')
                else:
                    opspec = (jnp.where(it == 0, j - 1, j), 1, (2 * it + NRB - 1) % NRB, 'add')
                if c < 3:
                    qpspec = (j, (c + 1) % 2, 2 * it + (c + 1) // 2)
                elif first:
                    qpspec = (jnp.where(it == 7, j + 1, j), 0, (2 * it + 2) % NRB)
                else:
                    qpspec = (j, 0, jnp.minimum(2 * it + 2, NRB - 1))
                unit(j, c % 2, chk, opspec, qpspec, pcs[c], (SEQ_FIRST if first else SEQ_LAST)[c])
            chk_put(chk, False)
            if not first:
                @pl.when(it >= 1)
                def _():
                    cp_o(2 * it - 2).start(); cp_o(2 * it - 1).start()
            return carry
        lax.fori_loop(0, NRB // 2, body, 0)
        ok_s[0] = chk_ok(chk_v[0:8, :], chk_v[8:16, :])

    def slow_step(j):
        def body(c, carry):
            rb = c // 2
            hb = c % 2
            q = None
            for t in range(5):
                d = qp_tile(j, hb, _chunk(rb), t)
                q = d if q is None else q + d
            qs[...] = (q * QSCALE).astype(BF16)
            ms[...] = jnp.full((T, T), -jnp.inf, F32)
            def scores(t, carry_):
                s = lax.dot_general(qs[...], k_v[j % NKV, _chunk(t), :], NT, preferred_element_type=F32)
                ss[t] = s
                ms[...] = jnp.maximum(ms[...], s)
                return carry_
            lax.fori_loop(0, S // T, scores, 0)
            ms[...] = jnp.broadcast_to(jnp.max(ms[...], axis=1, keepdims=True), (T, T))
            ls[...] = jnp.zeros((T, T), F32)
            os_[...] = jnp.zeros((T, T), F32)
            def weights(t, carry_):
                p = jnp.exp2(ss[t] - ms[...])
                ls[...] += p
                os_[...] += jnp.dot(p.astype(BF16), v_v[j % NKV, _chunk(t), :], preferred_element_type=F32)
                return carry_
            lax.fori_loop(0, S // T, weights, 0)
            l = jnp.sum(ls[...], axis=1, keepdims=True)
            o1[...] = (os_[...] * (1.0 / l)).astype(BF16)
            @pl.when(c < NPER - 1)
            def _():
                def proj(t, carry_):
                    rows = pl.ds(pl.multiple_of(t * 144, 16), 144)
                    u = lax.dot_general(wsl(wo_v, j, rows, hb), o1[...], NT, preferred_element_type=F32)
                    dlt[rb, rows, :] = jnp.where(hb == 0, 0.0, dlt[rb, rows, :]) + u
                    return carry_
                lax.fori_loop(0, 4, proj, 0)
                @pl.when(jnp.logical_and(j == HKV - 1, hb == 1))
                def _():
                    run(ln2_pieces(rb, False))
            return carry
        lax.fori_loop(0, NPER, body, 0)

    cp_wm1.start(); cp_c.start(); cp_x(0).start(); cp_wq00.start(); cp_k(0).start()
    o1[...] = jnp.zeros((T, DH), BF16)
    dlt[0] = jnp.zeros((D, T), F32)
    cp_x(0).wait()
    p0 = ln1_pieces(0, False)
    run(p0[:2 * NB])
    cp_v(0).start()
    cp_c.wait(); cp_wm1.wait()
    cp_x(1).start(); cp_wo0.start()
    mod = _r(jnp.dot(silu_c8(), wm1_v[...], preferred_element_type=F32))
    modr[0:1, :] = 1.0 + mod[0:1, D:2 * D]
    modr[1:2, :] = mod[0:1, 0:D]
    run(p0[2 * NB:])
    cp_wq00.wait()
    q = None
    for t in range(5):
        d = qp_tile(0, 0, _chunk(0), t)
        q = d if q is None else q + d
    q0[...] = (q * QSCALE).astype(BF16)
    cp_x(2).start(); cp_x(3).start()
    cp_x(1).wait()
    run(ln1_pieces(1, False))
    cp_k(0).wait(); cp_v(0).wait(); cp_wo0.wait()

    def step(j, carry):
        @pl.when(j == 0)
        def _():
            edge_step(0, True)

        @pl.when(jnp.logical_and(j > 0, j < HKV - 1))
        def _():
            cp_k(j).wait(); cp_v(j).wait(); cp_wo(j).wait(); cp_wq(j + 1).wait()
            @pl.when(j + 2 < HKV)
            def _():
                cp_wq(j + 2).start()
            @pl.when(j == 1)
            def _():
                cp_wm2.wait(); cp_wr.wait()
                mod_b()
                cp_wg.start()
            @pl.when(j == 2)
            def _():
                cp_wu.start()
            @pl.when(j == 3)
            def _():
                cp_wd.start()
            cp_k(j + 1).start(); cp_v(j + 1).start(); cp_wo(j + 1).start()
            mid_step(j)

        @pl.when(j == HKV - 1)
        def _():
            cp_k(HKV - 1).wait(); cp_v(HKV - 1).wait(); cp_wo(HKV - 1).wait()
            edge_step(HKV - 1, False)
            run(ln2_pieces(NRB - 2, False))

        @pl.when(ok_s[0] < 0.5)
        def _():
            @pl.when(j == HKV - 1)
            def _():
                for rb in range(NRB - 2):
                    cp_o(rb).wait()
            slow_step(j)
            @pl.when(j == HKV - 1)
            def _():
                for rb in range(NRB - 2):
                    cp_o(rb).start()
        return carry
    lax.fori_loop(0, HKV, step, 0)

    cp_o(NRB - 2).start()
    for t in range(4):
        op_piece(HKV - 1, 1, o1, NRB - 1, t, 'add')
    run(ln2_pieces(NRB - 1, False))
    cp_o(NRB - 1).start()

    bits = pltpu.bitcast(r_v[...], jnp.int32) >> 16
    u = jnp.where(bits < 0, ~bits, bits | 0x8000) & 0xFFFF
    tok = lax.broadcasted_iota(jnp.int32, (NRB, T), 0) * T + lax.broadcasted_iota(jnp.int32, (NRB, T), 1)
    key = pltpu.bitcast(((u << 11) | (S - 1 - tok)) + (1 << 27), F32)
    subs = lax.broadcasted_iota(jnp.int32, (8, T), 0)
    lane = lax.broadcasted_iota(jnp.int32, (8, T), 1)
    ksel = jnp.zeros((8, T), jnp.int32)
    for t in range(C):
        mx = jnp.max(jnp.max(key, axis=0, keepdims=True), axis=1, keepdims=True)
        key = jnp.where(key == mx, 0.0, key)
        ksel = jnp.where(subs == t, pltpu.bitcast(jnp.broadcast_to(mx, (8, T)), jnp.int32), ksel)
    ksel = ksel - (1 << 27)
    idxv = (S - 1) - (ksel & (S - 1))
    uu = ksel >> 11
    rsel = pltpu.bitcast(jnp.where((uu & 0x8000) != 0, uu & 0x7FFF, (~uu) & 0xFFFF) << 16, F32)
    idxs = [jnp.max(jnp.where(subs == t, idxv, 0).astype(F32)).astype(jnp.int32) for t in range(C)]
    tiles = [jnp.clip(idxs[t] // T, 0, NRB - 1) for t in range(C)]

    xs = None
    for t in range(C):
        oh = jnp.where((subs == t) & (lane == (idxv & (T - 1))), 1.0, 0.0).astype(BF16)
        d = lax.dot_general(oh, h2c[tiles[t]], NT, preferred_element_type=F32)
        xs = d if xs is None else xs + d

    cp_wg.wait(); cp_wu.wait(); cp_wd.wait()
    xb = xs.astype(BF16)
    g = _r(jnp.dot(xb, wg_v[...], preferred_element_type=F32))
    up = _r(jnp.dot(xb, wu_v[...], preferred_element_type=F32))
    g = _r(g * jax.nn.sigmoid(g))
    a = (g * up).astype(BF16)
    y = _r(lax.dot_general(a, wd_v[...], NT, preferred_element_type=F32))
    y = _r(y * _r(jax.nn.sigmoid(rsel[:, 0:1])))

    for rb in range(NRB):
        cp_o(rb).wait()
    yT = jnp.concatenate([y, jnp.zeros((T - C, D), F32)], axis=0).T.astype(BF16)
    rowk = lax.broadcasted_iota(jnp.int32, (T, T), 0)
    lanes = lax.broadcasted_iota(jnp.int32, (T, T), 1)
    final = []
    for t in range(C):
        f = jnp.bool_(True)
        for s in range(t + 1, C):
            f = jnp.logical_and(f, tiles[s] != tiles[t])
        final.append(f)
    for g0 in range(0, C, 2):
        for t in range(g0, g0 + 2):
            sel = jnp.where((rowk == t) & (lanes == (idxs[t] & (T - 1))), 1.0, 0.0).astype(BF16)
            for p in range(4):
                rows = slice(p * 144, (p + 1) * 144)
                upd = jnp.dot(yT[rows, :], sel, preferred_element_type=F32)
                out_c[tiles[t], rows, :] = (out_c[tiles[t], rows, :].astype(F32) + modc[3, rows, :] * upd).astype(BF16)
        for t in range(g0, g0 + 2):
            @pl.when(final[t])
            def _(t=t):
                cp_o(tiles[t]).start()
    for t in range(C):
        @pl.when(final[t])
        def _(t=t):
            cp_o(tiles[t]).wait()


@jax.jit
def pallas_adaLN_cond__gqa_block_cached__moe_arch_mod__prompt_kernel(
    A_x: jax.Array,
    A_k_cache: jax.Array,
    A_v_cache: jax.Array,
    A_wq: jax.Array,
    A_wo: jax.Array,
    B_x: jax.Array,
    B_w_r: jax.Array,
    B_w_gate: jax.Array,
    B_w_up: jax.Array,
    B_w_down: jax.Array,
    c: jax.Array,
    w_mod: jax.Array,
):
    del B_x
    any_spec = pl.BlockSpec(memory_space=pl.ANY)
    tile = pltpu.VMEM((T, DH), BF16)
    outT = pl.pallas_call(
        _kernel,
        in_specs=[any_spec] * 11,
        out_specs=any_spec,
        out_shape=jax.ShapeDtypeStruct((D, S), BF16),
        scratch_shapes=[
            pltpu.VMEM((NRB, D, T), BF16),
            pltpu.VMEM((NKV, S, DH), BF16),
            pltpu.VMEM((NKV, S, DH), BF16),
            pltpu.VMEM((NW, D, 2 * T), BF16),
            pltpu.VMEM((NW, D, 2 * T), BF16),
            pltpu.VMEM((D,), BF16),
            pltpu.VMEM((1, D), BF16),
            pltpu.VMEM((D, M1), BF16),
            pltpu.VMEM((D, 4 * D), BF16),
            pltpu.VMEM((D, FF), BF16),
            pltpu.VMEM((D, FF), BF16),
            pltpu.VMEM((D, FF), BF16),
            pltpu.VMEM((8, D), F32),
            pltpu.VMEM((5, D, T), F32),
            pltpu.VMEM((5, S, T), BF16),
            pltpu.VMEM((NRB, D, T), F32),
            pltpu.VMEM((NRB, D, T), F32),
            tile, tile, tile, tile,
            pltpu.VMEM((NRB, D, T), BF16),
            pltpu.VMEM((NRB, D, T), BF16),
            pltpu.VMEM((NRB, T), F32),
            pltpu.VMEM((D, T), F32),
            tile,
            pltpu.VMEM((S // T, T, T), F32),
            pltpu.VMEM((T, T), F32), pltpu.VMEM((T, T), F32), pltpu.VMEM((T, T), F32),
            pltpu.VMEM((16, T), F32),
            pltpu.SMEM((1,), F32),
            pltpu.SemaphoreType.DMA((NRB,)),
            pltpu.SemaphoreType.DMA((14,)),
        ],
        compiler_params=pltpu.CompilerParams(vmem_limit_bytes=100 * 1024 * 1024),
    )(A_x.reshape(S, D).T, A_k_cache.reshape(HKV, S, DH), A_v_cache.reshape(HKV, S, DH), A_wq, A_wo.T,
      B_w_r, B_w_gate, B_w_up, B_w_down.T, c, w_mod)
    return outT.T.reshape(1, S, D)
```
